```python
import jax
import jax.numpy as jnp

def _softmax(x, axis=-1):
    return jax.nn.softmax(x, axis=axis)

def _gelu(x):
    return jax.nn.gelu(x, approximate=True)

def _silu(x):
    return jax.nn.silu(x)

def _sigmoid(x):
    return jax.nn.sigmoid(x)

def _layernorm(x, axis=-1, eps=1e-05):
    m = jnp.mean(x, axis=axis, keepdims=True)
    v = jnp.var(x, axis=axis, keepdims=True)
    return (x - m) / jnp.sqrt(v + eps)

def _scatter_add(tgt, idx, src, axis=0):
    return tgt.at[idx].add(src)

def _segment_sum(src, seg, n):
    return jax.ops.segment_sum(src, seg, n)

class _Rng:

    def __init__(self, key):
        self._k = key

    def _next(self):
        self._k, sub = jax.random.split(self._k)
        return sub

    def normal(self, shape):
        return jax.random.normal(self._next(), shape, dtype=jnp.bfloat16)

    def randint(self, lo, hi, shape):
        return jax.random.randint(self._next(), shape, lo, hi, dtype=jnp.int32)

    def uniform(self, shape, lo=0.0, hi=1.0):
        return jax.random.uniform(self._next(), shape, jnp.bfloat16, lo, hi)

    def permutation(self, n):
        return jax.random.permutation(self._next(), n)
kernel_name = 'concat_heads__spectral_gfnet__memory_aug_recurrent_mem_tr__prompt'

def setup_inputs():
    _rng = _Rng(jax.random.key(int.from_bytes(__import__("os").urandom(4), "little")))
    _w = lambda a: (lambda t: t.astype(jnp.bfloat16) if jnp.issubdtype(t.dtype, jnp.floating) else t)(jnp.asarray(a))

    def _A_setup():
        B, S, D = (1, 2048, 1024)
        Df = D // 2 + 1
        return {'x': _w((lambda *s: _rng.normal(s) * 0.05)(B, S, D)), 'w_r': _w((lambda *s: _rng.normal(s) * 0.05)(S, Df) * 0.02), 'w_i': _w((lambda *s: _rng.normal(s) * 0.05)(S, Df) * 0.02)}
    _A_in = _A_setup()

    def _B_setup():
        B, S, Dm = (1, 2048, 1024)
        H, Dh = (32, 128)
        M, seg = (8, 32)
        seg = min(seg, S)
        S = S // seg * seg
        return {'x': _w((lambda *s: _rng.normal(s) * 0.05)(B, S, Dm)), 'mem0': _w((lambda *s: _rng.normal(s) * 0.05)(B, M, Dm)), 'Wq': _w((lambda *s: _rng.normal(s) * 0.05)(Dm, H, Dh) * Dm ** (-0.5)), 'Wk': _w((lambda *s: _rng.normal(s) * 0.05)(Dm, H, Dh) * Dm ** (-0.5)), 'Wv': _w((lambda *s: _rng.normal(s) * 0.05)(Dm, H, Dh) * Dm ** (-0.5)), 'Wo': _w((lambda *s: _rng.normal(s) * 0.05)(H, Dh, Dm) * (H * Dh) ** (-0.5)), 'seg_len': seg}
    _B_in = _B_setup()
    return {'A_x': _A_in['x'], 'A_w_r': _A_in['w_r'], 'A_w_i': _A_in['w_i'], 'B_x': _B_in['x'], 'B_mem0': _B_in['mem0'], 'B_Wq': _B_in['Wq'], 'B_Wk': _B_in['Wk'], 'B_Wv': _B_in['Wv'], 'B_Wo': _B_in['Wo'], 'B_seg_len': _B_in['seg_len']}

def reference(A_x, A_w_r, A_w_i, B_x, B_mem0, B_Wq, B_Wk, B_Wv, B_Wo, B_seg_len):

    def _A_ref(x, w_r, w_i):
        B, S, D = x.shape
        X = (lambda x, axes=(-2, -1): jnp.fft.rfft2(x.astype(jnp.float32), axes=axes))(x, axes=(-2, -1))
        W = w_r + 1j * w_i
        X = X * W
        y = (lambda x, s, axes=(-2, -1): jnp.fft.irfft2(x, s=s, axes=axes).astype(jnp.bfloat16))(X, (S, D), axes=(-2, -1))
        return y

    def _B_ref(x, mem0, Wq, Wk, Wv, Wo, seg_len):
        B, S, Dm = x.shape
        H, Dh = (Wq.shape[1], Wq.shape[2])
        M = mem0.shape[1]
        scale = Dh ** (-0.5)
        n_seg = S // seg_len
        L = M + seg_len
        idx = jnp.arange(L)
        mask = (idx[:, None] < M) | (idx[:, None] >= idx[None, :])
        mem = mem0
        outs = []
        for s in range(n_seg):
            xs = x[:, s * seg_len:(s + 1) * seg_len, :].copy()
            h = jnp.concatenate([mem, xs], axis=1)
            q = jnp.einsum('btd,dhe->bhte', h, Wq)
            k = jnp.einsum('btd,dhe->bhte', h, Wk)
            v = jnp.einsum('btd,dhe->bhte', h, Wv)
            scores = jnp.einsum('bhqe,bhke->bhqk', q, k) * scale
            scores = jnp.where(mask[None, None], scores, -1000000000.0)
            p = _softmax(scores, axis=-1)
            o = jnp.einsum('bhqk,bhke->bhqe', p, v)
            o = jnp.einsum('bhte,hed->btd', o, Wo)
            mem = o[:, :M, :].copy()
            outs.append(o[:, M:, :])
        return jnp.concatenate(outs, axis=1)
    a = _A_ref(A_x, A_w_r, A_w_i)
    b = _B_ref(B_x, B_mem0, B_Wq, B_Wk, B_Wv, B_Wo, B_seg_len)
    return jnp.concatenate([a, b], axis=-1)
```

```python
import functools

import numpy as np
import jax
import jax.numpy as jnp
from jax import lax
import jax.experimental.pallas as pl
import jax.experimental.pallas.tpu as pltpu

S, D = 2048, 1024
H, DH = 32, 128
NMEM, SEG = 8, 32
NSEG = S // SEG
NPRE = NSEG * 8

F32, BF16, U32 = jnp.float32, jnp.bfloat16, jnp.uint32
_SQH = float(np.sqrt(0.5))
_C8, _S8 = float(np.cos(np.pi / 8)), float(np.sin(np.pi / 8))


def _pack_rows(m):
    b = np.asarray(m, np.float32).astype(jnp.bfloat16).view(np.uint16).astype(np.uint32)
    return b[..., 0::2, :] | (b[..., 1::2, :] << 16)


@functools.lru_cache(maxsize=None)
def _fft_constants():
    cls = {0: 0, 4: 0, 1: 1, 7: 1, 2: 2, 6: 2, 3: 3, 5: 3}
    kf = np.zeros((4, 128), np.int64)
    perm = np.zeros((4, 128, 128))
    for g in range(4):
        for t in range(4):
            js = [j for j in range(128) if cls[j % 8] == t]
            c = (t + g) % 4
            for i, j in enumerate(js):
                kf[t, 32 * c + i] = 128 * g + j
                perm[g, j, 32 * c + i] = 1.0
    d1 = np.arange(128)[:, None]
    mf = np.zeros((4, 256, 256))
    mi = np.zeros((4, 256, 256))
    for t in range(4):
        k = kf[t][None, :]
        th = 2 * np.pi * ((d1 * k) % D) / D
        co, si = np.cos(th), np.sin(th)
        r = k % 8
        if t == 0:
            m0, m4 = (r == 0), (r == 4)
            mf[t] = np.block([[co * m0, -si * m0], [co * m4, -si * m4]])
        else:
            sg = (-1.0 if t in (1, 2) else 1.0) * np.where(r == t, 1.0, -1.0)
            mf[t] = np.block([[co, -si], [sg * si, sg * co]])
        ck = np.where(kf[t] == 0, 1.0, 2.0) / (S * D)
        mi[t] = (mf[t] * np.concatenate([ck, ck])[None, :]).T
    nyq = np.zeros((128, 128))
    nyq[:, 0] = (-1.0) ** np.arange(128)
    small = np.concatenate([perm, nyq[None], nyq.T[None] / (S * D)], axis=0)
    m = np.arange(128)[:, None]
    s1 = np.arange(128)[None, :]
    gf = np.zeros((16, 256, 256))
    gi = np.zeros((16, 256, 256))
    for r in range(16):
        th = 2 * np.pi * ((s1 * (16 * m + r)) % S) / S
        gr, gim = np.cos(th), -np.sin(th)
        g = np.block([[gr, -gim], [gim, gr]])
        gf[r, :, 0::2], gf[r, :, 1::2] = g[:, :128], g[:, 128:]
        gi[r, :, 0::2], gi[r, :, 1::2] = g.T[:, :128], g.T[:, 128:]
    return (_pack_rows(np.concatenate([mf, mi], axis=0)), _pack_rows(small),
            _pack_rows(gf), _pack_rows(gi))


def _bfly8(x):
    x0, x1, x2, x3, x4, x5, x6, x7 = x
    t0, t1, t2, t3 = x0 + x4, x0 - x4, x2 + x6, x2 - x6
    t4, t5, t6, t7 = x1 + x5, x1 - x5, x3 + x7, x3 - x7
    u0, u1, u2, u3 = t0 + t2, t0 - t2, t4 + t6, t4 - t6
    p, q = _SQH * (t5 - t7), _SQH * (t5 + t7)
    return [(u0 + u2, u0 - u2), (t1 + p, t3 + q), (u1, u3), (t1 - p, t3 - q)]


def _bfly8_t(planes):
    (a0, a4), (a1r, a1i), (u1, u3), (a3r, a3i) = planes
    u0, u2 = a0 + a4, a0 - a4
    t1, p, t3, q = a1r + a3r, a1r - a3r, a1i + a3i, a1i - a3i
    t5, t7 = _SQH * (p + q), _SQH * (q - p)
    t0, t2, t4, t6 = u0 + u1, u0 - u1, u2 + u3, u2 - u3
    return [t0 + t1, t4 + t5, t2 + t3, t6 + t7, t0 - t1, t4 - t5, t2 - t3, t6 - t7]


def _dft4(z):
    (ar, ai), (br, bi), (cr, ci), (dr, di) = z
    er, ei, fr, fi = ar + cr, ai + ci, ar - cr, ai - ci
    gr, gi, hr, hi = br + dr, bi + di, br - dr, bi - di
    return [(er + gr, ei + gi), (fr + hi, fi - hr), (er - gr, ei - gi), (fr - hi, fi + hr)]


def _twiddle16(z, e):
    re, im = z
    if e == 0:
        return z
    if e == 4:
        return im, -re
    if e == 2:
        return _SQH * (re + im), _SQH * (im - re)
    if e == 6:
        return _SQH * (im - re), -_SQH * (re + im)
    c, s = {1: (_C8, _S8), 3: (_S8, _C8), 9: (-_C8, -_S8)}[e]
    return re * c + im * s, im * c - re * s


def _dft16(z):
    cols = [_dft4([z[a + 4 * b] for b in range(4)]) for a in range(4)]
    out = [None] * 16
    for r1 in range(4):
        y = _dft4([_twiddle16(cols[a][r1], a * r1) for a in range(4)])
        for r2 in range(4):
            out[r1 + 4 * r2] = y[r2]
    return out


def _idft16(z):
    return [(re, im) for im, re in _dft16([(im, re) for re, im in z])]


def _bf(x):
    return pltpu.bitcast(x, BF16)


def _dot(a, b):
    return jnp.dot(a, b, preferred_element_type=F32)


def _dot_nt(a, b):
    return lax.dot_general(a, b, (((1,), (1,)), ((), ())), preferred_element_type=F32)


def _kernel(ax_hbm, wr_hbm, wi_hbm, bx_hbm, mem0_hbm, wq_hbm, wk_hbm, wv_hbm, wo_hbm,
            md_hbm, ms_hbm, gf_hbm, gi_hbm,
            out_hbm,
            xa, wf, wnyq, md, ms, gf, gi, ybuf, ubuf, ystage,
            xs, xpre3, xpre, stage, wostage, wqkv, wo, pre, kvmem, obuf, opre,
            sem_xa, sem_c, sem_w, sem_wo, sem_b, sem_y, sem_o):
    copy = pltpu.make_async_copy
    w_hbm = (wq_hbm, wk_hbm, wv_hbm)

    def xa_copy(c):
        return copy(ax_hbm.at[:, c], xa.at[c], sem_xa.at[c])

    const_copies = [copy(md_hbm, md, sem_c.at[0]), copy(ms_hbm, ms, sem_c.at[1]),
                    copy(gf_hbm, gf, sem_c.at[2]), copy(gi_hbm, gi, sem_c.at[3])]
    for i, f_hbm in enumerate((wr_hbm, wi_hbm)):
        for g in range(4):
            const_copies.append(copy(f_hbm.bitcast(U32).at[:, pl.ds(128 * g, 128)],
                                     wf.at[pl.ds((5 * i + g) * (S // 2), S // 2)],
                                     sem_c.at[4 + 5 * i + g]))
        const_copies.append(copy(f_hbm.at[:, pl.ds(512, 1)], wnyq.at[i], sem_c.at[8 + 5 * i]))
    xpre_copy = copy(bx_hbm.at[:, 0], xpre3, sem_b.at[0])
    xs_copy = copy(bx_hbm.at[:, pl.ds(1, 3)], xs.at[pl.ds(0, NSEG), pl.ds(1, 3)], sem_b.at[1])
    mem_copy = copy(mem0_hbm, xs.at[0, 0], sem_b.at[2])

    def w_copy(piece):
        half, mat = divmod(piece, 3)
        src = w_hbm[mat].bitcast(U32).at[:, pl.ds(8 * half, 8), :]
        return copy(src, stage.at[piece % 2], sem_w.at[piece % 2])

    def wo_copy(i):
        return copy(wo_hbm.at[pl.ds(1024 * i, 1024)], wostage.at[i % 2], sem_wo.at[i % 2])

    def y_copy(c, slot):
        return copy(ystage.at[slot], out_hbm.at[:, c, :, pl.ds(0, D)], sem_y.at[slot])

    def o_copy(s):
        return copy(xs.at[s, pl.ds(1, 3)],
                    out_hbm.at[s // 4, pl.ds(4 * (s % 4) + 1, 3), :, pl.ds(D, D)], sem_o.at[0])

    def opre_copy(s):
        return copy(xs.at[s, 0], out_hbm.at[s // 4, 4 * (s % 4), :, pl.ds(D, D)], sem_o.at[1])

    const_copies[0].start()
    const_copies[1].start()
    for c in range(16):
        xa_copy(c).start()
    for cp in const_copies[2:]:
        cp.start()
    xpre_copy.start()
    w_copy(0).start()
    w_copy(1).start()
    xs_copy.start()
    mem_copy.start()
    wo_copy(0).start()
    wo_copy(1).start()

    const_copies[0].wait()
    const_copies[1].wait()

    def a_forward(c, carry):
        xa_copy(c).wait()
        x = xa[c].astype(F32).reshape(128, D)
        planes = _bfly8([x[:, 128 * i:128 * (i + 1)] for i in range(8)])
        row = pl.ds(pl.multiple_of(c * 8, 8), 8)
        for t in range(5):
            if t < 4:
                lhs = jnp.concatenate(planes[t], axis=1).astype(BF16)
                x1 = _dot(lhs, _bf(md[t]))
                re, im = x1[:, :128], x1[:, 128:]
            else:
                re = _dot(planes[0][0].astype(BF16), _bf(ms[4]))
                im = jnp.zeros_like(re)
            y = _dft16([(re[8 * b:8 * b + 8], im[8 * b:8 * b + 8]) for b in range(16)])
            for r in range(16):
                ybuf[r, row, 128 * t:128 * (t + 1)] = pltpu.pack_elementwise(
                    list(y[r]), packed_dtype=BF16)
        return carry

    lax.fori_loop(0, 16, a_forward, 0)

    for cp in const_copies[2:]:
        cp.wait()
    for i in range(2):
        lane0 = lax.broadcasted_iota(jnp.int32, (S, 128), 1) == 0
        wf[pl.ds((5 * i + 4) * (S // 2), S // 2), :] = pltpu.bitcast(
            jnp.where(lane0, wnyq[i].astype(F32), 0.0).astype(BF16), U32)

    def a_filter(r, carry):
        shift = (16 * (1 - r % 2)).astype(U32)
        lane = lax.broadcasted_iota(jnp.int32, (128, 128), 1)
        grp = lane // 32

        def filt(i):
            def rows(g):
                w = wf[pl.ds((5 * i + g) * (S // 2) + r // 2, 128, stride=8), :]
                return pltpu.bitcast((w << shift) & jnp.uint32(0xFFFF0000), F32)
            pg = [_dot(rows(g).astype(BF16), _bf(ms[g])) for g in range(4)]
            out = []
            for t in range(4):
                o = pg[(0 - t) % 4]
                for c in range(1, 4):
                    o = jnp.where(grp == c, pg[(c - t) % 4], o)
                out.append(o)
            out.append(rows(4))
            return out

        fr, fi = filt(0), filt(1)
        x2 = _dot(_bf(gf[r]), _bf(ybuf[r]))
        z = []
        for t in range(5):
            a, b = x2[:128, 128 * t:128 * (t + 1)], x2[128:, 128 * t:128 * (t + 1)]
            z.append(pltpu.pack_elementwise(
                [a * fr[t] - b * fi[t], a * fi[t] + b * fr[t]], packed_dtype=BF16))
        ubuf[r] = _dot(_bf(gi[r]), _bf(jnp.concatenate(z, axis=1)))
        return carry

    lax.fori_loop(0, 16, a_filter, 0)

    def a_inverse(c, carry):
        slot = c % 2
        r0 = pl.multiple_of(c * 8, 8)
        planes = []
        for t in range(5):
            cols = slice(128 * t, 128 * (t + 1))
            x3 = _idft16([(ubuf[r, pl.ds(r0, 8), cols], ubuf[r, pl.ds(128 + r0, 8), cols])
                          for r in range(16)])
            re = jnp.concatenate([v[0] for v in x3], axis=0)
            if t < 4:
                im = jnp.concatenate([v[1] for v in x3], axis=0)
                o = _dot(jnp.concatenate([re, im], axis=1).astype(BF16), _bf(md[4 + t]))
                planes.append([o[:, :128], o[:, 128:]])
            else:
                planes[0][0] = planes[0][0] + _dot(re.astype(BF16), _bf(ms[5]))
        y = jnp.concatenate(_bfly8_t(planes), axis=1)

        @pl.when(c >= 2)
        def _():
            y_copy(c - 2, slot).wait()

        ystage[slot] = y.reshape(16, 8, D).astype(BF16)
        y_copy(c, slot).start()
        return carry

    lax.fori_loop(0, 16, a_inverse, 0)

    xpre_copy.wait()
    xpre[...] = pltpu.bitcast(xpre3[...].reshape(NPRE, D), U32)
    stage2 = stage.reshape(2 * 8192, 128)

    for piece in range(6):
        half, mat = divmod(piece, 3)
        w_copy(piece).wait()

        def project(j, carry, piece=piece, half=half, mat=mat):
            ev = stage2[pl.ds((piece % 2) * 8192 + j, 512, stride=16), :]
            od = stage2[pl.ds((piece % 2) * 8192 + j + 8, 512, stride=16), :]
            lo = (ev & jnp.uint32(0xFFFF)) | (od << 16)
            hi = (ev >> 16) | (od & jnp.uint32(0xFFFF0000))
            head = 16 * half + 2 * j
            wqkv[3 * head + mat] = lo
            wqkv[3 * (head + 1) + mat] = hi
            p = _dot(_bf(xpre[...]), _bf(jnp.concatenate([lo, hi], axis=1))).astype(BF16)
            pre[mat, head] = p[:, :DH]
            pre[mat, head + 1] = p[:, DH:]
            return carry

        lax.fori_loop(0, 8, project, 0)
        if piece + 2 < 6:
            w_copy(piece + 2).start()
        if piece < 4:
            wo_copy(piece).wait()
            wo[pl.ds(512 * piece, 512), :] = pltpu.bitcast(wostage[piece % 2], U32)
            if piece + 2 < 4:
                wo_copy(piece + 2).start()

    xs_copy.wait()
    mem_copy.wait()
    scale = DH ** -0.5

    def step(s, carry):
        row = lax.broadcasted_iota(jnp.int32, (32, 48), 0)
        col = lax.broadcasted_iota(jnp.int32, (32, 48), 1)
        allowed = ((row < NMEM) | (col >= 32) | (col <= row)) & (col < 40)
        p0 = pl.ds(pl.multiple_of(s * 8, 8), 8)
        h = xs[s].reshape(32, D)
        zeros = jnp.zeros((8, DH), BF16)
        st = {}

        def qkv(hd):
            q, k, v = [_dot(h, _bf(wqkv[3 * hd + i])).astype(BF16) for i in range(3)]
            kvmem[0, hd, p0, :] = k[:NMEM]
            kvmem[1, hd, p0, :] = v[:NMEM]
            st[hd] = (q, k, v)

        def scores(hd):
            q, k, v = st[hd]
            ka = jnp.concatenate([k, pre[1, hd, p0, :], zeros], axis=0)
            sc = jnp.where(allowed, _dot_nt(q, ka) * scale, -jnp.inf)
            e = jnp.exp(sc - jnp.max(sc, axis=-1, keepdims=True))
            st[hd] = (e.astype(BF16), 1.0 / jnp.sum(e, axis=-1, keepdims=True), v)

        def context(hd):
            e, rl, v = st.pop(hd)
            va = jnp.concatenate([v, pre[2, hd, p0, :], zeros], axis=0)
            obuf[:, hd * DH:(hd + 1) * DH] = (_dot(e, va) * rl).astype(BF16)

        d1, d2, grp = 1, 3, 4
        for hd in range(H):
            qkv(hd)
            if hd >= d1:
                scores(hd - d1)
            if hd >= d2:
                context(hd - d2)
        acc = None
        for g in range(H // grp):
            t = _dot(obuf[:, g * grp * DH:(g + 1) * grp * DH],
                     _bf(wo[g * grp * 64:(g + 1) * grp * 64, :]))
            acc = t if acc is None else acc + t
            if H + g - d1 < H:
                scores(H + g - d1)
            if H + g - d2 < H:
                context(H + g - d2)
        ob = acc.astype(BF16).reshape(4, 8, D)
        xs[s, pl.ds(1, 3)] = ob[1:]
        xs[s + 1, 0] = ob[0]
        o_copy(s).start()
        return carry

    lax.fori_loop(0, NSEG, step, 0)

    def finish(g, carry):
        row = lax.broadcasted_iota(jnp.int32, (64, 128), 0)
        col = lax.broadcasted_iota(jnp.int32, (64, 128), 1)
        allowed = ((col % 64) // 8 == row // 8) & ((col < 64) | (col % 8 <= row % 8))
        for hd in range(H):
            for a in range(2):
                rows = pl.ds(pl.multiple_of(g * 128 + a * 64, 64), 64)
                ka = jnp.concatenate([kvmem[0, hd, rows, :], pre[1, hd, rows, :]], axis=0)
                va = jnp.concatenate([kvmem[1, hd, rows, :], pre[2, hd, rows, :]], axis=0)
                sc = jnp.where(allowed, _dot_nt(pre[0, hd, rows, :], ka) * scale, -jnp.inf)
                e = jnp.exp(sc - jnp.max(sc, axis=-1, keepdims=True))
                o = _dot(e.astype(BF16), va) * (1.0 / jnp.sum(e, axis=-1, keepdims=True))
                opre[a * 64:(a + 1) * 64, hd * DH:(hd + 1) * DH] = o.astype(BF16)
        y = _dot(opre[...], _bf(wo[...])).astype(BF16)
        xs[pl.ds(g * 16, 16), 0] = y.reshape(16, 8, D)
        for i in range(16):
            opre_copy(g * 16 + i).start()
        return carry

    lax.fori_loop(0, 4, finish, 0)

    y_copy(14, 0).wait()
    y_copy(15, 1).wait()

    def drain(s, carry):
        o_copy(s).wait()
        opre_copy(s).wait()
        return carry

    lax.fori_loop(0, NSEG, drain, 0)


@functools.partial(jax.jit, static_argnames=("B_seg_len",))
def pallas_concat_heads__spectral_gfnet__memory_aug_recurrent_mem_tr__prompt_kernel(
    A_x, A_w_r, A_w_i, B_x, B_mem0, B_Wq, B_Wk, B_Wv, B_Wo, B_seg_len=SEG,
):
    assert A_x.shape == (1, S, D) and B_x.shape == (1, S, D)
    assert A_w_r.shape == A_w_i.shape == (S, D // 2 + 1)
    assert B_mem0.shape == (1, NMEM, D) and B_seg_len == SEG
    assert B_Wq.shape == B_Wk.shape == B_Wv.shape == (D, H, DH) and B_Wo.shape == (H, DH, D)

    vmem = pltpu.VMEM
    dma = pltpu.SemaphoreType.DMA
    scratch = [
        vmem((16, 16, 8, D), BF16),
        vmem((10 * S // 2, 128), U32),
        vmem((2, S, 1), BF16),
        vmem((8, 128, 256), U32),
        vmem((6, 64, 128), U32),
        vmem((16, 128, 256), U32),
        vmem((16, 128, 256), U32),
        vmem((16, 128, 640), U32),
        vmem((16, 256, 640), F32),
        vmem((2, 16, 8, D), BF16),
        vmem((NSEG + 1, 4, 8, D), BF16),
        vmem((NSEG, 8, D), BF16),
        vmem((NPRE // 2, D), U32),
        vmem((2, D, 8, 128), U32),
        vmem((2, 1024, D), BF16),
        vmem((3 * H, D // 2, DH), U32),
        vmem((H * DH // 2, D), U32),
        vmem((3, H, NPRE, DH), BF16),
        vmem((2, H, NPRE, DH), BF16),
        vmem((32, H * DH), BF16),
        vmem((128, H * DH), BF16),
        dma((16,)), dma((14,)), dma((2,)), dma((2,)), dma((3,)), dma((2,)), dma((2,)),
    ]
    out = pl.pallas_call(
        _kernel,
        out_shape=jax.ShapeDtypeStruct((16, 16, 8, 2 * D), BF16),
        in_specs=[pl.BlockSpec(memory_space=pl.ANY)] * 13,
        out_specs=pl.BlockSpec(memory_space=pl.ANY),
        scratch_shapes=scratch,
        compiler_params=pltpu.CompilerParams(vmem_limit_bytes=124 * 1024 * 1024),
    )(A_x.reshape(16, 16, 8, D), A_w_r, A_w_i,
      B_x.reshape(NSEG, 4, 8, D), B_mem0.reshape(NMEM, D),
      B_Wq, B_Wk, B_Wv, B_Wo.reshape(H * DH, D),
      *[jnp.asarray(c) for c in _fft_constants()])
    return out.reshape(1, S, 2 * D)
```

```python
import functools

import numpy as np
import jax
import jax.numpy as jnp
from jax import lax
import jax.experimental.pallas as pl
import jax.experimental.pallas.tpu as pltpu

S, D = 2048, 1024
H, DH = 32, 128
NMEM, SEG = 8, 32
NSEG = S // SEG
NPRE = NSEG * 8
NSLOT = 12

F32, BF16, U32 = jnp.float32, jnp.bfloat16, jnp.uint32
_SQH = float(np.sqrt(0.5))
_C8, _S8 = float(np.cos(np.pi / 8)), float(np.sin(np.pi / 8))


def _pack_rows(m):
    b = np.asarray(m, np.float32).astype(jnp.bfloat16).view(np.uint16).astype(np.uint32)
    return b[..., 0::2, :] | (b[..., 1::2, :] << 16)


@functools.lru_cache(maxsize=None)
def _fft_constants():
    d1 = np.arange(128)[:, None]
    mf = np.zeros((4, 256, 256))
    mi = np.zeros((4, 256, 256))
    for t, res in enumerate(((0, 4), (1, 7), (2, 6), (3, 5))):
        kf = 8 * (np.arange(128) % 64) + np.repeat(res, 64)
        k = kf[None, :]
        th = 2 * np.pi * ((d1 * k) % D) / D
        co, si = np.cos(th), np.sin(th)
        if t == 0:
            m0, m4 = (k % 8 == 0), (k % 8 == 4)
            mf[t] = np.block([[co * m0, -si * m0], [co * m4, -si * m4]])
        else:
            sg = (-1.0 if t in (1, 2) else 1.0) * np.where(k % 8 == t, 1.0, -1.0)
            mf[t] = np.block([[co, -si], [sg * si, sg * co]])
        ck = np.where(kf == 0, 1.0, 2.0) / (S * D)
        mi[t] = (mf[t] * np.concatenate([ck, ck])[None, :]).T
    m = np.arange(128)[:, None]
    s1 = np.arange(128)[None, :]
    gf = np.zeros((16, 256, 256))
    gi = np.zeros((16, 256, 256))
    for r in range(16):
        th = 2 * np.pi * ((s1 * (16 * m + r)) % S) / S
        gr, gim = np.cos(th), -np.sin(th)
        g = np.block([[gr, -gim], [gim, gr]])
        gf[r, :, 0::2], gf[r, :, 1::2] = g[:, :128], g[:, 128:]
        gi[r, :, 0::2], gi[r, :, 1::2] = g.T[:, :128], g.T[:, 128:]
    alt = (-1.0) ** np.arange(128)
    idx = np.arange(128)
    live = (idx[:, None] < 16) & (idx[None, :] < 16)
    th16 = 2 * np.pi * (idx[:, None] * idx[None, :] % 16) / 16
    small = np.stack([
        np.tile(alt[:, None], (1, 128)),
        np.tile(alt[None, :], (128, 1)) / (S * D),
        np.cos(th16) * live, -np.sin(th16) * live,
        (idx[:, None] % 16 == idx[None, :]) * 1.0,
    ])
    thw = 2 * np.pi * (idx[:, None] * idx[None, :] % S) / S
    tw = np.stack([np.cos(thw), -np.sin(thw)]).astype(np.float32)
    return (_pack_rows(mf), _pack_rows(mi), _pack_rows(small), tw,
            _pack_rows(gf), _pack_rows(gi))


def _bfly8(x):
    x0, x1, x2, x3, x4, x5, x6, x7 = x
    t0, t1, t2, t3 = x0 + x4, x0 - x4, x2 + x6, x2 - x6
    t4, t5, t6, t7 = x1 + x5, x1 - x5, x3 + x7, x3 - x7
    u0, u1, u2, u3 = t0 + t2, t0 - t2, t4 + t6, t4 - t6
    p, q = _SQH * (t5 - t7), _SQH * (t5 + t7)
    return [(u0 + u2, u0 - u2), (t1 + p, t3 + q), (u1, u3), (t1 - p, t3 - q)]


def _bfly8_t(planes):
    (a0, a4), (a1r, a1i), (u1, u3), (a3r, a3i) = planes
    u0, u2 = a0 + a4, a0 - a4
    t1, p, t3, q = a1r + a3r, a1r - a3r, a1i + a3i, a1i - a3i
    t5, t7 = _SQH * (p + q), _SQH * (q - p)
    t0, t2, t4, t6 = u0 + u1, u0 - u1, u2 + u3, u2 - u3
    return [t0 + t1, t4 + t5, t2 + t3, t6 + t7, t0 - t1, t4 - t5, t2 - t3, t6 - t7]


def _dft4(z):
    (ar, ai), (br, bi), (cr, ci), (dr, di) = z
    er, ei, fr, fi = ar + cr, ai + ci, ar - cr, ai - ci
    gr, gi, hr, hi = br + dr, bi + di, br - dr, bi - di
    return [(er + gr, ei + gi), (fr + hi, fi - hr), (er - gr, ei - gi), (fr - hi, fi + hr)]


def _twiddle16(z, e):
    re, im = z
    if e == 0:
        return z
    if e == 4:
        return im, -re
    if e == 2:
        return _SQH * (re + im), _SQH * (im - re)
    if e == 6:
        return _SQH * (im - re), -_SQH * (re + im)
    c, s = {1: (_C8, _S8), 3: (_S8, _C8), 9: (-_C8, -_S8)}[e]
    return re * c + im * s, im * c - re * s


def _dft16(z):
    cols = [_dft4([z[a + 4 * b] for b in range(4)]) for a in range(4)]
    out = [None] * 16
    for r1 in range(4):
        y = _dft4([_twiddle16(cols[a][r1], a * r1) for a in range(4)])
        for r2 in range(4):
            out[r1 + 4 * r2] = y[r2]
    return out


def _idft16(z):
    return [(re, im) for im, re in _dft16([(im, re) for re, im in z])]


def _bf(x):
    return pltpu.bitcast(x, BF16)


def _pack(re, im):
    return pltpu.pack_elementwise([re, im], packed_dtype=BF16)


def _low_halves(a, b):
    return (a & jnp.uint32(0xFFFF)) | (b << 16)


def _high_halves(a, b):
    return (a >> 16) | (b & jnp.uint32(0xFFFF0000))


def _dot(a, b):
    return jnp.dot(a, b, preferred_element_type=F32)


def _dot_nt(a, b):
    return lax.dot_general(a, b, (((1,), (1,)), ((), ())), preferred_element_type=F32)


def _softmax(sc):
    e = jnp.exp(sc - jnp.max(sc, axis=-1, keepdims=True))
    return e * (1.0 / jnp.sum(e, axis=-1, keepdims=True))


def _scope(name):
    return jax.named_scope(name)


def _kernel(ax_hbm, wr_hbm, wi_hbm, bx_hbm, mem0_hbm, wq_hbm, wk_hbm, wv_hbm, wo_hbm,
            mf_hbm, mi_hbm, ms_hbm, tw_hbm, gf_hbm, gi_hbm,
            out_hbm,
            xa, wraw, wnyq, wp, mf, mi, ms, tw, gf, gi, ybuf, ubuf, nyq,
            xs, xpre3, xpre, stage, wqkv, wo, pre, kvmem, obuf, opre,
            sem_xa, sem_c, sem_f, sem_g, sem_w, sem_wo, sem_out):
    copy = pltpu.make_async_copy
    w_hbm = (wq_hbm, wk_hbm, wv_hbm)
    f_hbm = (wr_hbm, wi_hbm)

    def xa_copy(c):
        return copy(ax_hbm.at[:, c], xa.at[c], sem_xa.at[c])

    mf_copy = copy(mf_hbm, mf, sem_c.at[0])
    ms_copy = copy(ms_hbm, ms, sem_c.at[1])
    xpre_copy = copy(bx_hbm.at[:, 0], xpre3, sem_c.at[2])
    tw_copy = copy(tw_hbm, tw, sem_c.at[3])
    mi_copy = copy(mi_hbm, mi, sem_c.at[4])
    xs_copy = copy(bx_hbm.at[:, pl.ds(1, 3)], xs.at[pl.ds(0, NSEG), pl.ds(1, 3)], sem_c.at[5])
    mem_copy = copy(mem0_hbm, xs.at[0, 0], sem_c.at[6])
    nyq_copies = [copy(f_hbm[i].at[pl.ds(D // 2, 1)], wnyq.at[i], sem_c.at[7 + i])
                  for i in range(2)]

    def f_copy(i, kap):
        src = f_hbm[i].at[pl.ds(0, D // 2)].bitcast(U32)
        return copy(src.at[:, pl.ds(pl.multiple_of(kap * 128, 128), 128)],
                    wraw.at[pl.ds(pl.multiple_of((kap * 2 + i) * 256, 256), 256)],
                    sem_f.at[kap * 2 + i])

    def g_copies(it):
        return [copy(src.at[pl.ds(4 * it, 4)], dst.at[pl.ds(4 * it, 4)], sem_g.at[2 * it + i])
                for i, (src, dst) in enumerate(((gf_hbm, gf), (gi_hbm, gi)))]

    def w_copy(mat, pair, slot):
        return copy(w_hbm[mat].bitcast(U32).at[:, pair, :],
                    stage.at[pl.ds(pl.multiple_of(slot * D, D), D)], sem_w.at[slot])

    def wo_copy(n):
        return copy(wo_hbm.bitcast(U32).at[:, pl.ds(pl.multiple_of(n * 128, 128), 128)],
                    wo.at[n], sem_wo.at[n])

    def y_copy(c):
        return copy(xa.at[c], out_hbm.at[:, c // 4, c % 4, :, pl.ds(0, D)], sem_out.at[0])

    def o_copy(s):
        return copy(xs.at[s, pl.ds(1, 3)],
                    out_hbm.at[s // 4, s % 4, pl.ds(1, 3), :, pl.ds(D, D)], sem_out.at[1])

    def opre_copy(b):
        return copy(xs.at[pl.ds(4 * b, 4), 0],
                    out_hbm.at[b, :, 0, :, pl.ds(D, D)], sem_out.at[2])

    mf_copy.start()
    ms_copy.start()
    pl.loop(0, 16)(lambda c: xa_copy(c).start())
    xpre_copy.start()
    pl.loop(0, NSLOT)(lambda slot: w_copy(0, slot, slot).start())

    lane = lax.broadcasted_iota(jnp.int32, (8, 128), 1)

    def a_forward(c):
        x = xa[c].astype(F32).reshape(128, D)
        planes = _bfly8([x[:, 128 * i:128 * (i + 1)] for i in range(8)])
        row = pl.ds(pl.multiple_of(c * 8, 8), 8)
        x1 = [_dot(jnp.concatenate(planes[t], axis=1).astype(BF16), _bf(mf[t]))
              for t in range(4)]
        bn = _dot(planes[0][0].astype(BF16), _bf(ms[0]))
        for t in range(4):
            y = _dft16([(x1[t][8 * b:8 * b + 8, :128], x1[t][8 * b:8 * b + 8, 128:])
                        for b in range(16)])
            for r in range(16):
                ybuf[r, row, 128 * t:128 * (t + 1)] = _pack(*y[r])
        acc = jnp.zeros((8, 128), F32)
        for b in range(16):
            acc = jnp.where(lane == b, bn[8 * b:8 * b + 8], acc)
        nyq[row, :] = acc

    def a_filter_layout(kap):
        base = kap * 512
        wr = [wraw[pl.ds(base + j, 64, stride=4), :] for j in range(4)]
        wi = [wraw[pl.ds(base + 256 + j, 64, stride=4), :] for j in range(4)]
        res = [(_low_halves, _high_halves)[k % 2](wr[k // 2], wi[k // 2]) for k in range(8)]
        for t, (lo, hi) in enumerate(((0, 4), (1, 7), (2, 6), (3, 5))):
            rows = pl.ds(pl.multiple_of(t * S + kap * 128, 128), 128)
            wp[rows, :] = jnp.concatenate([res[lo], res[hi]], axis=0).T

    def a_nyquist():
        b = nyq[...].astype(BF16)
        yr, yi = _dot(b, _bf(ms[2])), _dot(b, _bf(ms[3]))
        tc, ts = tw[0], tw[1]
        x2 = _dot(_bf(gf[0]), _bf(_pack(yr * tc - yi * ts, yr * ts + yi * tc)))
        sub = lax.broadcasted_iota(jnp.int32, (8, 128), 0)
        wn = []
        for i in range(2):
            w = wnyq[i].astype(F32)
            spread = jnp.concatenate(
                [jnp.where(lane // 16 == sub, w[:, 128 * k:128 * (k + 1)], 0.0)
                 for k in range(16)], axis=0)
            wn.append(_dot(spread.astype(BF16), _bf(ms[4])))
        a, b2 = x2[:128], x2[128:]
        u = _dot(_bf(gi[0]), _bf(_pack(a * wn[0] - b2 * wn[1], a * wn[1] + b2 * wn[0])))
        ur, ui = u[:128], u[128:]
        nyq[...] = (_dot((ur * tc + ui * ts).astype(BF16), _bf(ms[2]))
                    + _dot((ui * tc - ur * ts).astype(BF16), _bf(ms[3])))

    def a_filter(it, carry):
        z = {}

        def fwd(i):
            r = 4 * it + i
            x2 = _dot(_bf(gf[r]), _bf(ybuf[r]))
            parts = []
            for t in range(4):
                w = wp[pl.ds(t * S + r, 128, stride=16), :]
                wr = pltpu.bitcast(w << 16, F32)
                wi = pltpu.bitcast(w & jnp.uint32(0xFFFF0000), F32)
                a, b = x2[:128, 128 * t:128 * (t + 1)], x2[128:, 128 * t:128 * (t + 1)]
                parts.append(_pack(a * wr - b * wi, a * wi + b * wr))
            z[i] = jnp.concatenate(parts, axis=1)

        def inv(i):
            r = 4 * it + i
            ubuf[r] = _dot(_bf(gi[r]), _bf(z.pop(i)))

        fwd(0)
        for i in range(4):
            if i + 1 < 4:
                fwd(i + 1)
            inv(i)
        return carry

    def a_inverse(c):
        r0 = pl.multiple_of(c * 8, 8)
        planes = []
        for t in range(4):
            cols = slice(128 * t, 128 * (t + 1))
            x3 = _idft16([(ubuf[r, pl.ds(r0, 8), cols], ubuf[r, pl.ds(128 + r0, 8), cols])
                          for r in range(16)])
            lhs = jnp.concatenate([jnp.concatenate([v[p] for v in x3], axis=0)
                                   for p in range(2)], axis=1)
            o = _dot(lhs.astype(BF16), _bf(mi[t]))
            planes.append([o[:, :128], o[:, 128:]])
        bn = nyq[pl.ds(r0, 8), :]
        spread = jnp.concatenate([jnp.where(lane == b, bn, 0.0) for b in range(16)], axis=0)
        planes[0][0] = planes[0][0] + _dot(spread.astype(BF16), _bf(ms[1]))
        y = jnp.concatenate(_bfly8_t(planes), axis=1)
        xa[c] = y.reshape(16, 8, D).astype(BF16)

    mf_copy.wait()
    ms_copy.wait()

    def forward_loop(i, carry):
        for j in range(2):
            xa_copy(2 * i + j).wait()
        for j in range(2):
            a_forward(2 * i + j)
        return carry

    with _scope("A_fwd"):
        lax.fori_loop(0, 8, forward_loop, 0)

    xpre_copy.wait()
    xpre[...] = pltpu.bitcast(xpre3[...].reshape(NPRE, D), U32)

    def project_loop(mat):
        def body(it, carry):
            slot0 = ((4 * mat + it) % 3) * 4
            for i in range(4):
                w_copy(mat, 4 * it + i, slot0 + i).wait()
                if mat == 1:
                    f_copy(0, 4 * it + i).wait()
                    f_copy(1, 4 * it + i).wait()
            for i in range(4):
                base = (slot0 + i) * D
                ev = stage[pl.ds(base, D // 2, stride=2), :]
                od = stage[pl.ds(base + 1, D // 2, stride=2), :]
                lo, hi = _low_halves(ev, od), _high_halves(ev, od)
                head = 8 * it + 2 * i
                wqkv[3 * head + mat] = lo
                wqkv[3 * (head + 1) + mat] = hi
                p = _dot(_bf(xpre[...]), _bf(jnp.concatenate([lo, hi], axis=1))).astype(BF16)
                pre[mat, head] = p[:, :DH]
                pre[mat, head + 1] = p[:, DH:]
                if mat == 1:
                    a_filter_layout(4 * it + i)
                elif mat == 2:
                    a_inverse(4 * it + i)

            @pl.when(it < 1)
            def _():
                for i in range(4):
                    w_copy(mat, 4 * (it + 3) + i, slot0 + i).start()

            if mat < 2:
                @pl.when(it >= 1)
                def _():
                    for i in range(4):
                        w_copy(mat + 1, 4 * (it - 1) + i, slot0 + i).start()

            if mat == 0:
                for i in range(4):
                    f_copy(0, 4 * it + i).start()
                    f_copy(1, 4 * it + i).start()
                for cp in g_copies(it):
                    cp.start()
            elif mat == 1:
                wo_copy(2 * it).start()
                wo_copy(2 * it + 1).start()
            else:
                for i in range(4):
                    y_copy(4 * it + i).start()
            return carry

        with _scope("B_proj"):
            lax.fori_loop(0, 4, body, 0)

    project_loop(0)
    for cp in (tw_copy, *nyq_copies, mi_copy):
        cp.start()
    project_loop(1)
    xs_copy.start()
    mem_copy.start()
    with _scope("g_wait"):
        for it in range(4):
            for cp in g_copies(it):
                cp.wait()
        for cp in (tw_copy, *nyq_copies, mi_copy):
            cp.wait()
    with _scope("A_nyq"):
        a_nyquist()
    with _scope("A_filt"):
        lax.fori_loop(0, 4, a_filter, 0)
    project_loop(2)

    with _scope("wo_wait"):
        for n in range(8):
            wo_copy(n).wait()
        xs_copy.wait()
        mem_copy.wait()
    scale = DH ** -0.5

    def out_proj(lhs, h0, h1):
        return jnp.concatenate(
            [_dot(lhs, _bf(wo[n, h0 * 64:h1 * 64, :])) for n in range(8)], axis=1)

    def step(s, carry):
        row = lax.broadcasted_iota(jnp.int32, (32, 48), 0)
        col = lax.broadcasted_iota(jnp.int32, (32, 48), 1)
        allowed = ((row < NMEM) | (col >= 32) | (col <= row)) & (col < 40)
        p0 = pl.ds(pl.multiple_of(s * 8, 8), 8)
        h = xs[s].reshape(32, D)
        zeros = jnp.zeros((8, DH), BF16)
        st = {}

        def qkv(hd):
            q, k, v = [_dot(h, _bf(wqkv[3 * hd + i])).astype(BF16) for i in range(3)]
            kvmem[0, hd, p0, :] = k[:NMEM]
            kvmem[1, hd, p0, :] = v[:NMEM]
            st[hd] = (q, k, v)

        def scores(hd):
            q, k, v = st[hd]
            ka = jnp.concatenate([k, pre[1, hd, p0, :], zeros], axis=0)
            sc = jnp.where(allowed, _dot_nt(q, ka) * scale, -jnp.inf)
            st[hd] = (_softmax(sc).astype(BF16), v)

        def context(hd):
            p, v = st.pop(hd)
            va = jnp.concatenate([v, pre[2, hd, p0, :], zeros], axis=0)
            obuf[:, hd * DH:(hd + 1) * DH] = _dot(p, va).astype(BF16)

        acc = [None]

        def project(g):
            t = out_proj(obuf[:, 4 * g * DH:4 * (g + 1) * DH], 4 * g, 4 * (g + 1))
            acc[0] = t if acc[0] is None else acc[0] + t

        d1, d2, first = 1, 3, 26
        for hd in range(H):
            qkv(hd)
            if hd >= d1:
                scores(hd - d1)
            if hd >= d2:
                context(hd - d2)
            if hd >= first and (hd - first) % 4 == 0:
                project((hd - first) // 4)
        done = (H - 1 - first) // 4 + 1
        for t, g in enumerate(range(done, H // 4)):
            project(g)
            if H + t - d1 < H:
                scores(H + t - d1)
            if H + t - d2 < H:
                context(H + t - d2)
        ob = acc[0].astype(BF16).reshape(4, 8, D)
        xs[s, pl.ds(1, 3)] = ob[1:]
        xs[s + 1, 0] = ob[0]
        o_copy(s).start()
        return carry

    with _scope("B_step"):
        lax.fori_loop(0, NSEG, step, 0)

    def finish(g, carry):
        row = lax.broadcasted_iota(jnp.int32, (64, 128), 0)
        col = lax.broadcasted_iota(jnp.int32, (64, 128), 1)
        allowed = ((col % 64) // 8 == row // 8) & ((col < 64) | (col % 8 <= row % 8))
        st = {}

        def rows(a):
            return pl.ds(pl.multiple_of(g * 128 + a * 64, 64), 64)

        def scores(hd):
            for a in range(2):
                ka = jnp.concatenate([kvmem[0, hd, rows(a), :], pre[1, hd, rows(a), :]], axis=0)
                sc = jnp.where(allowed, _dot_nt(pre[0, hd, rows(a), :], ka) * scale, -jnp.inf)
                st[hd, a] = _softmax(sc).astype(BF16)

        def context(hd):
            for a in range(2):
                va = jnp.concatenate([kvmem[1, hd, rows(a), :], pre[2, hd, rows(a), :]], axis=0)
                opre[a * 64:(a + 1) * 64, hd * DH:(hd + 1) * DH] = (
                    _dot(st.pop((hd, a)), va).astype(BF16))

        acc = [None]

        def project(c):
            t = out_proj(opre[:, 4 * c * DH:4 * (c + 1) * DH], 4 * c, 4 * (c + 1))
            acc[0] = t if acc[0] is None else acc[0] + t

        for c in range(H // 4 + 2):
            if c < H // 4:
                for hd in range(4 * c, 4 * c + 4):
                    scores(hd)
            if 2 <= c:
                project(c - 2)
            if 1 <= c <= H // 4:
                for hd in range(4 * (c - 1), 4 * c):
                    context(hd)
        xs[pl.ds(g * 16, 16), 0] = acc[0].astype(BF16).reshape(16, 8, D)
        for i in range(4):
            opre_copy(g * 4 + i).start()
        return carry

    with _scope("B_fin"):
        lax.fori_loop(0, 4, finish, 0)

    with _scope("drain"):
        for c in range(16):
            y_copy(c).wait()

        def drain(s, carry):
            o_copy(s).wait()
            return carry

        lax.fori_loop(0, NSEG, drain, 0)
        for b in range(16):
            opre_copy(b).wait()


@functools.partial(jax.jit, static_argnames=("B_seg_len",))
def pallas_concat_heads__spectral_gfnet__memory_aug_recurrent_mem_tr__prompt_kernel(
    A_x, A_w_r, A_w_i, B_x, B_mem0, B_Wq, B_Wk, B_Wv, B_Wo, B_seg_len=SEG,
):
    assert A_x.shape == (1, S, D) and B_x.shape == (1, S, D)
    assert A_w_r.shape == A_w_i.shape == (S, D // 2 + 1)
    assert B_mem0.shape == (1, NMEM, D) and B_seg_len == SEG
    assert B_Wq.shape == B_Wk.shape == B_Wv.shape == (D, H, DH) and B_Wo.shape == (H, DH, D)

    vmem = pltpu.VMEM
    dma = pltpu.SemaphoreType.DMA
    scratch = [
        vmem((16, 16, 8, D), BF16),
        vmem((32 * 256, 128), U32),
        vmem((2, 1, S), BF16),
        vmem((4 * S, 128), U32),
        vmem((4, 128, 256), U32),
        vmem((4, 128, 256), U32),
        vmem((5, 64, 128), U32),
        vmem((2, 128, 128), F32),
        vmem((16, 128, 256), U32),
        vmem((16, 128, 256), U32),
        vmem((16, 128, 512), U32),
        vmem((16, 256, 512), F32),
        vmem((128, 128), F32),
        vmem((NSEG + 1, 4, 8, D), BF16),
        vmem((NSEG, 8, D), BF16),
        vmem((NPRE // 2, D), U32),
        vmem((NSLOT * D, 128), U32),
        vmem((3 * H, D // 2, DH), U32),
        vmem((8, H * DH // 2, 128), U32),
        vmem((3, H, NPRE, DH), BF16),
        vmem((2, H, NPRE, DH), BF16),
        vmem((32, H * DH), BF16),
        vmem((128, H * DH), BF16),
        dma((16,)), dma((9,)), dma((32,)), dma((8,)), dma((NSLOT,)), dma((8,)), dma((3,)),
    ]
    hbm = pl.BlockSpec(memory_space=pltpu.HBM)
    out = pl.pallas_call(
        _kernel,
        out_shape=jax.ShapeDtypeStruct((16, 4, 4, 8, 2 * D), BF16),
        in_specs=[hbm] * 15,
        out_specs=hbm,
        scratch_shapes=scratch,
        compiler_params=pltpu.CompilerParams(vmem_limit_bytes=124 * 1024 * 1024),
    )(A_x.reshape(16, 16, 8, D), A_w_r.T, A_w_i.T,
      B_x.reshape(NSEG, 4, 8, D), B_mem0.reshape(NMEM, D),
      B_Wq, B_Wk, B_Wv, B_Wo.reshape(H * DH, D),
      *[jnp.asarray(c) for c in _fft_constants()])
    return out.reshape(1, S, 2 * D)
```

```python
import functools

import numpy as np
import jax
import jax.numpy as jnp
from jax import lax
import jax.experimental.pallas as pl
import jax.experimental.pallas.tpu as pltpu

S, D = 2048, 1024
H, DH = 32, 128
NMEM, SEG = 8, 32
NSEG = S // SEG
NPRE = NSEG * 8
UNROLL = 2
WP_ROWS = 33 * 64
NSLOT = 12

F32, BF16, U32 = jnp.float32, jnp.bfloat16, jnp.uint32
_SQH = float(np.sqrt(0.5))


def _pack_rows(m):
    b = np.asarray(m, np.float32).astype(jnp.bfloat16).view(np.uint16).astype(np.uint32)
    return b[..., 0::2, :] | (b[..., 1::2, :] << 16)


@functools.lru_cache(maxsize=None)
def _fft_constants():
    d1 = np.arange(128)[:, None]
    mf = np.zeros((4, 256, 256))
    mi = np.zeros((4, 256, 256))
    for t, res in enumerate(((0, 4), (1, 7), (2, 6), (3, 5))):
        kf = 8 * (np.arange(128) % 64) + np.repeat(res, 64)
        k = kf[None, :]
        th = 2 * np.pi * ((d1 * k) % D) / D
        co, si = np.cos(th), np.sin(th)
        if t == 0:
            m0, m4 = (k % 8 == 0), (k % 8 == 4)
            mf[t] = np.block([[co * m0, -si * m0], [co * m4, -si * m4]])
        else:
            sg = (-1.0 if t in (1, 2) else 1.0) * np.where(k % 8 == t, 1.0, -1.0)
            mf[t] = np.block([[co, -si], [sg * si, sg * co]])
        ck = np.where(kf == 0, 1.0, 2.0) / (S * D)
        mi[t] = (mf[t] * np.concatenate([ck, ck])[None, :]).T
    m = np.arange(64)[:, None]
    s1 = np.arange(64)[None, :]
    gf = np.zeros((32, 128, 128))
    gi = np.zeros((32, 128, 128))
    for r in range(32):
        th = 2 * np.pi * ((s1 * (32 * m + r)) % S) / S
        gr, gim = np.cos(th), -np.sin(th)
        g = np.block([[gr, -gim], [gim, gr]])
        gf[r, :, 0::2], gf[r, :, 1::2] = g[:, :64], g[:, 64:]
        gi[r, :, 0::2], gi[r, :, 1::2] = g.T[:, :64], g.T[:, 64:]
    alt = (-1.0) ** np.arange(128)
    idx = np.arange(128)
    lane, r = idx[:, None], idx[None, :]
    live = (lane < 32) & (r < 32) & (lane // 16 == r % 2)
    th32 = 2 * np.pi * ((lane % 16) * r % 32) / 32
    fc, fs = np.cos(th32) * live, -np.sin(th32) * live
    small = np.stack([
        np.tile(alt[:, None], (1, 128)),
        np.tile(alt[None, :], (128, 1)) / (S * D),
        fc, fs, fc.T, fs.T,
        (lane % 32 == r) * 1.0,
    ])
    thw = 2 * np.pi * (idx[:64, None] * idx[None, :] % S) / S
    tw = np.stack([np.cos(thw), -np.sin(thw)]).astype(np.float32)
    return (_pack_rows(mf), _pack_rows(mi), _pack_rows(small), tw,
            _pack_rows(gf), _pack_rows(gi))


def _bfly8(x):
    x0, x1, x2, x3, x4, x5, x6, x7 = x
    t0, t1, t2, t3 = x0 + x4, x0 - x4, x2 + x6, x2 - x6
    t4, t5, t6, t7 = x1 + x5, x1 - x5, x3 + x7, x3 - x7
    u0, u1, u2, u3 = t0 + t2, t0 - t2, t4 + t6, t4 - t6
    p, q = _SQH * (t5 - t7), _SQH * (t5 + t7)
    return [(u0 + u2, u0 - u2), (t1 + p, t3 + q), (u1, u3), (t1 - p, t3 - q)]


def _bfly8_t(planes):
    (a0, a4), (a1r, a1i), (u1, u3), (a3r, a3i) = planes
    u0, u2 = a0 + a4, a0 - a4
    t1, p, t3, q = a1r + a3r, a1r - a3r, a1i + a3i, a1i - a3i
    t5, t7 = _SQH * (p + q), _SQH * (q - p)
    t0, t2, t4, t6 = u0 + u1, u0 - u1, u2 + u3, u2 - u3
    return [t0 + t1, t4 + t5, t2 + t3, t6 + t7, t0 - t1, t4 - t5, t2 - t3, t6 - t7]


def _dft4(z):
    (ar, ai), (br, bi), (cr, ci), (dr, di) = z
    er, ei, fr, fi = ar + cr, ai + ci, ar - cr, ai - ci
    gr, gi, hr, hi = br + dr, bi + di, br - dr, bi - di
    return [(er + gr, ei + gi), (fr + hi, fi - hr), (er - gr, ei - gi), (fr - hi, fi + hr)]


def _twiddle(z, e):
    re, im = z
    if e == 0:
        return z
    if e == 8:
        return im, -re
    if e == 4:
        return _SQH * (re + im), _SQH * (im - re)
    if e == 12:
        return _SQH * (im - re), -_SQH * (re + im)
    c, s = float(np.cos(np.pi * e / 16)), float(np.sin(np.pi * e / 16))
    return re * c + im * s, im * c - re * s


def _dft16(z):
    cols = [_dft4([z[a + 4 * b] for b in range(4)]) for a in range(4)]
    out = [None] * 16
    for r1 in range(4):
        y = _dft4([_twiddle(cols[a][r1], 2 * a * r1) for a in range(4)])
        for r2 in range(4):
            out[r1 + 4 * r2] = y[r2]
    return out


def _swap(z):
    return [(im, re) for re, im in z]


def _half_dft32(z, odd):
    return _dft16([_twiddle(v, b * odd) for b, v in enumerate(z)])


def _half_idft32(z, odd):
    return _swap([_twiddle(v, b * odd) for b, v in enumerate(_dft16(_swap(z)))])


def _bf(x):
    return pltpu.bitcast(x, BF16)


def _pack(re, im):
    return pltpu.pack_elementwise([re, im], packed_dtype=BF16)


def _low_halves(a, b):
    return (a & jnp.uint32(0xFFFF)) | (b << 16)


def _high_halves(a, b):
    return (a >> 16) | (b & jnp.uint32(0xFFFF0000))


def _dot(a, b):
    return jnp.dot(a, b, preferred_element_type=F32)


def _dot_nt(a, b):
    return lax.dot_general(a, b, (((1,), (1,)), ((), ())), preferred_element_type=F32)


def _softmax(sc):
    e = jnp.exp(sc - jnp.max(sc, axis=-1, keepdims=True))
    return e * (1.0 / jnp.sum(e, axis=-1, keepdims=True))


def _scope(name):
    return jax.named_scope(name)


def _kernel(ax_hbm, wr_hbm, wi_hbm, bx_hbm, mem0_hbm, wq_hbm, wk_hbm, wv_hbm, wo_hbm,
            mf_hbm, mi_hbm, ms_hbm, tw_hbm, gf_hbm, gi_hbm,
            out_hbm,
            xa, wraw, wnyq, wp, mf, mi, ms, tw, gf, gi, ybuf, ubuf, nyq,
            xs, xpre3, xpre, stage, wqkv, wo, pre, kvmem, obuf, opre, part,
            sem_xa, sem_c, sem_f, sem_g, sem_w, sem_wo, sem_out):
    copy = pltpu.make_async_copy
    w_hbm = (wq_hbm, wk_hbm, wv_hbm)
    f_hbm = (wr_hbm, wi_hbm)

    def xa_copy(c):
        return copy(ax_hbm.at[:, c], xa.at[c], sem_xa.at[c])

    mf_copy = copy(mf_hbm, mf, sem_c.at[0])
    ms_copy = copy(ms_hbm, ms, sem_c.at[1])
    xpre_copy = copy(bx_hbm.at[:, :, 0], xpre3, sem_c.at[2])
    tw_copy = copy(tw_hbm, tw, sem_c.at[3])
    mi_copy = copy(mi_hbm, mi, sem_c.at[4])
    xs_copy = copy(bx_hbm.at[:, :, pl.ds(1, 3)], xs.at[pl.ds(0, 32), :, pl.ds(1, 3)], sem_c.at[5])
    mem_copy = copy(mem0_hbm, xs.at[0, 0, 0], sem_c.at[6])
    nyq_copies = [copy(f_hbm[i].at[pl.ds(D // 2, 1)], wnyq.at[i], sem_c.at[7 + i])
                  for i in range(2)]

    def f_copy(i, kap):
        src = f_hbm[i].at[pl.ds(0, D // 2)].bitcast(U32)
        return copy(src.at[:, pl.ds(pl.multiple_of(kap * 128, 128), 128)],
                    wraw.at[pl.ds(pl.multiple_of((kap * 2 + i) * 256, 256), 256)],
                    sem_f.at[kap * 2 + i])

    def g_copies(it):
        return [copy(src.at[pl.ds(8 * it, 8)], dst.at[pl.ds(8 * it, 8)], sem_g.at[2 * it + i])
                for i, (src, dst) in enumerate(((gf_hbm, gf), (gi_hbm, gi)))]

    def w_copy(mat, pair, slot):
        return copy(w_hbm[mat].bitcast(U32).at[:, pair, :],
                    stage.at[pl.ds(pl.multiple_of(slot * D, D), D)], sem_w.at[slot])

    def wo_copy(n):
        return copy(wo_hbm.bitcast(U32).at[:, pl.ds(pl.multiple_of(n * 128, 128), 128)],
                    wo.at[n], sem_wo.at[n])

    def y_copy(c):
        return copy(xa.at[c], out_hbm.at[:, c // 4, c % 4, :, pl.ds(0, D)], sem_out.at[0])

    def o_copy(i):
        rows = pl.ds((UNROLL // 2) * i, UNROLL // 2)
        return copy(xs.at[rows, :, pl.ds(1, 3)],
                    out_hbm.at[rows, :, pl.ds(1, 3), :, pl.ds(D, D)], sem_out.at[1])

    def opre_copy(g):
        return copy(xs.at[pl.ds(8 * g, 8), :, 0],
                    out_hbm.at[pl.ds(8 * g, 8), :, 0, :, pl.ds(D, D)], sem_out.at[2])

    mf_copy.start()
    ms_copy.start()
    pl.loop(0, 8)(lambda c: xa_copy(c).start())
    xpre_copy.start()
    pl.loop(0, NSLOT)(lambda slot: w_copy(0, slot, slot).start())

    lane = lax.broadcasted_iota(jnp.int32, (8, 128), 1)

    def a_forward(c):
        x = xa[c].astype(F32).reshape(256, D)
        row = pl.ds(pl.multiple_of(c * 8, 8), 8)
        acc = jnp.zeros((8, 128), F32)
        for odd in range(2):
            xh = x[:128] - x[128:] if odd else x[:128] + x[128:]
            planes = _bfly8([xh[:, 128 * i:128 * (i + 1)] for i in range(8)])
            x1 = [_dot(jnp.concatenate(planes[t], axis=1).astype(BF16), _bf(mf[t]))
                  for t in range(4)]
            bn = _dot(planes[0][0].astype(BF16), _bf(ms[0]))
            for t in range(4):
                y = _half_dft32([(x1[t][8 * b:8 * b + 8, :128], x1[t][8 * b:8 * b + 8, 128:])
                                 for b in range(16)], odd)
                for r in range(16):
                    ybuf[2 * r + odd, row, 128 * t:128 * (t + 1)] = _pack(*y[r])
            for b in range(16):
                acc = jnp.where(lane == 16 * odd + b, bn[8 * b:8 * b + 8], acc)
        nyq[row, :] = acc

    def a_filter_layout(it, i):
        base = (4 * it + i) * 512
        wr = [wraw[pl.ds(base + j, 64, stride=4), :] for j in range(4)]
        wi = [wraw[pl.ds(base + 256 + j, 64, stride=4), :] for j in range(4)]
        res = [(_low_halves, _high_halves)[k % 2](wr[k // 2], wi[k // 2]) for k in range(8)]
        for t, (lo, hi) in enumerate(((0, 4), (1, 7), (2, 6), (3, 5))):
            tile = jnp.concatenate([res[lo], res[hi]], axis=0).T
            dst = wp.at[pl.ds(pl.multiple_of(t * WP_ROWS + it * 528, 8), 528)]
            for mm in range(4):
                dst[pl.ds(33 * (4 * i + mm), 32), :] = tile[32 * mm:32 * (mm + 1)]

    def a_nyquist():
        b = nyq[...].astype(BF16)
        yr, yi = _dot(b, _bf(ms[2])), _dot(b, _bf(ms[3]))
        tc, ts = tw[0], tw[1]
        x2 = _dot(_bf(gf[0]), _bf(_pack(yr * tc - yi * ts, yr * ts + yi * tc)))
        sub = lax.broadcasted_iota(jnp.int32, (8, 128), 0)
        wn = []
        for i in range(2):
            w = wnyq[i].astype(F32)
            spread = jnp.concatenate(
                [jnp.where(lane // 32 == sub % 4,
                           jnp.where(sub < 4, w[:, 256 * k:256 * k + 128],
                                     w[:, 256 * k + 128:256 * k + 256]), 0.0)
                 for k in range(8)], axis=0)
            wn.append(_dot(spread.astype(BF16), _bf(ms[6])))
        a, b2 = x2[:64], x2[64:]
        u = _dot(_bf(gi[0]), _bf(_pack(a * wn[0] - b2 * wn[1], a * wn[1] + b2 * wn[0])))
        ur, ui = u[:64], u[64:]
        nyq[...] = (_dot((ur * tc + ui * ts).astype(BF16), _bf(ms[4]))
                    + _dot((ui * tc - ur * ts).astype(BF16), _bf(ms[5])))

    def a_filter(it, carry):
        z = {}

        def fwd(i):
            r = 8 * it + i
            x2 = _dot(_bf(gf[r]), _bf(ybuf[r]))
            parts = []
            for t in range(4):
                w = wp[pl.ds(t * WP_ROWS + r, 64, stride=33), :]
                wr = pltpu.bitcast(w << 16, F32)
                wi = pltpu.bitcast(w & jnp.uint32(0xFFFF0000), F32)
                a, b = x2[:64, 128 * t:128 * (t + 1)], x2[64:, 128 * t:128 * (t + 1)]
                parts.append(_pack(a * wr - b * wi, a * wi + b * wr))
            z[i] = jnp.concatenate(parts, axis=1)

        def inv(i):
            r = 8 * it + i
            ubuf[r] = _dot(_bf(gi[r]), _bf(z.pop(i)))

        lag = 2
        for i in range(8 + lag):
            if i < 8:
                fwd(i)
            if i >= lag:
                inv(i - lag)
        return carry

    def a_inverse(c):
        r0 = pl.multiple_of(c * 8, 8)
        bn = nyq[pl.ds(r0, 8), :]
        halves = []
        for odd in range(2):
            planes = []
            for t in range(4):
                cols = slice(128 * t, 128 * (t + 1))
                x3 = _half_idft32(
                    [(ubuf[2 * r + odd, pl.ds(r0, 8), cols],
                      ubuf[2 * r + odd, pl.ds(64 + r0, 8), cols]) for r in range(16)], odd)
                lhs = jnp.concatenate([jnp.concatenate([v[p] for v in x3], axis=0)
                                       for p in range(2)], axis=1)
                o = _dot(lhs.astype(BF16), _bf(mi[t]))
                planes.append([o[:, :128], o[:, 128:]])
            spread = jnp.concatenate(
                [jnp.where(lane == 16 * odd + b, bn, 0.0) for b in range(16)], axis=0)
            planes[0][0] = planes[0][0] + _dot(spread.astype(BF16), _bf(ms[1]))
            halves.append(jnp.concatenate(_bfly8_t(planes), axis=1))
        y = jnp.concatenate([halves[0] + halves[1], halves[0] - halves[1]], axis=0)
        xa[c] = y.reshape(32, 8, D).astype(BF16)

    mf_copy.wait()
    ms_copy.wait()

    def forward_loop(c, carry):
        xa_copy(c).wait()
        a_forward(c)
        return carry

    with _scope("A_fwd"):
        lax.fori_loop(0, 8, forward_loop, 0)

    xpre_copy.wait()
    xpre[...] = pltpu.bitcast(xpre3[...].reshape(NPRE, D), U32)

    def project_loop(mat):
        def body(it, carry):
            slot0 = ((4 * mat + it) % 3) * 4
            for i in range(4):
                w_copy(mat, 4 * it + i, slot0 + i).wait()
                if mat == 1:
                    f_copy(0, 4 * it + i).wait()
                    f_copy(1, 4 * it + i).wait()
            for i in range(4):
                base = (slot0 + i) * D
                ev = stage[pl.ds(base, D // 2, stride=2), :]
                od = stage[pl.ds(base + 1, D // 2, stride=2), :]
                lo, hi = _low_halves(ev, od), _high_halves(ev, od)
                head = 8 * it + 2 * i
                wqkv[3 * head + mat] = lo
                wqkv[3 * (head + 1) + mat] = hi
                p = _dot(_bf(xpre[...]), _bf(jnp.concatenate([lo, hi], axis=1))).astype(BF16)
                pre[mat, head] = p[:, :DH]
                pre[mat, head + 1] = p[:, DH:]
                if mat == 1:
                    a_filter_layout(it, i)
                elif mat == 2 and i % 2 == 0:
                    a_inverse(2 * it + i // 2)

            @pl.when(it < 1)
            def _():
                for i in range(4):
                    w_copy(mat, 4 * (it + 3) + i, slot0 + i).start()

            if mat < 2:
                @pl.when(it >= 1)
                def _():
                    for i in range(4):
                        w_copy(mat + 1, 4 * (it - 1) + i, slot0 + i).start()

            if mat == 0:
                for i in range(4):
                    f_copy(0, 4 * it + i).start()
                    f_copy(1, 4 * it + i).start()
                for cp in g_copies(it):
                    cp.start()
            elif mat == 1:
                wo_copy(2 * it).start()
                wo_copy(2 * it + 1).start()
            else:
                for i in range(2):
                    y_copy(2 * it + i).start()
            return carry

        with _scope("B_proj"):
            lax.fori_loop(0, 4, body, 0)

    project_loop(0)
    for cp in (tw_copy, *nyq_copies, mi_copy):
        cp.start()
    project_loop(1)
    xs_copy.start()
    mem_copy.start()
    with _scope("g_wait"):
        for it in range(4):
            for cp in g_copies(it):
                cp.wait()
        for cp in (tw_copy, *nyq_copies, mi_copy):
            cp.wait()
    with _scope("A_nyq"):
        a_nyquist()
    with _scope("A_filt"):
        lax.fori_loop(0, 4, a_filter, 0)
    project_loop(2)

    with _scope("wo_wait"):
        for n in range(8):
            wo_copy(n).wait()
        xs_copy.wait()
        mem_copy.wait()
    scale = DH ** -0.5

    def out_proj(lhs, h0, h1):
        return jnp.concatenate(
            [_dot(lhs, _bf(wo[n, h0 * 64:h1 * 64, :])) for n in range(8)], axis=1)

    def segment(s, h, split):
        row = lax.broadcasted_iota(jnp.int32, (32, 48), 0)
        col = lax.broadcasted_iota(jnp.int32, (32, 48), 1)
        allowed = ((row < NMEM) | (col >= 32) | (col <= row)) & (col < 40)
        p0 = pl.ds(pl.multiple_of(s * 8, 8), 8)
        zeros = jnp.zeros((8, DH), BF16)
        st = {}

        def half(i, a):
            return _dot(h[:, 512 * a:512 * (a + 1)], _bf(wqkv[i, 256 * a:256 * (a + 1), :]))

        def qkv(hd):
            if hd == 0 and split:
                for i in range(3):
                    part[i] = half(i, 0)
                q, k, v = [(part[i] + half(i, 1)).astype(BF16) for i in range(3)]
            else:
                q, k, v = [_dot(h, _bf(wqkv[3 * hd + i])).astype(BF16) for i in range(3)]
            kvmem[0, hd, p0, :] = k[:NMEM]
            kvmem[1, hd, p0, :] = v[:NMEM]
            st[hd] = (q, k, v)

        def scores(hd):
            q, k, v = st[hd]
            ka = jnp.concatenate([k, pre[1, hd, p0, :], zeros], axis=0)
            sc = jnp.where(allowed, _dot_nt(q, ka) * scale, -jnp.inf)
            st[hd] = (_softmax(sc).astype(BF16), v)

        def context(hd):
            p, v = st.pop(hd)
            va = jnp.concatenate([v, pre[2, hd, p0, :], zeros], axis=0)
            obuf[:, hd * DH:(hd + 1) * DH] = _dot(p, va).astype(BF16)

        acc = [None] * 8

        def project(g):
            lhs = obuf[:, 4 * g * DH:4 * (g + 1) * DH]
            for n in range(8):
                t = _dot(lhs, _bf(wo[n, 256 * g:256 * (g + 1), :]))
                acc[n] = t if acc[n] is None else acc[n] + t

        d1, d2, first = 1, 3, 28
        for hd in range(H):
            qkv(hd)
            if hd >= d1:
                scores(hd - d1)
            if hd >= d2:
                context(hd - d2)
            if hd == first:
                project(0)
        for t, g in enumerate(range(1, H // 4)):
            project(g)
            if t < d1:
                scores(H + t - d1)
            if t < d2:
                context(H + t - d2)
        return acc

    def steps(i, carry):
        h = xs[(UNROLL // 2) * i, 0].reshape(32, D)
        for u in range(UNROLL):
            acc = segment(UNROLL * i + u, h, u > 0)
            nxt = ((UNROLL // 2) * i + (u + 1) // 2, (u + 1) % 2)
            if u + 1 < UNROLL:
                xt = xs[nxt[0], nxt[1], pl.ds(1, 3)].astype(F32).reshape(24, D)
                h = jnp.concatenate(
                    [jnp.concatenate([acc[n][:NMEM], xt[:, 128 * n:128 * (n + 1)]],
                                     axis=0).astype(BF16) for n in range(8)], axis=1)
            ob = jnp.concatenate(acc, axis=1).astype(BF16).reshape(4, 8, D)
            xs[(UNROLL // 2) * i + u // 2, u % 2, pl.ds(1, 3)] = ob[1:]
            if u + 1 == UNROLL:
                xs[nxt[0], nxt[1], 0] = ob[0]
        o_copy(i).start()
        return carry

    with _scope("B_step"):
        lax.fori_loop(0, NSEG // UNROLL, steps, 0)

    def finish(g, carry):
        row = lax.broadcasted_iota(jnp.int32, (64, 128), 0)
        col = lax.broadcasted_iota(jnp.int32, (64, 128), 1)
        allowed = ((col % 64) // 8 == row // 8) & ((col < 64) | (col % 8 <= row % 8))
        st = {}

        def rows(a):
            return pl.ds(pl.multiple_of(g * 128 + a * 64, 64), 64)

        def scores(hd):
            for a in range(2):
                ka = jnp.concatenate([kvmem[0, hd, rows(a), :], pre[1, hd, rows(a), :]], axis=0)
                sc = jnp.where(allowed, _dot_nt(pre[0, hd, rows(a), :], ka) * scale, -jnp.inf)
                st[hd, a] = _softmax(sc).astype(BF16)

        def context(hd):
            for a in range(2):
                va = jnp.concatenate([kvmem[1, hd, rows(a), :], pre[2, hd, rows(a), :]], axis=0)
                opre[a * 64:(a + 1) * 64, hd * DH:(hd + 1) * DH] = (
                    _dot(st.pop((hd, a)), va).astype(BF16))

        acc = [None]

        def project(c):
            t = out_proj(opre[:, 4 * c * DH:4 * (c + 1) * DH], 4 * c, 4 * (c + 1))
            acc[0] = t if acc[0] is None else acc[0] + t

        for c in range(H // 4 + 2):
            if c < H // 4:
                for hd in range(4 * c, 4 * c + 4):
                    scores(hd)
            if 2 <= c:
                project(c - 2)
            if 1 <= c <= H // 4:
                for hd in range(4 * (c - 1), 4 * c):
                    context(hd)
        xs[pl.ds(g * 8, 8), :, 0] = acc[0].astype(BF16).reshape(8, 2, 8, D)
        opre_copy(g).start()
        return carry

    with _scope("B_fin"):
        lax.fori_loop(0, 4, finish, 0)

    with _scope("drain"):
        for c in range(8):
            y_copy(c).wait()
        for i in range(NSEG // UNROLL):
            o_copy(i).wait()
        for g in range(4):
            opre_copy(g).wait()


@functools.partial(jax.jit, static_argnames=("B_seg_len",))
def pallas_concat_heads__spectral_gfnet__memory_aug_recurrent_mem_tr__prompt_kernel(
    A_x, A_w_r, A_w_i, B_x, B_mem0, B_Wq, B_Wk, B_Wv, B_Wo, B_seg_len=SEG,
):
    assert A_x.shape == (1, S, D) and B_x.shape == (1, S, D)
    assert A_w_r.shape == A_w_i.shape == (S, D // 2 + 1)
    assert B_mem0.shape == (1, NMEM, D) and B_seg_len == SEG
    assert B_Wq.shape == B_Wk.shape == B_Wv.shape == (D, H, DH) and B_Wo.shape == (H, DH, D)

    vmem = pltpu.VMEM
    dma = pltpu.SemaphoreType.DMA
    scratch = [
        vmem((8, 32, 8, D), BF16),
        vmem((32 * 256, 128), U32),
        vmem((2, 1, S), BF16),
        vmem((4 * WP_ROWS, 128), U32),
        vmem((4, 128, 256), U32),
        vmem((4, 128, 256), U32),
        vmem((7, 64, 128), U32),
        vmem((2, 64, 128), F32),
        vmem((32, 64, 128), U32),
        vmem((32, 64, 128), U32),
        vmem((32, 64, 512), U32),
        vmem((32, 128, 512), F32),
        vmem((64, 128), F32),
        vmem((33, 2, 4, 8, D), BF16),
        vmem((32, 2, 8, D), BF16),
        vmem((NPRE // 2, D), U32),
        vmem((NSLOT * D, 128), U32),
        vmem((3 * H, D // 2, DH), U32),
        vmem((8, H * DH // 2, 128), U32),
        vmem((3, H, NPRE, DH), BF16),
        vmem((2, H, NPRE, DH), BF16),
        vmem((32, H * DH), BF16),
        vmem((128, H * DH), BF16),
        vmem((3, 32, DH), F32),
        dma((8,)), dma((9,)), dma((32,)), dma((8,)), dma((NSLOT,)), dma((8,)), dma((3,)),
    ]
    hbm = pl.BlockSpec(memory_space=pltpu.HBM)
    out = pl.pallas_call(
        _kernel,
        out_shape=jax.ShapeDtypeStruct((32, 2, 4, 8, 2 * D), BF16),
        in_specs=[hbm] * 15,
        out_specs=hbm,
        scratch_shapes=scratch,
        compiler_params=pltpu.CompilerParams(vmem_limit_bytes=124 * 1024 * 1024),
    )(A_x.reshape(32, 8, 8, D), A_w_r.T, A_w_i.T,
      B_x.reshape(32, 2, 4, 8, D), B_mem0.reshape(NMEM, D),
      B_Wq, B_Wk, B_Wv, B_Wo.reshape(H * DH, D),
      *[jnp.asarray(c) for c in _fft_constants()])
    return out.reshape(1, S, 2 * D)
```

```python
import functools

import numpy as np
import jax
import jax.numpy as jnp
from jax import lax
import jax.experimental.pallas as pl
import jax.experimental.pallas.tpu as pltpu

S, D = 2048, 1024
H, DH = 32, 128
NMEM, SEG = 8, 32
NSEG = S // SEG
NPRE = NSEG * 8
UNROLL = 2
WP_ROWS = 33 * 64
NSLOT = 12

F32, BF16, U32 = jnp.float32, jnp.bfloat16, jnp.uint32
_SQH = float(np.sqrt(0.5))


def _pack_rows(m):
    b = np.asarray(m, np.float32).astype(jnp.bfloat16).view(np.uint16).astype(np.uint32)
    return b[..., 0::2, :] | (b[..., 1::2, :] << 16)


@functools.lru_cache(maxsize=None)
def _fft_constants():
    d1 = np.arange(128)[:, None]
    mf = np.zeros((4, 256, 256))
    mi = np.zeros((4, 256, 256))
    for t, res in enumerate(((0, 4), (1, 7), (2, 6), (3, 5))):
        kf = 8 * (np.arange(128) % 64) + np.repeat(res, 64)
        k = kf[None, :]
        th = 2 * np.pi * ((d1 * k) % D) / D
        co, si = np.cos(th), np.sin(th)
        sg = (-1.0 if t in (1, 2) else 1.0) * np.where(k % 8 == t, 1.0, -1.0)
        mf[t] = np.block([[co, -si], [sg * si, sg * co]])
        mi[t] = mf[t].T * (2.0 / (S * D))
        if t == 0:
            m0 = np.concatenate([co[:, :64], -si[:, :64]], axis=1)
            m0[:, 64] = (-1.0) ** np.arange(128)
            m4 = np.concatenate([-si[:, 64:], co[:, 64:]], axis=1)
            w0 = np.where(np.arange(128) % 64 == 0, 1.0, 2.0)
            mf[0], mi[0] = 0.0, 0.0
            mf[0, :128, :128], mf[0, :128, 128:] = m0, m4
            mi[0, :128, :128] = (m0 * w0).T / (S * D)
            mi[0, :128, 128:] = m4.T * (2.0 / (S * D))
    m = np.arange(64)[:, None]
    s1 = np.arange(64)[None, :]
    gf = np.zeros((32, 128, 128))
    gi = np.zeros((32, 128, 128))
    for r in range(32):
        th = 2 * np.pi * ((s1 * (32 * m + r)) % S) / S
        gr, gim = np.cos(th), -np.sin(th)
        g = np.block([[gr, -gim], [gim, gr]])
        gf[r, :, 0::2], gf[r, :, 1::2] = g[:, :64], g[:, 64:]
        gi[r, :, 0::2], gi[r, :, 1::2] = g.T[:, :64], g.T[:, 64:]
    idx = np.arange(128)
    lane, r = idx[:, None], idx[None, :]
    live = (lane < 32) & (r < 32) & (lane // 16 == r % 2)
    th32 = 2 * np.pi * ((lane % 16) * r % 32) / 32
    fc, fs = np.cos(th32) * live, -np.sin(th32) * live
    small = np.stack([fc, fs, fc.T, fs.T,
                      (lane % 32 == r) * 1.0])
    thw = 2 * np.pi * (idx[:64, None] * idx[None, :] % S) / S
    tw = np.stack([np.cos(thw), -np.sin(thw)]).astype(np.float32)
    return (_pack_rows(mf), _pack_rows(mi), _pack_rows(small), tw,
            _pack_rows(gf), _pack_rows(gi))


def _bfly8(x):
    x0, x1, x2, x3, x4, x5, x6, x7 = x
    t0, t1, t2, t3 = x0 + x4, x0 - x4, x2 + x6, x2 - x6
    t4, t5, t6, t7 = x1 + x5, x1 - x5, x3 + x7, x3 - x7
    u0, u1, u2, u3 = t0 + t2, t0 - t2, t4 + t6, t4 - t6
    p, q = _SQH * (t5 - t7), _SQH * (t5 + t7)
    return [(u0 + u2, u0 - u2), (t1 + p, t3 + q), (u1, u3), (t1 - p, t3 - q)]


def _bfly8_t(planes):
    (a0, a4), (a1r, a1i), (u1, u3), (a3r, a3i) = planes
    u0, u2 = a0 + a4, a0 - a4
    t1, p, t3, q = a1r + a3r, a1r - a3r, a1i + a3i, a1i - a3i
    t5, t7 = _SQH * (p + q), _SQH * (q - p)
    t0, t2, t4, t6 = u0 + u1, u0 - u1, u2 + u3, u2 - u3
    return [t0 + t1, t4 + t5, t2 + t3, t6 + t7, t0 - t1, t4 - t5, t2 - t3, t6 - t7]


def _dft4(z):
    (ar, ai), (br, bi), (cr, ci), (dr, di) = z
    er, ei, fr, fi = ar + cr, ai + ci, ar - cr, ai - ci
    gr, gi, hr, hi = br + dr, bi + di, br - dr, bi - di
    return [(er + gr, ei + gi), (fr + hi, fi - hr), (er - gr, ei - gi), (fr - hi, fi + hr)]


def _twiddle(z, e):
    re, im = z
    if e == 0:
        return z
    if e == 8:
        return im, -re
    if e == 4:
        return _SQH * (re + im), _SQH * (im - re)
    if e == 12:
        return _SQH * (im - re), -_SQH * (re + im)
    c, s = float(np.cos(np.pi * e / 16)), float(np.sin(np.pi * e / 16))
    return re * c + im * s, im * c - re * s


def _dft16(z):
    cols = [_dft4([z[a + 4 * b] for b in range(4)]) for a in range(4)]
    out = [None] * 16
    for r1 in range(4):
        y = _dft4([_twiddle(cols[a][r1], 2 * a * r1) for a in range(4)])
        for r2 in range(4):
            out[r1 + 4 * r2] = y[r2]
    return out


def _swap(z):
    return [(im, re) for re, im in z]


def _half_dft32(z, odd):
    return _dft16([_twiddle(v, b * odd) for b, v in enumerate(z)])


def _half_idft32(z, odd):
    return _swap([_twiddle(v, b * odd) for b, v in enumerate(_dft16(_swap(z)))])


def _bf(x):
    return pltpu.bitcast(x, BF16)


def _pack(re, im):
    return pltpu.pack_elementwise([re, im], packed_dtype=BF16)


def _low_halves(a, b):
    return (a & jnp.uint32(0xFFFF)) | (b << 16)


def _high_halves(a, b):
    return (a >> 16) | (b & jnp.uint32(0xFFFF0000))


def _dot(a, b):
    return jnp.dot(a, b, preferred_element_type=F32)


def _dot_nt(a, b):
    return lax.dot_general(a, b, (((1,), (1,)), ((), ())), preferred_element_type=F32)


def _softmax(sc):
    e = jnp.exp(sc - jnp.max(sc, axis=-1, keepdims=True))
    return e * (1.0 / jnp.sum(e, axis=-1, keepdims=True))


def _scope(name):
    return jax.named_scope(name)


def _kernel(ax_hbm, wr_hbm, wi_hbm, bx_hbm, mem0_hbm, wq_hbm, wk_hbm, wv_hbm, wo_hbm,
            mf_hbm, mi_hbm, ms_hbm, tw_hbm, gf_hbm, gi_hbm,
            out_hbm,
            xa, wraw, wnyq, wp, mf, mi, ms, tw, gf, gi, ybuf, ubuf, nyq,
            xs, xpre3, xpre, stage, wqkv, wo, pre, kvmem, obuf, opre, part,
            sem_xa, sem_c, sem_f, sem_g, sem_w, sem_wo, sem_out):
    copy = pltpu.make_async_copy
    w_hbm = (wq_hbm, wk_hbm, wv_hbm)
    f_hbm = (wr_hbm, wi_hbm)

    def xa_copy(c):
        return copy(ax_hbm.at[:, c], xa.at[c], sem_xa.at[c])

    mf_copy = copy(mf_hbm, mf, sem_c.at[0])
    ms_copy = copy(ms_hbm, ms, sem_c.at[1])
    xpre_copy = copy(bx_hbm.at[:, :, 0], xpre3, sem_c.at[2])
    tw_copy = copy(tw_hbm, tw, sem_c.at[3])
    mi_copy = copy(mi_hbm, mi, sem_c.at[4])
    xs_copy = copy(bx_hbm.at[:, :, pl.ds(1, 3)], xs.at[pl.ds(0, 32), :, pl.ds(1, 3)], sem_c.at[5])
    mem_copy = copy(mem0_hbm, xs.at[0, 0, 0], sem_c.at[6])
    nyq_copies = [copy(f_hbm[i].at[pl.ds(D // 2, 1)], wnyq.at[i], sem_c.at[7 + i])
                  for i in range(2)]

    def f_copy(i, kap):
        src = f_hbm[i].at[pl.ds(0, D // 2)].bitcast(U32)
        return copy(src.at[:, pl.ds(pl.multiple_of(kap * 128, 128), 128)],
                    wraw.at[pl.ds(pl.multiple_of((kap * 2 + i) * 256, 256), 256)],
                    sem_f.at[kap * 2 + i])

    gf_copy = copy(gf_hbm, gf, sem_g.at[0])
    gi_copy = copy(gi_hbm, gi, sem_g.at[1])

    def w_copy(mat, pair, slot):
        return copy(w_hbm[mat].bitcast(U32).at[:, pair, :],
                    stage.at[pl.ds(pl.multiple_of(slot * D, D), D)], sem_w.at[slot])

    def wo_copy(n):
        return copy(wo_hbm.bitcast(U32).at[:, pl.ds(pl.multiple_of(n * 128, 128), 128)],
                    wo.at[n], sem_wo.at[n])

    def y_copy(c):
        return copy(xa.at[c], out_hbm.at[:, c // 4, c % 4, :, pl.ds(0, D)], sem_out.at[0])

    def o_copy(i):
        rows = pl.ds((UNROLL // 2) * i, UNROLL // 2)
        return copy(xs.at[rows, :, pl.ds(1, 3)],
                    out_hbm.at[rows, :, pl.ds(1, 3), :, pl.ds(D, D)], sem_out.at[1])

    def opre_copy(g):
        return copy(xs.at[pl.ds(8 * g, 8), :, 0],
                    out_hbm.at[pl.ds(8 * g, 8), :, 0, :, pl.ds(D, D)], sem_out.at[2])

    xpre_copy.start()
    pl.loop(0, NSLOT)(lambda slot: w_copy(0, slot, slot).start())
    mf_copy.start()
    ms_copy.start()

    lane = lax.broadcasted_iota(jnp.int32, (8, 128), 1)
    lanes = lax.broadcasted_iota(jnp.int32, (128, 128), 1)

    def a_forward(c, odd):
        row = pl.ds(pl.multiple_of(c * 8, 8), 8)
        lhs = []
        for part_ in range(2):
            lo = xa[c, pl.ds(8 * part_, 8)].astype(F32).reshape(64, D)
            hi = xa[c, pl.ds(16 + 8 * part_, 8)].astype(F32).reshape(64, D)
            xh = lo - hi if odd else lo + hi
            planes = _bfly8([xh[:, 128 * i:128 * (i + 1)] for i in range(8)])
            lhs.append([jnp.concatenate(planes[t], axis=1).astype(BF16) for t in range(4)])
            yield
        lhs = [jnp.concatenate([lhs[0][t], lhs[1][t]], axis=0) for t in range(4)]
        x1 = {}

        def butterflies(t):
            v = x1.pop(t)
            y = _half_dft32([(v[8 * b:8 * b + 8, :128], v[8 * b:8 * b + 8, 128:])
                             for b in range(16)], odd)
            for r in range(16):
                ybuf[2 * r + odd, row, 128 * t:128 * (t + 1)] = _pack(*y[r])

        p0 = _dot(lhs[0][:, :128], _bf(mf[0, :64, :128]))
        p4 = _dot(lhs[0][:, 128:], _bf(mf[0, :64, 128:]))
        x1[1] = _dot(lhs[1], _bf(mf[1]))
        low = lanes < 64
        im = pltpu.roll(jnp.where(low, p4, p0), 64, 1)
        x1[0] = jnp.concatenate([jnp.where(low, p0, p4), jnp.where(lanes == 0, 0.0, im)], axis=1)
        acc = nyq[row, :] if odd else jnp.zeros((8, 128), F32)
        for b in range(16):
            k = 16 * odd + b
            v = im[8 * b:8 * b + 8]
            acc = jnp.where(lane == k, pltpu.roll(v, k, 1) if k else v, acc)
        nyq[row, :] = acc
        butterflies(0)
        yield
        x1[2] = _dot(lhs[2], _bf(mf[2]))
        x1[3] = _dot(lhs[3], _bf(mf[3]))
        butterflies(1)
        yield
        butterflies(2)
        yield
        butterflies(3)
        yield

    def a_filter_layout(it, i):
        base = (4 * it + i) * 512
        wr = [wraw[pl.ds(base + j, 64, stride=4), :] for j in range(4)]
        wi = [wraw[pl.ds(base + 256 + j, 64, stride=4), :] for j in range(4)]
        res = [(_low_halves, _high_halves)[k % 2](wr[k // 2], wi[k // 2]) for k in range(8)]
        for t, (lo, hi) in enumerate(((0, 4), (1, 7), (2, 6), (3, 5))):
            tile = jnp.concatenate([res[lo], res[hi]], axis=0).T
            dst = wp.at[pl.ds(pl.multiple_of(t * WP_ROWS + it * 528, 8), 528)]
            for mm in range(4):
                dst[pl.ds(33 * (4 * i + mm), 32), :] = tile[32 * mm:32 * (mm + 1)]

    def a_nyquist():
        b = nyq[...].astype(BF16)
        yr, yi = _dot(b, _bf(ms[0])), _dot(b, _bf(ms[1]))
        tc, ts = tw[0], tw[1]
        x2 = _dot(_bf(gf[0]), _bf(_pack(yr * tc - yi * ts, yr * ts + yi * tc)))
        sub = lax.broadcasted_iota(jnp.int32, (8, 128), 0)
        wn = []
        for i in range(2):
            w = wnyq[i].astype(F32)
            spread = jnp.concatenate(
                [jnp.where(lane // 32 == sub % 4,
                           jnp.where(sub < 4, w[:, 256 * k:256 * k + 128],
                                     w[:, 256 * k + 128:256 * k + 256]), 0.0)
                 for k in range(8)], axis=0)
            wn.append(_dot(spread.astype(BF16), _bf(ms[4])))
        a, b2 = x2[:64], x2[64:]
        u = _dot(_bf(gi[0]), _bf(_pack(a * wn[0] - b2 * wn[1], a * wn[1] + b2 * wn[0])))
        ur, ui = u[:64], u[64:]
        nyq[...] = (_dot((ur * tc + ui * ts).astype(BF16), _bf(ms[2]))
                    + _dot((ui * tc - ur * ts).astype(BF16), _bf(ms[3])))

    def a_filter(it, carry):
        z = {}

        def fwd(i):
            r = 8 * it + i
            x2 = _dot(_bf(gf[r]), _bf(ybuf[r]))
            parts = []
            for t in range(4):
                w = wp[pl.ds(t * WP_ROWS + r, 64, stride=33), :]
                wr = pltpu.bitcast(w << 16, F32)
                wi = pltpu.bitcast(w & jnp.uint32(0xFFFF0000), F32)
                a, b = x2[:64, 128 * t:128 * (t + 1)], x2[64:, 128 * t:128 * (t + 1)]
                parts.append(_pack(a * wr - b * wi, a * wi + b * wr))
            z[i] = jnp.concatenate(parts, axis=1)

        def inv(i):
            r = 8 * it + i
            ubuf[r] = _dot(_bf(gi[r]), _bf(z.pop(i)))

        lag = 2
        for i in range(8 + lag):
            if i < 8:
                fwd(i)
            if i >= lag:
                inv(i - lag)
        return carry

    def a_inverse(c, odd, halves):
        r0 = pl.multiple_of(c * 8, 8)
        planes = []

        def tile(t):
            cols = slice(128 * t, 128 * (t + 1))
            x3 = _half_idft32(
                [(ubuf[2 * r + odd, pl.ds(r0, 8), cols],
                  ubuf[2 * r + odd, pl.ds(64 + r0, 8), cols]) for r in range(16)], odd)
            re, im = [jnp.concatenate([v[p] for v in x3], axis=0) for p in range(2)]
            if t:
                o = _dot(jnp.concatenate([re, im], axis=1).astype(BF16), _bf(mi[t]))
                planes.append((o[:, :128], o[:, 128:]))
                return
            bn = nyq[pl.ds(r0, 8), :]
            bn = jnp.concatenate(
                [pltpu.roll(bn, 64 - 16 * odd - b, 1) for b in range(16)], axis=0)
            low = lanes < 64
            im = pltpu.roll(im, 64, 1)
            q0 = jnp.where(low, re, jnp.where(lanes == 64, bn, im))
            q4 = jnp.where(low, im, re)
            planes.append((_dot(q0.astype(BF16), _bf(mi[0, :64, :128])),
                           _dot(q4.astype(BF16), _bf(mi[0, :64, 128:]))))

        tile(0)
        yield
        tile(1)
        tile(2)
        yield
        tile(3)
        yield
        halves.append(jnp.concatenate(_bfly8_t(planes), axis=1))
        if odd:
            y = jnp.concatenate([halves[0] + halves[1], halves[0] - halves[1]], axis=0)
            xa[c] = y.reshape(32, 8, D).astype(BF16)
        yield

    xpre_copy.wait()
    xpre[...] = pltpu.bitcast(xpre3[...].reshape(NPRE, D), U32)

    def project_pair(mat, pair, slot, side):
        ev = stage[pl.ds(slot * D, D // 2, stride=2), :]
        od = stage[pl.ds(slot * D + 1, D // 2, stride=2), :]
        lo, hi = _low_halves(ev, od), _high_halves(ev, od)
        wqkv[6 * pair + mat] = lo
        wqkv[6 * pair + 3 + mat] = hi
        if side is None:
            p = _dot(_bf(xpre[...]), _bf(jnp.concatenate([lo, hi], axis=1))).astype(BF16)
            pre[mat, 2 * pair] = p[:, :DH]
            pre[mat, 2 * pair + 1] = p[:, DH:]
            return
        for j in range(4):
            next(side)
            if j:
                lo, hi = wqkv[6 * pair + mat], wqkv[6 * pair + 3 + mat]
            p = _dot(_bf(xpre[64 * j:64 * (j + 1), :]),
                     _bf(jnp.concatenate([lo, hi], axis=1))).astype(BF16)
            pre[mat, 2 * pair, 128 * j:128 * (j + 1), :] = p[:, :DH]
            pre[mat, 2 * pair + 1, 128 * j:128 * (j + 1), :] = p[:, DH:]

    def project_loop(name, mat, npair, before, side, after):
        def body(it, carry):
            first = npair * it
            slot0 = (16 * mat + first) % NSLOT
            for i in range(npair):
                w_copy(mat, first + i, slot0 + i).wait()
            before(it)
            work = side(it)
            for i in range(npair):
                project_pair(mat, first + i, slot0 + i, work)

            @pl.when(first + NSLOT < 16)
            def _():
                for i in range(npair):
                    w_copy(mat, first + NSLOT + i, slot0 + i).start()

            if mat < 2:
                @pl.when(first + NSLOT >= 16)
                def _():
                    for i in range(npair):
                        w_copy(mat + 1, first + NSLOT - 16 + i, slot0 + i).start()

            after(it)
            return carry

        with _scope(name):
            lax.fori_loop(0, 16 // npair, body, 0)

    def nothing(*_):
        pass

    def fetch_a_inputs(it):
        xa_copy(it).start()
        for kap in range(2):
            f_copy(0, 2 * it + kap).start()
            f_copy(1, 2 * it + kap).start()

    def wait_a_inputs(it):
        for c in range(2):
            xa_copy(2 * it + c).wait()
        for kap in range(4):
            f_copy(0, 4 * it + kap).wait()
            f_copy(1, 4 * it + kap).wait()

    def forward_fft(it):
        units = [a_forward(2 * it + u // 2, u % 2) for u in range(4)]
        for u in range(4):
            for stage_ in range(4):
                if u and stage_ < 2:
                    next(units[u - 1])
                next(units[u])
                if stage_ == 2:
                    a_filter_layout(it, u)
                if u == 3 and stage_ == 3:
                    next(units[u])
                    next(units[u])
                yield

    def fetch_late_inputs(it):
        wo_copy(2 * it).start()
        wo_copy(2 * it + 1).start()

    def inverse_fft(it):
        for c in range(2):
            halves = []
            for odd in range(2):
                yield from a_inverse(2 * it + c, odd, halves)

    def store_y(it):
        for c in range(2):
            y_copy(2 * it + c).start()

    project_loop("B_proj_q", 0, 2, nothing, nothing, fetch_a_inputs)
    for cp in (tw_copy, *nyq_copies, mi_copy, gf_copy, gi_copy):
        cp.start()
    mf_copy.wait()
    ms_copy.wait()
    project_loop("B_proj_k", 1, 4, wait_a_inputs, forward_fft, fetch_late_inputs)
    xs_copy.start()
    mem_copy.start()
    with _scope("g_wait"):
        for cp in (tw_copy, *nyq_copies, mi_copy, gf_copy, gi_copy):
            cp.wait()
    with _scope("A_nyq"):
        a_nyquist()
    with _scope("A_filt"):
        lax.fori_loop(0, 4, a_filter, 0)
    project_loop("B_proj_v", 2, 4, nothing, inverse_fft, store_y)

    with _scope("wo_wait"):
        for n in range(8):
            wo_copy(n).wait()
        xs_copy.wait()
        mem_copy.wait()
    scale = DH ** -0.5

    def out_proj(lhs, h0, h1):
        return jnp.concatenate(
            [_dot(lhs, _bf(wo[n, h0 * 64:h1 * 64, :])) for n in range(8)], axis=1)

    def segment(s, h, split):
        row = lax.broadcasted_iota(jnp.int32, (32, 48), 0)
        col = lax.broadcasted_iota(jnp.int32, (32, 48), 1)
        allowed = ((row < NMEM) | (col >= 32) | (col <= row)) & (col < 40)
        p0 = pl.ds(pl.multiple_of(s * 8, 8), 8)
        zeros = jnp.zeros((8, DH), BF16)
        st = {}

        def half(i, a):
            return _dot(h[:, 512 * a:512 * (a + 1)], _bf(wqkv[i, 256 * a:256 * (a + 1), :]))

        def qkv(hd):
            if hd == 0 and split:
                for i in range(3):
                    part[i] = half(i, 0)
                q, k, v = [(part[i] + half(i, 1)).astype(BF16) for i in range(3)]
            else:
                q, k, v = [_dot(h, _bf(wqkv[3 * hd + i])).astype(BF16) for i in range(3)]
            kvmem[0, hd, p0, :] = k[:NMEM]
            kvmem[1, hd, p0, :] = v[:NMEM]
            st[hd] = (q, k, v)

        def scores(hd):
            q, k, v = st[hd]
            ka = jnp.concatenate([k, pre[1, hd, p0, :], zeros], axis=0)
            sc = jnp.where(allowed, _dot_nt(q, ka) * scale, -jnp.inf)
            st[hd] = (_softmax(sc).astype(BF16), v)

        def context(hd):
            p, v = st.pop(hd)
            va = jnp.concatenate([v, pre[2, hd, p0, :], zeros], axis=0)
            obuf[:, hd * DH:(hd + 1) * DH] = _dot(p, va).astype(BF16)

        acc = [None] * 8

        def project(g):
            lhs = obuf[:, 4 * g * DH:4 * (g + 1) * DH]
            for n in range(8):
                t = _dot(lhs, _bf(wo[n, 256 * g:256 * (g + 1), :]))
                acc[n] = t if acc[n] is None else acc[n] + t

        d1, d2, first = 1, 3, 28
        for hd in range(H):
            qkv(hd)
            if hd >= d1:
                scores(hd - d1)
            if hd >= d2:
                context(hd - d2)
            if hd == first:
                project(0)
        for t, g in enumerate(range(1, H // 4)):
            project(g)
            if t < d1:
                scores(H + t - d1)
            if t < d2:
                context(H + t - d2)
        return acc

    def steps(i, carry):
        h = xs[(UNROLL // 2) * i, 0].reshape(32, D)
        for u in range(UNROLL):
            acc = segment(UNROLL * i + u, h, u > 0)
            nxt = ((UNROLL // 2) * i + (u + 1) // 2, (u + 1) % 2)
            if u + 1 < UNROLL:
                xt = xs[nxt[0], nxt[1], pl.ds(1, 3)].astype(F32).reshape(24, D)
                h = jnp.concatenate(
                    [jnp.concatenate([acc[n][:NMEM], xt[:, 128 * n:128 * (n + 1)]],
                                     axis=0).astype(BF16) for n in range(8)], axis=1)
            ob = jnp.concatenate(acc, axis=1).astype(BF16).reshape(4, 8, D)
            xs[(UNROLL // 2) * i + u // 2, u % 2, pl.ds(1, 3)] = ob[1:]
            if u + 1 == UNROLL:
                xs[nxt[0], nxt[1], 0] = ob[0]
        o_copy(i).start()
        return carry

    with _scope("B_step"):
        lax.fori_loop(0, NSEG // UNROLL, steps, 0)

    def finish(g, carry):
        row = lax.broadcasted_iota(jnp.int32, (64, 128), 0)
        col = lax.broadcasted_iota(jnp.int32, (64, 128), 1)
        allowed = ((col % 64) // 8 == row // 8) & ((col < 64) | (col % 8 <= row % 8))
        st = {}

        def rows(a):
            return pl.ds(pl.multiple_of(g * 128 + a * 64, 64), 64)

        def scores(hd):
            for a in range(2):
                ka = jnp.concatenate([kvmem[0, hd, rows(a), :], pre[1, hd, rows(a), :]], axis=0)
                sc = jnp.where(allowed, _dot_nt(pre[0, hd, rows(a), :], ka) * scale, -jnp.inf)
                st[hd, a] = _softmax(sc).astype(BF16)

        def context(hd):
            for a in range(2):
                va = jnp.concatenate([kvmem[1, hd, rows(a), :], pre[2, hd, rows(a), :]], axis=0)
                opre[a * 64:(a + 1) * 64, hd * DH:(hd + 1) * DH] = (
                    _dot(st.pop((hd, a)), va).astype(BF16))

        acc = [None]

        def project(c):
            t = out_proj(opre[:, 4 * c * DH:4 * (c + 1) * DH], 4 * c, 4 * (c + 1))
            acc[0] = t if acc[0] is None else acc[0] + t

        for c in range(H // 4 + 2):
            if c < H // 4:
                for hd in range(4 * c, 4 * c + 4):
                    scores(hd)
            if 2 <= c:
                project(c - 2)
            if 1 <= c <= H // 4:
                for hd in range(4 * (c - 1), 4 * c):
                    context(hd)
        xs[pl.ds(g * 8, 8), :, 0] = acc[0].astype(BF16).reshape(8, 2, 8, D)
        opre_copy(g).start()
        return carry

    with _scope("B_fin"):
        lax.fori_loop(0, 4, finish, 0)

    with _scope("drain"):
        for c in range(8):
            y_copy(c).wait()
        for i in range(NSEG // UNROLL):
            o_copy(i).wait()
        for g in range(4):
            opre_copy(g).wait()


@functools.partial(jax.jit, static_argnames=("B_seg_len",))
def pallas_concat_heads__spectral_gfnet__memory_aug_recurrent_mem_tr__prompt_kernel(
    A_x, A_w_r, A_w_i, B_x, B_mem0, B_Wq, B_Wk, B_Wv, B_Wo, B_seg_len=SEG,
):
    assert A_x.shape == (1, S, D) and B_x.shape == (1, S, D)
    assert A_w_r.shape == A_w_i.shape == (S, D // 2 + 1)
    assert B_mem0.shape == (1, NMEM, D) and B_seg_len == SEG
    assert B_Wq.shape == B_Wk.shape == B_Wv.shape == (D, H, DH) and B_Wo.shape == (H, DH, D)

    vmem = pltpu.VMEM
    dma = pltpu.SemaphoreType.DMA
    scratch = [
        vmem((8, 32, 8, D), BF16),
        vmem((32 * 256 + 32, 128), U32),
        vmem((2, 1, S), BF16),
        vmem((4 * WP_ROWS + 32, 128), U32),
        vmem((4, 128, 256), U32),
        vmem((4, 128, 256), U32),
        vmem((5, 64, 128), U32),
        vmem((2, 64, 128), F32),
        vmem((32, 64, 128), U32),
        vmem((32, 64, 128), U32),
        vmem((32, 64, 512), U32),
        vmem((32, 128, 512), F32),
        vmem((64, 128), F32),
        vmem((33, 2, 4, 8, D), BF16),
        vmem((32, 2, 8, D), BF16),
        vmem((NPRE // 2, D), U32),
        vmem((NSLOT * D + 32, 128), U32),
        vmem((3 * H, D // 2, DH), U32),
        vmem((8, H * DH // 2, 128), U32),
        vmem((3, H, NPRE, DH), BF16),
        vmem((2, H, NPRE, DH), BF16),
        vmem((32, H * DH), BF16),
        vmem((128, H * DH), BF16),
        vmem((3, 32, DH), F32),
        dma((8,)), dma((9,)), dma((32,)), dma((2,)), dma((NSLOT,)), dma((8,)), dma((3,)),
    ]
    hbm = pl.BlockSpec(memory_space=pltpu.HBM)
    out = pl.pallas_call(
        _kernel,
        out_shape=jax.ShapeDtypeStruct((32, 2, 4, 8, 2 * D), BF16),
        in_specs=[hbm] * 15,
        out_specs=hbm,
        scratch_shapes=scratch,
        compiler_params=pltpu.CompilerParams(vmem_limit_bytes=124 * 1024 * 1024),
    )(A_x.reshape(32, 8, 8, D), A_w_r.T, A_w_i.T,
      B_x.reshape(32, 2, 4, 8, D), B_mem0.reshape(NMEM, D),
      B_Wq, B_Wk, B_Wv, B_Wo.reshape(H * DH, D),
      *[jnp.asarray(c) for c in _fft_constants()])
    return out.reshape(1, S, 2 * D)
```

```python
import functools

import numpy as np
import jax
import jax.numpy as jnp
from jax import lax
import jax.experimental.pallas as pl
import jax.experimental.pallas.tpu as pltpu

S, D = 2048, 1024
H, DH = 32, 128
NMEM, SEG = 8, 32
NSEG = S // SEG
NPRE = NSEG * 8
UNROLL = 2
WP_ROWS = 33 * 64
NSLOT = 12

F32, BF16, U32 = jnp.float32, jnp.bfloat16, jnp.uint32
_SQH = float(np.sqrt(0.5))


def _pack_rows(m):
    b = np.asarray(m, np.float32).astype(jnp.bfloat16).view(np.uint16).astype(np.uint32)
    return b[..., 0::2, :] | (b[..., 1::2, :] << 16)


@functools.lru_cache(maxsize=None)
def _fft_constants():
    d1 = np.arange(128)[:, None]
    mf = np.zeros((4, 256, 256))
    mi = np.zeros((4, 256, 256))
    for t, res in enumerate(((0, 4), (1, 7), (2, 6), (3, 5))):
        kf = 8 * (np.arange(128) % 64) + np.repeat(res, 64)
        k = kf[None, :]
        th = 2 * np.pi * ((d1 * k) % D) / D
        co, si = np.cos(th), np.sin(th)
        sg = (-1.0 if t in (1, 2) else 1.0) * np.where(k % 8 == t, 1.0, -1.0)
        mf[t] = np.block([[co, -si], [sg * si, sg * co]])
        mi[t] = mf[t].T * (2.0 / (S * D))
        if t == 0:
            m0 = np.concatenate([co[:, :64], -si[:, :64]], axis=1)
            m0[:, 64] = (-1.0) ** np.arange(128)
            m4 = np.concatenate([-si[:, 64:], co[:, 64:]], axis=1)
            w0 = np.where(np.arange(128) % 64 == 0, 1.0, 2.0)
            mf[0], mi[0] = 0.0, 0.0
            mf[0, :128, :128], mf[0, :128, 128:] = m0, m4
            mi[0, :128, :128] = (m0 * w0).T / (S * D)
            mi[0, :128, 128:] = m4.T * (2.0 / (S * D))
    m = np.arange(64)[:, None]
    s1 = np.arange(64)[None, :]
    gf = np.zeros((32, 128, 128))
    gi = np.zeros((32, 128, 128))
    for r in range(32):
        th = 2 * np.pi * ((s1 * (32 * m + r)) % S) / S
        gr, gim = np.cos(th), -np.sin(th)
        g = np.block([[gr, -gim], [gim, gr]])
        gf[r, :, 0::2], gf[r, :, 1::2] = g[:, :64], g[:, 64:]
        gi[r, :, 0::2], gi[r, :, 1::2] = g.T[:, :64], g.T[:, 64:]
    idx = np.arange(128)
    lane, r = idx[:, None], idx[None, :]
    live = (lane < 32) & (r < 32) & (lane // 16 == r % 2)
    th32 = 2 * np.pi * ((lane % 16) * r % 32) / 32
    fc, fs = np.cos(th32) * live, -np.sin(th32) * live
    small = np.stack([fc, fs, fc.T, fs.T,
                      (lane % 32 == r) * 1.0])
    thw = 2 * np.pi * (idx[:64, None] * idx[None, :] % S) / S
    tw = np.stack([np.cos(thw), -np.sin(thw)]).astype(np.float32)
    return (_pack_rows(mf), _pack_rows(mi), _pack_rows(small), tw,
            _pack_rows(gf), _pack_rows(gi))


def _bfly8(x):
    x0, x1, x2, x3, x4, x5, x6, x7 = x
    t0, t1, t2, t3 = x0 + x4, x0 - x4, x2 + x6, x2 - x6
    t4, t5, t6, t7 = x1 + x5, x1 - x5, x3 + x7, x3 - x7
    u0, u1, u2, u3 = t0 + t2, t0 - t2, t4 + t6, t4 - t6
    p, q = _SQH * (t5 - t7), _SQH * (t5 + t7)
    return [(u0 + u2, u0 - u2), (t1 + p, t3 + q), (u1, u3), (t1 - p, t3 - q)]


def _bfly8_t(planes):
    (a0, a4), (a1r, a1i), (u1, u3), (a3r, a3i) = planes
    u0, u2 = a0 + a4, a0 - a4
    t1, p, t3, q = a1r + a3r, a1r - a3r, a1i + a3i, a1i - a3i
    t5, t7 = _SQH * (p + q), _SQH * (q - p)
    t0, t2, t4, t6 = u0 + u1, u0 - u1, u2 + u3, u2 - u3
    return [t0 + t1, t4 + t5, t2 + t3, t6 + t7, t0 - t1, t4 - t5, t2 - t3, t6 - t7]


def _dft4(z):
    (ar, ai), (br, bi), (cr, ci), (dr, di) = z
    er, ei, fr, fi = ar + cr, ai + ci, ar - cr, ai - ci
    gr, gi, hr, hi = br + dr, bi + di, br - dr, bi - di
    return [(er + gr, ei + gi), (fr + hi, fi - hr), (er - gr, ei - gi), (fr - hi, fi + hr)]


def _twiddle(z, e):
    re, im = z
    if e == 0:
        return z
    if e == 8:
        return im, -re
    if e == 4:
        return _SQH * (re + im), _SQH * (im - re)
    if e == 12:
        return _SQH * (im - re), -_SQH * (re + im)
    c, s = float(np.cos(np.pi * e / 16)), float(np.sin(np.pi * e / 16))
    return re * c + im * s, im * c - re * s


def _dft16(z):
    cols = [_dft4([z[a + 4 * b] for b in range(4)]) for a in range(4)]
    out = [None] * 16
    for r1 in range(4):
        y = _dft4([_twiddle(cols[a][r1], 2 * a * r1) for a in range(4)])
        for r2 in range(4):
            out[r1 + 4 * r2] = y[r2]
    return out


def _swap(z):
    return [(im, re) for re, im in z]


def _half_dft32(z, odd):
    return _dft16([_twiddle(v, b * odd) for b, v in enumerate(z)])


def _half_idft32(z, odd):
    return _swap([_twiddle(v, b * odd) for b, v in enumerate(_dft16(_swap(z)))])


def _bf(x):
    return pltpu.bitcast(x, BF16)


def _pack(re, im):
    return pltpu.pack_elementwise([re, im], packed_dtype=BF16)


def _low_halves(a, b):
    return (a & jnp.uint32(0xFFFF)) | (b << 16)


def _high_halves(a, b):
    return (a >> 16) | (b & jnp.uint32(0xFFFF0000))


def _dot(a, b):
    return jnp.dot(a, b, preferred_element_type=F32)


def _dot_nt(a, b):
    return lax.dot_general(a, b, (((1,), (1,)), ((), ())), preferred_element_type=F32)


def _softmax(sc):
    e = jnp.exp(sc - jnp.max(sc, axis=-1, keepdims=True))
    l = jnp.sum(e, axis=-1, keepdims=True)
    r = pltpu.reciprocal(l, approx=True)
    return e * (r * (2.0 - l * r))


def _scope(name):
    return jax.named_scope(name)


def _kernel(ax_hbm, wr_hbm, wi_hbm, bx_hbm, mem0_hbm, wq_hbm, wk_hbm, wv_hbm, wo_hbm,
            mf_hbm, mi_hbm, ms_hbm, tw_hbm, gf_hbm, gi_hbm,
            out_hbm,
            xa, wraw, wnyq, wp, mf, mi, ms, tw, gf, gi, ybuf, ubuf, nyq,
            xs, xpre3, xpre, stage, wqkv, wo, pre, kvmem, obuf, opre, part,
            sem_xa, sem_c, sem_f, sem_g, sem_w, sem_wo, sem_out):
    copy = pltpu.make_async_copy
    w_hbm = (wq_hbm, wk_hbm, wv_hbm)
    f_hbm = (wr_hbm, wi_hbm)

    def xa_copy(c):
        return copy(ax_hbm.at[:, c], xa.at[c], sem_xa.at[c])

    mf_copy = copy(mf_hbm, mf, sem_c.at[0])
    ms_copy = copy(ms_hbm, ms, sem_c.at[1])
    xpre_copy = copy(bx_hbm.at[:, :, 0], xpre3, sem_c.at[2])
    tw_copy = copy(tw_hbm, tw, sem_c.at[3])
    mi_copy = copy(mi_hbm, mi, sem_c.at[4])
    xs_copy = copy(bx_hbm.at[:, :, pl.ds(1, 3)], xs.at[pl.ds(0, 32), :, pl.ds(1, 3)], sem_c.at[5])
    mem_copy = copy(mem0_hbm, xs.at[0, 0, 0], sem_c.at[6])
    nyq_copies = [copy(f_hbm[i].at[pl.ds(D // 2, 1)], wnyq.at[i], sem_c.at[7 + i])
                  for i in range(2)]

    def f_copy(i, kap):
        src = f_hbm[i].at[pl.ds(0, D // 2)].bitcast(U32)
        return copy(src.at[:, pl.ds(pl.multiple_of(kap * 128, 128), 128)],
                    wraw.at[pl.ds(pl.multiple_of((kap * 2 + i) * 256, 256), 256)],
                    sem_f.at[kap * 2 + i])

    gf_copy = copy(gf_hbm, gf, sem_g.at[0])
    gi_copy = copy(gi_hbm, gi, sem_g.at[1])

    def w_copy(mat, pair, slot):
        return copy(w_hbm[mat].bitcast(U32).at[:, pair, :],
                    stage.at[pl.ds(pl.multiple_of(slot * D, D), D)], sem_w.at[slot])

    def wo_copy(n):
        return copy(wo_hbm.bitcast(U32).at[:, pl.ds(pl.multiple_of(n * 128, 128), 128)],
                    wo.at[n], sem_wo.at[n])

    def y_copy(c):
        return copy(xa.at[c], out_hbm.at[:, c // 4, c % 4, :, pl.ds(0, D)], sem_out.at[0])

    o_copy = copy(xs.at[pl.ds(0, 32), :, pl.ds(1, 3)],
                  out_hbm.at[:, :, pl.ds(1, 3), :, pl.ds(D, D)], sem_out.at[1])

    def opre_copy(g):
        return copy(xs.at[pl.ds(8 * g, 8), :, 0],
                    out_hbm.at[pl.ds(8 * g, 8), :, 0, :, pl.ds(D, D)], sem_out.at[2])

    xpre_copy.start()
    pl.loop(0, NSLOT)(lambda slot: w_copy(0, slot, slot).start())
    mf_copy.start()
    ms_copy.start()

    lane = lax.broadcasted_iota(jnp.int32, (8, 128), 1)
    lanes = lax.broadcasted_iota(jnp.int32, (128, 128), 1)

    def a_forward(c, odd):
        row = pl.ds(pl.multiple_of(c * 8, 8), 8)
        lhs = []
        for part_ in range(2):
            lo = xa[c, pl.ds(8 * part_, 8)].astype(F32).reshape(64, D)
            hi = xa[c, pl.ds(16 + 8 * part_, 8)].astype(F32).reshape(64, D)
            xh = lo - hi if odd else lo + hi
            planes = _bfly8([xh[:, 128 * i:128 * (i + 1)] for i in range(8)])
            lhs.append([jnp.concatenate(planes[t], axis=1).astype(BF16) for t in range(4)])
            yield
        lhs = [jnp.concatenate([lhs[0][t], lhs[1][t]], axis=0) for t in range(4)]
        x1 = {}

        def butterflies(t):
            v = x1.pop(t)
            y = _half_dft32([(v[8 * b:8 * b + 8, :128], v[8 * b:8 * b + 8, 128:])
                             for b in range(16)], odd)
            for r in range(16):
                ybuf[2 * r + odd, row, 128 * t:128 * (t + 1)] = _pack(*y[r])

        p0 = _dot(lhs[0][:, :128], _bf(mf[0, :64, :128]))
        p4 = _dot(lhs[0][:, 128:], _bf(mf[0, :64, 128:]))
        x1[1] = _dot(lhs[1], _bf(mf[1]))
        low = lanes < 64
        im = pltpu.roll(jnp.where(low, p4, p0), 64, 1)
        x1[0] = jnp.concatenate([jnp.where(low, p0, p4), jnp.where(lanes == 0, 0.0, im)], axis=1)
        acc = nyq[row, :] if odd else jnp.zeros((8, 128), F32)
        for b in range(16):
            k = 16 * odd + b
            v = im[8 * b:8 * b + 8]
            acc = jnp.where(lane == k, pltpu.roll(v, k, 1) if k else v, acc)
        nyq[row, :] = acc
        butterflies(0)
        yield
        x1[2] = _dot(lhs[2], _bf(mf[2]))
        x1[3] = _dot(lhs[3], _bf(mf[3]))
        butterflies(1)
        yield
        butterflies(2)
        yield
        butterflies(3)
        yield

    def a_filter_layout(it, i):
        base = (4 * it + i) * 512
        wr = [wraw[pl.ds(base + j, 64, stride=4), :] for j in range(4)]
        wi = [wraw[pl.ds(base + 256 + j, 64, stride=4), :] for j in range(4)]
        res = [(_low_halves, _high_halves)[k % 2](wr[k // 2], wi[k // 2]) for k in range(8)]
        for t, (lo, hi) in enumerate(((0, 4), (1, 7), (2, 6), (3, 5))):
            tile = jnp.concatenate([res[lo], res[hi]], axis=0).T
            dst = wp.at[pl.ds(pl.multiple_of(t * WP_ROWS + it * 528, 8), 528)]
            for mm in range(4):
                dst[pl.ds(33 * (4 * i + mm), 32), :] = tile[32 * mm:32 * (mm + 1)]

    def a_nyquist():
        b = nyq[...].astype(BF16)
        yr, yi = _dot(b, _bf(ms[0])), _dot(b, _bf(ms[1]))
        sub = lax.broadcasted_iota(jnp.int32, (8, 128), 0)
        wn = []
        for i in range(2):
            w = wnyq[i].astype(F32)
            spread = jnp.concatenate(
                [jnp.where(lane // 32 == sub % 4,
                           jnp.where(sub < 4, w[:, 256 * k:256 * k + 128],
                                     w[:, 256 * k + 128:256 * k + 256]), 0.0)
                 for k in range(8)], axis=0)
            wn.append(_dot(spread.astype(BF16), _bf(ms[4])))
        yield
        yield
        tc, ts = tw[0], tw[1]
        x2 = _dot(_bf(gf[0]), _bf(_pack(yr * tc - yi * ts, yr * ts + yi * tc)))
        yield
        yield
        a, b2 = x2[:64], x2[64:]
        u = _dot(_bf(gi[0]), _bf(_pack(a * wn[0] - b2 * wn[1], a * wn[1] + b2 * wn[0])))
        yield
        yield
        ur, ui = u[:64], u[64:]
        nyq[...] = (_dot((ur * tc + ui * ts).astype(BF16), _bf(ms[2]))
                    + _dot((ui * tc - ur * ts).astype(BF16), _bf(ms[3])))

    def a_filter(it, side=()):
        z = {}
        side = iter(side)

        def fwd(i):
            r = 8 * it + i
            x2 = _dot(_bf(gf[r]), _bf(ybuf[r]))
            parts = []
            for t in range(4):
                w = wp[pl.ds(t * WP_ROWS + r, 64, stride=33), :]
                wr = pltpu.bitcast(w << 16, F32)
                wi = pltpu.bitcast(w & jnp.uint32(0xFFFF0000), F32)
                a, b = x2[:64, 128 * t:128 * (t + 1)], x2[64:, 128 * t:128 * (t + 1)]
                parts.append(_pack(a * wr - b * wi, a * wi + b * wr))
            z[i] = jnp.concatenate(parts, axis=1)

        def inv(i):
            r = 8 * it + i
            ubuf[r] = _dot(_bf(gi[r]), _bf(z.pop(i)))

        lag = 2
        for i in range(8 + lag):
            next(side, None)
            if i < 8:
                fwd(i)
            if i >= lag:
                inv(i - lag)

    def a_inverse(c, odd, halves):
        r0 = pl.multiple_of(c * 8, 8)
        planes = []

        def tile(t):
            cols = slice(128 * t, 128 * (t + 1))
            x3 = _half_idft32(
                [(ubuf[2 * r + odd, pl.ds(r0, 8), cols],
                  ubuf[2 * r + odd, pl.ds(64 + r0, 8), cols]) for r in range(16)], odd)
            re, im = [jnp.concatenate([v[p] for v in x3], axis=0) for p in range(2)]
            if t:
                o = _dot(jnp.concatenate([re, im], axis=1).astype(BF16), _bf(mi[t]))
                planes.append((o[:, :128], o[:, 128:]))
                return
            bn = nyq[pl.ds(r0, 8), :]
            bn = jnp.concatenate(
                [pltpu.roll(bn, 64 - 16 * odd - b, 1) for b in range(16)], axis=0)
            low = lanes < 64
            im = pltpu.roll(im, 64, 1)
            q0 = jnp.where(low, re, jnp.where(lanes == 64, bn, im))
            q4 = jnp.where(low, im, re)
            planes.append((_dot(q0.astype(BF16), _bf(mi[0, :64, :128])),
                           _dot(q4.astype(BF16), _bf(mi[0, :64, 128:]))))

        tile(0)
        yield
        tile(1)
        tile(2)
        yield
        tile(3)
        yield
        halves.append(jnp.concatenate(_bfly8_t(planes), axis=1))
        if odd:
            y = jnp.concatenate([halves[0] + halves[1], halves[0] - halves[1]], axis=0)
            xa[c] = y.reshape(32, 8, D).astype(BF16)
        yield

    xpre_copy.wait()
    xpre[...] = pltpu.bitcast(xpre3[...].reshape(NPRE, D), U32)

    def project_pair(mat, pair, slot, side):
        ev = stage[pl.ds(slot * D, D // 2, stride=2), :]
        od = stage[pl.ds(slot * D + 1, D // 2, stride=2), :]
        lo, hi = _low_halves(ev, od), _high_halves(ev, od)
        wqkv[6 * pair + mat] = lo
        wqkv[6 * pair + 3 + mat] = hi
        if side is None:
            p = _dot(_bf(xpre[...]), _bf(jnp.concatenate([lo, hi], axis=1))).astype(BF16)
            pre[mat, 2 * pair] = p[:, :DH]
            pre[mat, 2 * pair + 1] = p[:, DH:]
            return
        for j in range(4):
            next(side)
            if j:
                lo, hi = wqkv[6 * pair + mat], wqkv[6 * pair + 3 + mat]
            p = _dot(_bf(xpre[64 * j:64 * (j + 1), :]),
                     _bf(jnp.concatenate([lo, hi], axis=1))).astype(BF16)
            pre[mat, 2 * pair, 128 * j:128 * (j + 1), :] = p[:, :DH]
            pre[mat, 2 * pair + 1, 128 * j:128 * (j + 1), :] = p[:, DH:]

    def project_loop(name, mat, npair, before, side, after):
        def body(it, carry):
            first = npair * it
            slot0 = (16 * mat + first) % NSLOT
            for i in range(npair):
                w_copy(mat, first + i, slot0 + i).wait()
            before(it)
            work = side(it)
            for i in range(npair):
                project_pair(mat, first + i, slot0 + i, work)

            @pl.when(first + NSLOT < 16)
            def _():
                for i in range(npair):
                    w_copy(mat, first + NSLOT + i, slot0 + i).start()

            if mat < 2:
                @pl.when(first + NSLOT >= 16)
                def _():
                    for i in range(npair):
                        w_copy(mat + 1, first + NSLOT - 16 + i, slot0 + i).start()

            after(it)
            return carry

        with _scope(name):
            lax.fori_loop(0, 16 // npair, body, 0)

    def nothing(*_):
        pass

    def fetch_a_inputs(it):
        xa_copy(it).start()
        for kap in range(2):
            f_copy(0, 2 * it + kap).start()
            f_copy(1, 2 * it + kap).start()

    def wait_a_inputs(it):
        for c in range(2):
            xa_copy(2 * it + c).wait()
        for kap in range(4):
            f_copy(0, 4 * it + kap).wait()
            f_copy(1, 4 * it + kap).wait()

    def forward_fft(it):
        units = [a_forward(2 * it + u // 2, u % 2) for u in range(4)]
        for u in range(4):
            for stage_ in range(4):
                if u and stage_ < 2:
                    next(units[u - 1])
                next(units[u])
                if stage_ == 2:
                    a_filter_layout(it, u)
                if u == 3 and stage_ == 3:
                    next(units[u])
                    next(units[u])
                yield

    def fetch_late_inputs(it):
        wo_copy(2 * it).start()
        wo_copy(2 * it + 1).start()

    def inverse_fft(it):
        for c in range(2):
            halves = []
            for odd in range(2):
                yield from a_inverse(2 * it + c, odd, halves)

    def store_y(it):
        for c in range(2):
            y_copy(2 * it + c).start()

    project_loop("B_proj_q", 0, 2, nothing, nothing, fetch_a_inputs)
    for cp in (tw_copy, *nyq_copies, mi_copy, gf_copy, gi_copy):
        cp.start()
    mf_copy.wait()
    ms_copy.wait()
    project_loop("B_proj_k", 1, 4, wait_a_inputs, forward_fft, fetch_late_inputs)
    xs_copy.start()
    mem_copy.start()
    with _scope("g_wait"):
        for cp in (tw_copy, *nyq_copies, mi_copy, gf_copy, gi_copy):
            cp.wait()
    with _scope("A_filt"):
        a_filter(0, a_nyquist())
        pl.loop(1, 4)(a_filter)
    project_loop("B_proj_v", 2, 4, nothing, inverse_fft, store_y)

    with _scope("wo_wait"):
        for n in range(8):
            wo_copy(n).wait()
        xs_copy.wait()
        mem_copy.wait()
    scale = DH ** -0.5

    def out_proj(lhs, h0, h1):
        return jnp.concatenate(
            [_dot(lhs, _bf(wo[n, h0 * 64:h1 * 64, :])) for n in range(8)], axis=1)

    def segment(s, h, split):
        row = lax.broadcasted_iota(jnp.int32, (32, 48), 0)
        col = lax.broadcasted_iota(jnp.int32, (32, 48), 1)
        allowed = ((row < NMEM) | (col >= 32) | (col <= row)) & (col < 40)
        p0 = pl.ds(pl.multiple_of(s * 8, 8), 8)
        zeros = jnp.zeros((8, DH), BF16)
        st = {}

        def half(i, a):
            return _dot(h[:, 512 * a:512 * (a + 1)], _bf(wqkv[i, 256 * a:256 * (a + 1), :]))

        def qkv(hd):
            if hd == 0 and split:
                for i in range(3):
                    part[i] = half(i, 0)
                q, k, v = [(part[i] + half(i, 1)).astype(BF16) for i in range(3)]
            else:
                q, k, v = [_dot(h, _bf(wqkv[3 * hd + i])).astype(BF16) for i in range(3)]
            kvmem[0, hd, p0, :] = k[:NMEM]
            kvmem[1, hd, p0, :] = v[:NMEM]
            st[hd] = (q, k, v)

        def scores(hd):
            q, k, v = st[hd]
            ka = jnp.concatenate([k, pre[1, hd, p0, :], zeros], axis=0)
            sc = jnp.where(allowed, _dot_nt(q, ka) * scale, -jnp.inf)
            st[hd] = (_softmax(sc).astype(BF16), v)

        def context(hd):
            p, v = st.pop(hd)
            va = jnp.concatenate([v, pre[2, hd, p0, :], zeros], axis=0)
            obuf[:, hd * DH:(hd + 1) * DH] = _dot(p, va).astype(BF16)

        acc = [None] * 8

        def project(g):
            lhs = obuf[:, 4 * g * DH:4 * (g + 1) * DH]
            for n in range(8):
                t = _dot(lhs, _bf(wo[n, 256 * g:256 * (g + 1), :]))
                acc[n] = t if acc[n] is None else acc[n] + t

        d1, d2, first = 1, 3, 28
        for hd in range(H):
            qkv(hd)
            if hd >= d1:
                scores(hd - d1)
            if hd >= d2:
                context(hd - d2)
            if hd == first:
                project(0)
        for t, g in enumerate(range(1, H // 4)):
            project(g)
            if t < d1:
                scores(H + t - d1)
            if t < d2:
                context(H + t - d2)
        return acc

    def steps(i, carry):
        h = xs[(UNROLL // 2) * i, 0].reshape(32, D)
        for u in range(UNROLL):
            acc = segment(UNROLL * i + u, h, u > 0)
            nxt = ((UNROLL // 2) * i + (u + 1) // 2, (u + 1) % 2)
            if u + 1 < UNROLL:
                xt = xs[nxt[0], nxt[1], pl.ds(1, 3)].astype(F32).reshape(24, D)
                h = jnp.concatenate(
                    [jnp.concatenate([acc[n][:NMEM], xt[:, 128 * n:128 * (n + 1)]],
                                     axis=0).astype(BF16) for n in range(8)], axis=1)
            ob = jnp.concatenate(acc, axis=1).astype(BF16).reshape(4, 8, D)
            xs[(UNROLL // 2) * i + u // 2, u % 2, pl.ds(1, 3)] = ob[1:]
            if u + 1 == UNROLL:
                xs[nxt[0], nxt[1], 0] = ob[0]
        return carry

    with _scope("B_step"):
        lax.fori_loop(0, NSEG // UNROLL, steps, 0)
    o_copy.start()

    def finish(g, carry):
        row = lax.broadcasted_iota(jnp.int32, (64, 128), 0)
        col = lax.broadcasted_iota(jnp.int32, (64, 128), 1)
        allowed = ((col % 64) // 8 == row // 8) & ((col < 64) | (col % 8 <= row % 8))
        st = {}

        def rows(a):
            return pl.ds(pl.multiple_of(g * 128 + a * 64, 64), 64)

        def scores(hd):
            for a in range(2):
                ka = jnp.concatenate([kvmem[0, hd, rows(a), :], pre[1, hd, rows(a), :]], axis=0)
                sc = jnp.where(allowed, _dot_nt(pre[0, hd, rows(a), :], ka) * scale, -jnp.inf)
                st[hd, a] = _softmax(sc).astype(BF16)

        def context(hd):
            for a in range(2):
                va = jnp.concatenate([kvmem[1, hd, rows(a), :], pre[2, hd, rows(a), :]], axis=0)
                opre[a * 64:(a + 1) * 64, hd * DH:(hd + 1) * DH] = (
                    _dot(st.pop((hd, a)), va).astype(BF16))

        acc = [None]

        def project(c):
            t = out_proj(opre[:, 8 * c * DH:8 * (c + 1) * DH], 8 * c, 8 * (c + 1))
            acc[0] = t if acc[0] is None else acc[0] + t

        for c in range(H // 8 + 2):
            if c < H // 8:
                for hd in range(8 * c, 8 * c + 8):
                    scores(hd)
            if 2 <= c:
                project(c - 2)
            if 1 <= c <= H // 8:
                for hd in range(8 * (c - 1), 8 * c):
                    context(hd)
        xs[pl.ds(g * 8, 8), :, 0] = acc[0].astype(BF16).reshape(8, 2, 8, D)
        opre_copy(g).start()
        return carry

    with _scope("B_fin"):
        lax.fori_loop(0, 4, finish, 0)

    with _scope("drain"):
        for c in range(8):
            y_copy(c).wait()
        o_copy.wait()
        for g in range(4):
            opre_copy(g).wait()


@functools.partial(jax.jit, static_argnames=("B_seg_len",))
def pallas_concat_heads__spectral_gfnet__memory_aug_recurrent_mem_tr__prompt_kernel(
    A_x, A_w_r, A_w_i, B_x, B_mem0, B_Wq, B_Wk, B_Wv, B_Wo, B_seg_len=SEG,
):
    assert A_x.shape == (1, S, D) and B_x.shape == (1, S, D)
    assert A_w_r.shape == A_w_i.shape == (S, D // 2 + 1)
    assert B_mem0.shape == (1, NMEM, D) and B_seg_len == SEG
    assert B_Wq.shape == B_Wk.shape == B_Wv.shape == (D, H, DH) and B_Wo.shape == (H, DH, D)

    vmem = pltpu.VMEM
    dma = pltpu.SemaphoreType.DMA
    scratch = [
        vmem((8, 32, 8, D), BF16),
        vmem((32 * 256 + 32, 128), U32),
        vmem((2, 1, S), BF16),
        vmem((4 * WP_ROWS + 32, 128), U32),
        vmem((4, 128, 256), U32),
        vmem((4, 128, 256), U32),
        vmem((5, 64, 128), U32),
        vmem((2, 64, 128), F32),
        vmem((32, 64, 128), U32),
        vmem((32, 64, 128), U32),
        vmem((32, 64, 512), U32),
        vmem((32, 128, 512), F32),
        vmem((64, 128), F32),
        vmem((33, 2, 4, 8, D), BF16),
        vmem((32, 2, 8, D), BF16),
        vmem((NPRE // 2, D), U32),
        vmem((NSLOT * D + 32, 128), U32),
        vmem((3 * H, D // 2, DH), U32),
        vmem((8, H * DH // 2, 128), U32),
        vmem((3, H, NPRE, DH), BF16),
        vmem((2, H, NPRE, DH), BF16),
        vmem((32, H * DH), BF16),
        vmem((128, H * DH), BF16),
        vmem((3, 32, DH), F32),
        dma((8,)), dma((9,)), dma((32,)), dma((2,)), dma((NSLOT,)), dma((8,)), dma((3,)),
    ]
    hbm = pl.BlockSpec(memory_space=pltpu.HBM)
    out = pl.pallas_call(
        _kernel,
        out_shape=jax.ShapeDtypeStruct((32, 2, 4, 8, 2 * D), BF16),
        in_specs=[hbm] * 15,
        out_specs=hbm,
        scratch_shapes=scratch,
        compiler_params=pltpu.CompilerParams(vmem_limit_bytes=124 * 1024 * 1024),
    )(A_x.reshape(32, 8, 8, D), A_w_r.T, A_w_i.T,
      B_x.reshape(32, 2, 4, 8, D), B_mem0.reshape(NMEM, D),
      B_Wq, B_Wk, B_Wv, B_Wo.reshape(H * DH, D),
      *[jnp.asarray(c) for c in _fft_constants()])
    return out.reshape(1, S, 2 * D)
```

```python
import functools

import numpy as np
import jax
import jax.numpy as jnp
from jax import lax
import jax.experimental.pallas as pl
import jax.experimental.pallas.tpu as pltpu

S, D = 2048, 1024
H, DH = 32, 128
NMEM, SEG = 8, 32
NSEG = S // SEG
NPRE = NSEG * 8
NSLOT = 12
WP_ROWS = 33 * 64
RESIDUES = ((0, 4), (1, 7), (2, 6), (3, 5))

F32, BF16, U32 = jnp.float32, jnp.bfloat16, jnp.uint32
_SQH = float(np.sqrt(0.5))


def _pack_rows(m):
    b = np.asarray(m, np.float32).astype(jnp.bfloat16).view(np.uint16).astype(np.uint32)
    return b[..., 0::2, :] | (b[..., 1::2, :] << 16)


@functools.lru_cache(maxsize=None)
def _fft_constants():
    idx = np.arange(128)
    mf = np.zeros((4, 256, 256))
    mi = np.zeros((4, 256, 256))
    for t, res in enumerate(RESIDUES):
        k = (8 * (idx % 64) + np.repeat(res, 64))[None, :]
        th = 2 * np.pi * ((idx[:, None] * k) % D) / D
        co, si = np.cos(th), np.sin(th)
        if t:
            sg = (-1.0 if t in (1, 2) else 1.0) * np.where(k % 8 == t, 1.0, -1.0)
            mf[t] = np.block([[co, -si], [sg * si, sg * co]])
            mi[t] = mf[t].T * (2.0 / (S * D))
        else:
            m0 = np.concatenate([co[:, :64], -si[:, :64]], axis=1)
            m0[:, 64] = (-1.0) ** idx
            m4 = np.concatenate([-si[:, 64:], co[:, 64:]], axis=1)
            once = np.where(idx % 64 == 0, 1.0, 2.0)
            mf[0, :128, :128], mf[0, :128, 128:] = m0, m4
            mi[0, :128, :128] = (m0 * once).T / (S * D)
            mi[0, :128, 128:] = m4.T * (2.0 / (S * D))
    gf = np.zeros((32, 128, 128))
    gi = np.zeros((32, 128, 128))
    for r in range(32):
        th = 2 * np.pi * ((idx[None, :64] * (32 * idx[:64, None] + r)) % S) / S
        gr, gim = np.cos(th), -np.sin(th)
        g = np.block([[gr, -gim], [gim, gr]])
        gf[r, :, 0::2], gf[r, :, 1::2] = g[:, :64], g[:, 64:]
        gi[r, :, 0::2], gi[r, :, 1::2] = g.T[:, :64], g.T[:, 64:]
    lane, r = idx[:, None], idx[None, :]
    live = (lane < 32) & (r < 32) & (lane // 16 == r % 2)
    th = 2 * np.pi * ((lane % 16) * r % 32) / 32
    fc, fs = np.cos(th) * live, -np.sin(th) * live
    small = np.stack([fc, fs, fc.T, fs.T,
                      (lane % 32 == r) * 1.0])
    th = 2 * np.pi * (idx[:64, None] * idx[None, :] % S) / S
    tw = np.stack([np.cos(th), -np.sin(th)]).astype(np.float32)
    return (_pack_rows(mf), _pack_rows(mi), _pack_rows(small), tw,
            _pack_rows(gf), _pack_rows(gi))


def _bfly8(x):
    x0, x1, x2, x3, x4, x5, x6, x7 = x
    t0, t1, t2, t3 = x0 + x4, x0 - x4, x2 + x6, x2 - x6
    t4, t5, t6, t7 = x1 + x5, x1 - x5, x3 + x7, x3 - x7
    u0, u1, u2, u3 = t0 + t2, t0 - t2, t4 + t6, t4 - t6
    p, q = _SQH * (t5 - t7), _SQH * (t5 + t7)
    return [(u0 + u2, u0 - u2), (t1 + p, t3 + q), (u1, u3), (t1 - p, t3 - q)]


def _bfly8_t(planes):
    (a0, a4), (a1r, a1i), (u1, u3), (a3r, a3i) = planes
    u0, u2 = a0 + a4, a0 - a4
    t1, p, t3, q = a1r + a3r, a1r - a3r, a1i + a3i, a1i - a3i
    t5, t7 = _SQH * (p + q), _SQH * (q - p)
    t0, t2, t4, t6 = u0 + u1, u0 - u1, u2 + u3, u2 - u3
    return [t0 + t1, t4 + t5, t2 + t3, t6 + t7, t0 - t1, t4 - t5, t2 - t3, t6 - t7]


def _dft4(z):
    (ar, ai), (br, bi), (cr, ci), (dr, di) = z
    er, ei, fr, fi = ar + cr, ai + ci, ar - cr, ai - ci
    gr, gi, hr, hi = br + dr, bi + di, br - dr, bi - di
    return [(er + gr, ei + gi), (fr + hi, fi - hr), (er - gr, ei - gi), (fr - hi, fi + hr)]


def _twiddle(z, e):
    re, im = z
    if e == 0:
        return z
    if e == 8:
        return im, -re
    if e == 4:
        return _SQH * (re + im), _SQH * (im - re)
    if e == 12:
        return _SQH * (im - re), -_SQH * (re + im)
    c, s = float(np.cos(np.pi * e / 16)), float(np.sin(np.pi * e / 16))
    return re * c + im * s, im * c - re * s


def _dft16(z):
    cols = [_dft4([z[a + 4 * b] for b in range(4)]) for a in range(4)]
    out = [None] * 16
    for r1 in range(4):
        y = _dft4([_twiddle(cols[a][r1], 2 * a * r1) for a in range(4)])
        for r2 in range(4):
            out[r1 + 4 * r2] = y[r2]
    return out


def _swap(z):
    return [(im, re) for re, im in z]


def _half_dft32(z, odd):
    return _dft16([_twiddle(v, b * odd) for b, v in enumerate(z)])


def _half_idft32(z, odd):
    return _swap([_twiddle(v, b * odd) for b, v in enumerate(_dft16(_swap(z)))])


def _bf(x):
    return pltpu.bitcast(x, BF16)


def _pack(re, im):
    return pltpu.pack_elementwise([re, im], packed_dtype=BF16)


def _low_halves(a, b):
    return (a & jnp.uint32(0xFFFF)) | (b << 16)


def _high_halves(a, b):
    return (a >> 16) | (b & jnp.uint32(0xFFFF0000))


def _dot(a, b):
    return jnp.dot(a, b, preferred_element_type=F32)


def _dot_nt(a, b):
    return lax.dot_general(a, b, (((1,), (1,)), ((), ())), preferred_element_type=F32)


def _softmax(sc):
    e = jnp.exp(sc - jnp.max(sc, axis=-1, keepdims=True))
    l = jnp.sum(e, axis=-1, keepdims=True)
    r = pltpu.reciprocal(l, approx=True)
    return e * (r * (2.0 - l * r))


def _kernel(ax_hbm, wr_hbm, wi_hbm, bx_hbm, mem0_hbm, wq_hbm, wk_hbm, wv_hbm, wo_hbm,
            mf_hbm, mi_hbm, ms_hbm, tw_hbm, gf_hbm, gi_hbm,
            out_hbm,
            xa, wraw, wnyq, wp, mf, mi, ms, tw, gf, gi, ybuf, ubuf, nyq,
            xs, xpre3, xpre, stage, wqkv, wo, pre, kvmem, obuf, opre, part,
            sem, sem_a, sem_w):
    copy = pltpu.make_async_copy
    w_hbm = (wq_hbm, wk_hbm, wv_hbm)
    f_hbm = (wr_hbm, wi_hbm)
    scale = DH ** -0.5

    xpre_copy = copy(bx_hbm.at[:, :, 0], xpre3, sem.at[0])
    mf_copy = copy(mf_hbm, mf, sem.at[1])
    filter_stage_copies = [
        copy(src, dst, sem.at[2])
        for src, dst in ((ms_hbm, ms), (tw_hbm, tw), (mi_hbm, mi), (gf_hbm, gf), (gi_hbm, gi),
                         (wr_hbm.at[pl.ds(D // 2, 1)], wnyq.at[0]),
                         (wi_hbm.at[pl.ds(D // 2, 1)], wnyq.at[1]))]
    step_copies = [
        copy(bx_hbm.at[:, :, pl.ds(1, 3)], xs.at[pl.ds(0, 32), :, pl.ds(1, 3)], sem.at[3]),
        copy(mem0_hbm, xs.at[0, 0, 0], sem.at[3])]
    o_copy = copy(xs.at[pl.ds(0, 32), :, pl.ds(1, 3)],
                  out_hbm.at[:, :, pl.ds(1, 3), :, pl.ds(D, D)], sem.at[4])

    def opre_copy(g):
        return copy(xs.at[pl.ds(8 * g, 8), :, 0],
                    out_hbm.at[pl.ds(8 * g, 8), :, 0, :, pl.ds(D, D)], sem.at[4])

    def y_copy(c):
        return copy(xa.at[c], out_hbm.at[:, c // 4, c % 4, :, pl.ds(0, D)], sem.at[4])

    def wo_copy(n):
        return copy(wo_hbm.bitcast(U32).at[:, pl.ds(pl.multiple_of(n * 128, 128), 128)],
                    wo.at[n], sem.at[3])

    def a_copies(c):
        copies = [copy(ax_hbm.at[:, c], xa.at[c], sem_a.at[c])]
        for kap in (2 * c, 2 * c + 1):
            for i in range(2):
                src = f_hbm[i].at[pl.ds(0, D // 2)].bitcast(U32)
                copies.append(copy(
                    src.at[:, pl.ds(pl.multiple_of(kap * 128, 128), 128)],
                    wraw.at[pl.ds(pl.multiple_of((kap * 2 + i) * 256, 256), 256)],
                    sem_a.at[c]))
        return copies

    def w_copy(mat, pair, slot):
        return copy(w_hbm[mat].bitcast(U32).at[:, pair, :],
                    stage.at[pl.ds(pl.multiple_of(slot * D, D), D)], sem_w.at[slot])

    xpre_copy.start()
    pl.loop(0, NSLOT)(lambda slot: w_copy(0, slot, slot).start())
    mf_copy.start()

    lane = lax.broadcasted_iota(jnp.int32, (8, 128), 1)
    lanes = lax.broadcasted_iota(jnp.int32, (128, 128), 1)

    def a_forward(c, odd):
        row = pl.ds(pl.multiple_of(c * 8, 8), 8)
        lhs = []
        for blk in range(2):
            lo = xa[c, pl.ds(8 * blk, 8)].astype(F32).reshape(64, D)
            hi = xa[c, pl.ds(16 + 8 * blk, 8)].astype(F32).reshape(64, D)
            xh = lo - hi if odd else lo + hi
            planes = _bfly8([xh[:, 128 * i:128 * (i + 1)] for i in range(8)])
            lhs.append([jnp.concatenate(planes[t], axis=1).astype(BF16) for t in range(4)])
            yield
        lhs = [jnp.concatenate([lhs[0][t], lhs[1][t]], axis=0) for t in range(4)]
        x1 = {}

        def butterflies(t):
            v = x1.pop(t)
            y = _half_dft32([(v[8 * b:8 * b + 8, :128], v[8 * b:8 * b + 8, 128:])
                             for b in range(16)], odd)
            for r in range(16):
                ybuf[2 * r + odd, row, 128 * t:128 * (t + 1)] = _pack(*y[r])

        p0 = _dot(lhs[0][:, :128], _bf(mf[0, :64, :128]))
        p4 = _dot(lhs[0][:, 128:], _bf(mf[0, :64, 128:]))
        x1[1] = _dot(lhs[1], _bf(mf[1]))
        low = lanes < 64
        im = pltpu.roll(jnp.where(low, p4, p0), 64, 1)
        x1[0] = jnp.concatenate([jnp.where(low, p0, p4), jnp.where(lanes == 0, 0.0, im)], axis=1)
        acc = nyq[row, :] if odd else jnp.zeros((8, 128), F32)
        for b in range(16):
            k = 16 * odd + b
            v = im[8 * b:8 * b + 8]
            acc = jnp.where(lane == k, pltpu.roll(v, k, 1) if k else v, acc)
        nyq[row, :] = acc
        butterflies(0)
        yield
        x1[2] = _dot(lhs[2], _bf(mf[2]))
        x1[3] = _dot(lhs[3], _bf(mf[3]))
        butterflies(1)
        yield
        butterflies(2)
        yield
        butterflies(3)
        yield

    def a_filter_layout(it, i):
        base = (4 * it + i) * 512
        wr = [wraw[pl.ds(base + j, 64, stride=4), :] for j in range(4)]
        wi = [wraw[pl.ds(base + 256 + j, 64, stride=4), :] for j in range(4)]
        res = [(_low_halves, _high_halves)[k % 2](wr[k // 2], wi[k // 2]) for k in range(8)]
        for t, (lo, hi) in enumerate(RESIDUES):
            tile = jnp.concatenate([res[lo], res[hi]], axis=0).T
            dst = wp.at[pl.ds(pl.multiple_of(t * WP_ROWS + it * 528, 8), 528)]
            for m in range(4):
                dst[pl.ds(33 * (4 * i + m), 32), :] = tile[32 * m:32 * (m + 1)]

    def a_nyquist():
        b = nyq[...].astype(BF16)
        yr, yi = _dot(b, _bf(ms[0])), _dot(b, _bf(ms[1]))
        sub = lax.broadcasted_iota(jnp.int32, (8, 128), 0)
        wn = []
        for i in range(2):
            w = wnyq[i].astype(F32)
            spread = jnp.concatenate(
                [jnp.where(lane // 32 == sub % 4,
                           jnp.where(sub < 4, w[:, 256 * k:256 * k + 128],
                                     w[:, 256 * k + 128:256 * k + 256]), 0.0)
                 for k in range(8)], axis=0)
            wn.append(_dot(spread.astype(BF16), _bf(ms[4])))
        yield
        yield
        tc, ts = tw[0], tw[1]
        x2 = _dot(_bf(gf[0]), _bf(_pack(yr * tc - yi * ts, yr * ts + yi * tc)))
        yield
        yield
        a, b = x2[:64], x2[64:]
        u = _dot(_bf(gi[0]), _bf(_pack(a * wn[0] - b * wn[1], a * wn[1] + b * wn[0])))
        yield
        yield
        ur, ui = u[:64], u[64:]
        nyq[...] = (_dot((ur * tc + ui * ts).astype(BF16), _bf(ms[2]))
                    + _dot((ui * tc - ur * ts).astype(BF16), _bf(ms[3])))

    def a_filter(it, side=()):
        z = {}
        side = iter(side)

        def fwd(i):
            r = 8 * it + i
            x2 = _dot(_bf(gf[r]), _bf(ybuf[r]))
            tiles = []
            for t in range(4):
                w = wp[pl.ds(t * WP_ROWS + r, 64, stride=33), :]
                wr = pltpu.bitcast(w << 16, F32)
                wi = pltpu.bitcast(w & jnp.uint32(0xFFFF0000), F32)
                a, b = x2[:64, 128 * t:128 * (t + 1)], x2[64:, 128 * t:128 * (t + 1)]
                tiles.append(_pack(a * wr - b * wi, a * wi + b * wr))
            z[i] = jnp.concatenate(tiles, axis=1)

        def inv(i):
            r = 8 * it + i
            ubuf[r] = _dot(_bf(gi[r]), _bf(z.pop(i)))

        lag = 2
        for i in range(8 + lag):
            next(side, None)
            if i < 8:
                fwd(i)
            if i >= lag:
                inv(i - lag)

    def a_inverse(c, odd, halves):
        r0 = pl.multiple_of(c * 8, 8)
        planes = []

        def tile(t):
            cols = slice(128 * t, 128 * (t + 1))
            x3 = _half_idft32(
                [(ubuf[2 * r + odd, pl.ds(r0, 8), cols],
                  ubuf[2 * r + odd, pl.ds(64 + r0, 8), cols]) for r in range(16)], odd)
            re, im = [jnp.concatenate([v[p] for v in x3], axis=0) for p in range(2)]
            if t:
                o = _dot(jnp.concatenate([re, im], axis=1).astype(BF16), _bf(mi[t]))
                planes.append((o[:, :128], o[:, 128:]))
                return
            bn = nyq[pl.ds(r0, 8), :]
            bn = jnp.concatenate(
                [pltpu.roll(bn, 64 - 16 * odd - b, 1) for b in range(16)], axis=0)
            low = lanes < 64
            im = pltpu.roll(im, 64, 1)
            q0 = jnp.where(low, re, jnp.where(lanes == 64, bn, im))
            q4 = jnp.where(low, im, re)
            planes.append((_dot(q0.astype(BF16), _bf(mi[0, :64, :128])),
                           _dot(q4.astype(BF16), _bf(mi[0, :64, 128:]))))

        tile(0)
        yield
        tile(1)
        tile(2)
        yield
        tile(3)
        yield
        halves.append(jnp.concatenate(_bfly8_t(planes), axis=1))
        if odd:
            y = jnp.concatenate([halves[0] + halves[1], halves[0] - halves[1]], axis=0)
            xa[c] = y.reshape(32, 8, D).astype(BF16)
        yield

    def project_pair(mat, pair, slot, side):
        ev = stage[pl.ds(slot * D, D // 2, stride=2), :]
        od = stage[pl.ds(slot * D + 1, D // 2, stride=2), :]
        lo, hi = _low_halves(ev, od), _high_halves(ev, od)
        wqkv[6 * pair + mat] = lo
        wqkv[6 * pair + 3 + mat] = hi
        nslice = 1 if side is None else 4
        rows = NPRE // nslice
        for j in range(nslice):
            if side is not None:
                next(side)
            if j:
                lo, hi = wqkv[6 * pair + mat], wqkv[6 * pair + 3 + mat]
            p = _dot(_bf(xpre[rows // 2 * j:rows // 2 * (j + 1), :]),
                     _bf(jnp.concatenate([lo, hi], axis=1))).astype(BF16)
            pre[mat, 2 * pair, rows * j:rows * (j + 1), :] = p[:, :DH]
            pre[mat, 2 * pair + 1, rows * j:rows * (j + 1), :] = p[:, DH:]

    def project_loop(mat, npair, before, side, after):
        @pl.loop(0, 16 // npair)
        def _(it):
            first = npair * it
            slot0 = (16 * mat + first) % NSLOT
            for i in range(npair):
                w_copy(mat, first + i, slot0 + i).wait()
            before(it)
            work = side(it)
            for i in range(npair):
                project_pair(mat, first + i, slot0 + i, work)

            @pl.when(first + NSLOT < 16)
            def _():
                for i in range(npair):
                    w_copy(mat, first + NSLOT + i, slot0 + i).start()

            if mat < 2:
                @pl.when(first + NSLOT >= 16)
                def _():
                    for i in range(npair):
                        w_copy(mat + 1, first + NSLOT - 16 + i, slot0 + i).start()

            after(it)

    def nothing(it):
        return None

    def fetch_a_inputs(it):
        for cp in a_copies(it):
            cp.start()

    def wait_a_inputs(it):
        for cp in a_copies(2 * it) + a_copies(2 * it + 1):
            cp.wait()

    def forward_fft(it):
        units = [a_forward(2 * it + u // 2, u % 2) for u in range(4)]
        for u in range(4):
            for k in range(4):
                if u and k < 2:
                    next(units[u - 1])
                next(units[u])
                if k == 2:
                    a_filter_layout(it, u)
                if u == 3 and k == 3:
                    next(units[u])
                    next(units[u])
                yield

    def fetch_wo(it):
        wo_copy(2 * it).start()
        wo_copy(2 * it + 1).start()

    def inverse_fft(it):
        for c in range(2):
            halves = []
            for odd in range(2):
                yield from a_inverse(2 * it + c, odd, halves)

    def store_y(it):
        y_copy(2 * it).start()
        y_copy(2 * it + 1).start()

    xpre_copy.wait()
    xpre[...] = pltpu.bitcast(xpre3[...].reshape(NPRE, D), U32)
    project_loop(0, 2, nothing, nothing, fetch_a_inputs)
    for cp in filter_stage_copies:
        cp.start()
    mf_copy.wait()
    project_loop(1, 4, wait_a_inputs, forward_fft, fetch_wo)
    for cp in step_copies:
        cp.start()
    for cp in filter_stage_copies:
        cp.wait()
    a_filter(0, a_nyquist())
    pl.loop(1, 4)(a_filter)
    project_loop(2, 4, nothing, inverse_fft, store_y)

    for cp in step_copies + [wo_copy(n) for n in range(8)]:
        cp.wait()

    def segment(s, h, split):
        row = lax.broadcasted_iota(jnp.int32, (32, 48), 0)
        col = lax.broadcasted_iota(jnp.int32, (32, 48), 1)
        allowed = ((row < NMEM) | (col >= 32) | (col <= row)) & (col < 40)
        p0 = pl.ds(pl.multiple_of(s * 8, 8), 8)
        zeros = jnp.zeros((8, DH), BF16)
        st = {}

        def half(i, a):
            return _dot(h[:, 512 * a:512 * (a + 1)], _bf(wqkv[i, 256 * a:256 * (a + 1), :]))

        def qkv(hd):
            if hd == 0 and split:
                for i in range(3):
                    part[i] = half(i, 0)
                q, k, v = [(part[i] + half(i, 1)).astype(BF16) for i in range(3)]
            else:
                q, k, v = [_dot(h, _bf(wqkv[3 * hd + i])).astype(BF16) for i in range(3)]
            kvmem[0, hd, p0, :] = k[:NMEM]
            kvmem[1, hd, p0, :] = v[:NMEM]
            st[hd] = (q, k, v)

        def scores(hd):
            q, k, v = st[hd]
            ka = jnp.concatenate([k, pre[1, hd, p0, :], zeros], axis=0)
            sc = jnp.where(allowed, _dot_nt(q, ka) * scale, -jnp.inf)
            st[hd] = (_softmax(sc).astype(BF16), v)

        def context(hd):
            p, v = st.pop(hd)
            va = jnp.concatenate([v, pre[2, hd, p0, :], zeros], axis=0)
            obuf[:, hd * DH:(hd + 1) * DH] = _dot(p, va).astype(BF16)

        acc = [None] * 8

        def project(g):
            lhs = obuf[:, 4 * g * DH:4 * (g + 1) * DH]
            for n in range(8):
                t = _dot(lhs, _bf(wo[n, 256 * g:256 * (g + 1), :]))
                acc[n] = t if acc[n] is None else acc[n] + t

        lag_scores, lag_context = 1, 3
        for hd in range(H):
            qkv(hd)
            if hd >= lag_scores:
                scores(hd - lag_scores)
            if hd >= lag_context:
                context(hd - lag_context)
            if hd == 28:
                project(0)
        for t, g in enumerate(range(1, H // 4)):
            project(g)
            if t < lag_scores:
                scores(H + t - lag_scores)
            if t < lag_context:
                context(H + t - lag_context)
        return acc

    @pl.loop(0, NSEG // 2)
    def _(i):
        acc = segment(2 * i, xs[i, 0].reshape(32, D), False)
        xt = xs[i, 1, pl.ds(1, 3)].astype(F32).reshape(24, D)
        h = jnp.concatenate(
            [jnp.concatenate([acc[n][:NMEM], xt[:, 128 * n:128 * (n + 1)]],
                             axis=0).astype(BF16) for n in range(8)], axis=1)
        ob = jnp.concatenate(acc, axis=1).astype(BF16).reshape(4, 8, D)
        xs[i, 0, pl.ds(1, 3)] = ob[1:]
        acc = segment(2 * i + 1, h, True)
        ob = jnp.concatenate(acc, axis=1).astype(BF16).reshape(4, 8, D)
        xs[i, 1, pl.ds(1, 3)] = ob[1:]
        xs[i + 1, 0, 0] = ob[0]

    o_copy.start()

    @pl.loop(0, 4)
    def _(g):
        row = lax.broadcasted_iota(jnp.int32, (64, 128), 0)
        col = lax.broadcasted_iota(jnp.int32, (64, 128), 1)
        allowed = ((col % 64) // 8 == row // 8) & ((col < 64) | (col % 8 <= row % 8))
        st = {}

        def rows(a):
            return pl.ds(pl.multiple_of(g * 128 + a * 64, 64), 64)

        def scores(hd):
            for a in range(2):
                ka = jnp.concatenate([kvmem[0, hd, rows(a), :], pre[1, hd, rows(a), :]], axis=0)
                sc = jnp.where(allowed, _dot_nt(pre[0, hd, rows(a), :], ka) * scale, -jnp.inf)
                st[hd, a] = _softmax(sc).astype(BF16)

        def context(hd):
            for a in range(2):
                va = jnp.concatenate([kvmem[1, hd, rows(a), :], pre[2, hd, rows(a), :]], axis=0)
                opre[a * 64:(a + 1) * 64, hd * DH:(hd + 1) * DH] = (
                    _dot(st.pop((hd, a)), va).astype(BF16))

        acc = None
        for c in range(H // 8 + 2):
            if c < H // 8:
                for hd in range(8 * c, 8 * c + 8):
                    scores(hd)
            if c >= 2:
                lhs = opre[:, 8 * (c - 2) * DH:8 * (c - 1) * DH]
                t = jnp.concatenate([_dot(lhs, _bf(wo[n, 512 * (c - 2):512 * (c - 1), :]))
                                     for n in range(8)], axis=1)
                acc = t if acc is None else acc + t
            if 1 <= c <= H // 8:
                for hd in range(8 * (c - 1), 8 * c):
                    context(hd)
        xs[pl.ds(g * 8, 8), :, 0] = acc.astype(BF16).reshape(8, 2, 8, D)
        opre_copy(g).start()

    for cp in [y_copy(c) for c in range(8)] + [o_copy] + [opre_copy(g) for g in range(4)]:
        cp.wait()


@functools.partial(jax.jit, static_argnames=("B_seg_len",))
def pallas_concat_heads__spectral_gfnet__memory_aug_recurrent_mem_tr__prompt_kernel(
    A_x, A_w_r, A_w_i, B_x, B_mem0, B_Wq, B_Wk, B_Wv, B_Wo, B_seg_len=SEG,
):
    assert A_x.shape == (1, S, D) and B_x.shape == (1, S, D)
    assert A_w_r.shape == A_w_i.shape == (S, D // 2 + 1)
    assert B_mem0.shape == (1, NMEM, D) and B_seg_len == SEG
    assert B_Wq.shape == B_Wk.shape == B_Wv.shape == (D, H, DH) and B_Wo.shape == (H, DH, D)

    vmem = pltpu.VMEM
    dma = pltpu.SemaphoreType.DMA
    scratch = [
        vmem((8, 32, 8, D), BF16),
        vmem((32 * 256 + 32, 128), U32),
        vmem((2, 1, S), BF16),
        vmem((4 * WP_ROWS + 32, 128), U32),
        vmem((4, 128, 256), U32),
        vmem((4, 128, 256), U32),
        vmem((5, 64, 128), U32),
        vmem((2, 64, 128), F32),
        vmem((32, 64, 128), U32),
        vmem((32, 64, 128), U32),
        vmem((32, 64, 512), U32),
        vmem((32, 128, 512), F32),
        vmem((64, 128), F32),
        vmem((33, 2, 4, 8, D), BF16),
        vmem((32, 2, 8, D), BF16),
        vmem((NPRE // 2, D), U32),
        vmem((NSLOT * D + 32, 128), U32),
        vmem((3 * H, D // 2, DH), U32),
        vmem((8, H * DH // 2, 128), U32),
        vmem((3, H, NPRE, DH), BF16),
        vmem((2, H, NPRE, DH), BF16),
        vmem((32, H * DH), BF16),
        vmem((128, H * DH), BF16),
        vmem((3, 32, DH), F32),
        dma((5,)), dma((8,)), dma((NSLOT,)),
    ]
    hbm = pl.BlockSpec(memory_space=pltpu.HBM)
    out = pl.pallas_call(
        _kernel,
        out_shape=jax.ShapeDtypeStruct((32, 2, 4, 8, 2 * D), BF16),
        in_specs=[hbm] * 15,
        out_specs=hbm,
        scratch_shapes=scratch,
        compiler_params=pltpu.CompilerParams(vmem_limit_bytes=124 * 1024 * 1024),
    )(A_x.reshape(32, 8, 8, D), A_w_r.T, A_w_i.T,
      B_x.reshape(32, 2, 4, 8, D), B_mem0.reshape(NMEM, D),
      B_Wq, B_Wk, B_Wv, B_Wo.reshape(H * DH, D),
      *[jnp.asarray(c) for c in _fft_constants()])
    return out.reshape(1, S, 2 * D)
```

```python
import functools

import numpy as np
import jax
import jax.numpy as jnp
from jax import lax
import jax.experimental.pallas as pl
import jax.experimental.pallas.tpu as pltpu

S, D = 2048, 1024
H, DH = 32, 128
NMEM, SEG = 8, 32
NSEG = S // SEG
NPRE = NSEG * 8
NSLOT = 12
WP_ROWS = 33 * 64
RESIDUES = ((0, 4), (1, 7), (2, 6), (3, 5))

F32, BF16, U32 = jnp.float32, jnp.bfloat16, jnp.uint32
_SQH = float(np.sqrt(0.5))


def _pack_rows(m):
    b = np.asarray(m, np.float32).astype(jnp.bfloat16).view(np.uint16).astype(np.uint32)
    return b[..., 0::2, :] | (b[..., 1::2, :] << 16)


@functools.lru_cache(maxsize=None)
def _fft_constants():
    idx = np.arange(128)
    mf = np.zeros((4, 256, 256))
    mi = np.zeros((4, 256, 256))
    for t, res in enumerate(RESIDUES):
        k = (8 * (idx % 64) + np.repeat(res, 64))[None, :]
        th = 2 * np.pi * ((idx[:, None] * k) % D) / D
        co, si = np.cos(th), np.sin(th)
        if t:
            sg = (-1.0 if t in (1, 2) else 1.0) * np.where(k % 8 == t, 1.0, -1.0)
            mf[t] = np.block([[co, -si], [sg * si, sg * co]])
            mi[t] = mf[t].T * (2.0 / (S * D))
        else:
            m0 = np.concatenate([co[:, :64], -si[:, :64]], axis=1)
            m0[:, 64] = (-1.0) ** idx
            m4 = np.concatenate([-si[:, 64:], co[:, 64:]], axis=1)
            once = np.where(idx % 64 == 0, 1.0, 2.0)
            mf[0, :128, :128], mf[0, :128, 128:] = m0, m4
            mi[0, :128, :128] = (m0 * once).T / (S * D)
            mi[0, :128, 128:] = m4.T * (2.0 / (S * D))
    gf = np.zeros((32, 128, 128))
    gi = np.zeros((32, 128, 128))
    for r in range(32):
        th = 2 * np.pi * ((idx[None, :64] * (32 * idx[:64, None] + r)) % S) / S
        gr, gim = np.cos(th), -np.sin(th)
        g = np.block([[gr, -gim], [gim, gr]])
        gf[r, :, 0::2], gf[r, :, 1::2] = g[:, :64], g[:, 64:]
        gi[r, :, 0::2], gi[r, :, 1::2] = g.T[:, :64], g.T[:, 64:]
    lane, r = idx[:, None], idx[None, :]
    live = (lane < 32) & (r < 32) & (lane // 16 == r % 2)
    th = 2 * np.pi * ((lane % 16) * r % 32) / 32
    fc, fs = np.cos(th) * live, -np.sin(th) * live
    small = np.stack([fc, fs, fc.T, fs.T,
                      (lane % 32 == r) * 1.0])
    th = 2 * np.pi * (idx[:64, None] * idx[None, :] % S) / S
    tw = np.stack([np.cos(th), -np.sin(th)]).astype(np.float32)
    return (_pack_rows(mf), _pack_rows(mi), _pack_rows(small), tw,
            _pack_rows(gf), _pack_rows(gi))


def _bfly8(x):
    x0, x1, x2, x3, x4, x5, x6, x7 = x
    t0, t1, t2, t3 = x0 + x4, x0 - x4, x2 + x6, x2 - x6
    t4, t5, t6, t7 = x1 + x5, x1 - x5, x3 + x7, x3 - x7
    u0, u1, u2, u3 = t0 + t2, t0 - t2, t4 + t6, t4 - t6
    p, q = _SQH * (t5 - t7), _SQH * (t5 + t7)
    return [(u0 + u2, u0 - u2), (t1 + p, t3 + q), (u1, u3), (t1 - p, t3 - q)]


def _bfly8_t(planes):
    (a0, a4), (a1r, a1i), (u1, u3), (a3r, a3i) = planes
    u0, u2 = a0 + a4, a0 - a4
    t1, p, t3, q = a1r + a3r, a1r - a3r, a1i + a3i, a1i - a3i
    t5, t7 = _SQH * (p + q), _SQH * (q - p)
    t0, t2, t4, t6 = u0 + u1, u0 - u1, u2 + u3, u2 - u3
    return [t0 + t1, t4 + t5, t2 + t3, t6 + t7, t0 - t1, t4 - t5, t2 - t3, t6 - t7]


def _dft4(z):
    (ar, ai), (br, bi), (cr, ci), (dr, di) = z
    er, ei, fr, fi = ar + cr, ai + ci, ar - cr, ai - ci
    gr, gi, hr, hi = br + dr, bi + di, br - dr, bi - di
    return [(er + gr, ei + gi), (fr + hi, fi - hr), (er - gr, ei - gi), (fr - hi, fi + hr)]


def _twiddle(z, e):
    re, im = z
    if e == 0:
        return z
    if e == 8:
        return im, -re
    if e == 4:
        return _SQH * (re + im), _SQH * (im - re)
    if e == 12:
        return _SQH * (im - re), -_SQH * (re + im)
    c, s = float(np.cos(np.pi * e / 16)), float(np.sin(np.pi * e / 16))
    return re * c + im * s, im * c - re * s


def _dft16(z):
    cols = [_dft4([z[a + 4 * b] for b in range(4)]) for a in range(4)]
    out = [None] * 16
    for r1 in range(4):
        y = _dft4([_twiddle(cols[a][r1], 2 * a * r1) for a in range(4)])
        for r2 in range(4):
            out[r1 + 4 * r2] = y[r2]
    return out


def _swap(z):
    return [(im, re) for re, im in z]


def _half_dft32(z, odd):
    return _dft16([_twiddle(v, b * odd) for b, v in enumerate(z)])


def _half_idft32(z, odd):
    return _swap([_twiddle(v, b * odd) for b, v in enumerate(_dft16(_swap(z)))])


def _bf(x):
    return pltpu.bitcast(x, BF16)


def _pack(re, im):
    return pltpu.pack_elementwise([re, im], packed_dtype=BF16)


def _low_halves(a, b):
    return (a & jnp.uint32(0xFFFF)) | (b << 16)


def _high_halves(a, b):
    return (a >> 16) | (b & jnp.uint32(0xFFFF0000))


def _dot(a, b):
    return jnp.dot(a, b, preferred_element_type=F32)


def _dot_nt(a, b):
    return lax.dot_general(a, b, (((1,), (1,)), ((), ())), preferred_element_type=F32)


def _softmax(sc):
    e = jnp.exp(sc - jnp.max(sc, axis=-1, keepdims=True))
    l = jnp.sum(e, axis=-1, keepdims=True)
    r = pltpu.reciprocal(l, approx=True)
    return e * (r * (2.0 - l * r))


def _kernel(ax_hbm, wr_hbm, wi_hbm, bx_hbm, mem0_hbm, wq_hbm, wk_hbm, wv_hbm, wo_hbm,
            mf_hbm, mi_hbm, ms_hbm, tw_hbm, gf_hbm, gi_hbm,
            out_hbm,
            xa, wraw, wnyq, wp, mf, mi, ms, tw, gf, gi, ybuf, ubuf, nyq,
            xs, xpre3, xpre, stage, wqkv, wo, pre, kvmem, obuf, opre, part,
            sem, sem_a, sem_w):
    copy = pltpu.make_async_copy
    w_hbm = (wq_hbm, wk_hbm, wv_hbm)
    f_hbm = (wr_hbm, wi_hbm)
    scale = DH ** -0.5

    xpre_copy = copy(bx_hbm.at[:, :, 0], xpre3, sem.at[0])
    mf_copy = copy(mf_hbm, mf, sem.at[1])
    filter_stage_copies = [
        copy(src, dst, sem.at[2])
        for src, dst in ((ms_hbm, ms), (tw_hbm, tw), (mi_hbm, mi), (gf_hbm, gf), (gi_hbm, gi),
                         (wr_hbm.at[pl.ds(D // 2, 1)], wnyq.at[0]),
                         (wi_hbm.at[pl.ds(D // 2, 1)], wnyq.at[1]))]
    step_copies = [
        copy(bx_hbm.at[:, :, pl.ds(1, 3)], xs.at[pl.ds(0, 32), :, pl.ds(1, 3)], sem.at[3]),
        copy(mem0_hbm, xs.at[0, 0, 0], sem.at[3])]
    o_copy = copy(xs.at[pl.ds(0, 32), :, pl.ds(1, 3)],
                  out_hbm.at[:, :, pl.ds(1, 3), :, pl.ds(D, D)], sem.at[4])

    def opre_copy(g):
        return copy(xs.at[pl.ds(8 * g, 8), :, 0],
                    out_hbm.at[pl.ds(8 * g, 8), :, 0, :, pl.ds(D, D)], sem.at[4])

    def y_copy(c):
        return copy(xa.at[c], out_hbm.at[:, c // 4, c % 4, :, pl.ds(0, D)], sem.at[4])

    def wo_copy(n):
        return copy(wo_hbm.bitcast(U32).at[:, pl.ds(pl.multiple_of(n * 128, 128), 128)],
                    wo.at[n], sem.at[3])

    def a_copies(c):
        copies = [copy(ax_hbm.at[:, c], xa.at[c], sem_a.at[c])]
        for kap in (2 * c, 2 * c + 1):
            for i in range(2):
                src = f_hbm[i].at[pl.ds(0, D // 2)].bitcast(U32)
                copies.append(copy(
                    src.at[:, pl.ds(pl.multiple_of(kap * 128, 128), 128)],
                    wraw.at[pl.ds(pl.multiple_of((kap * 2 + i) * 256, 256), 256)],
                    sem_a.at[c]))
        return copies

    def w_copy(mat, pair, slot):
        return copy(w_hbm[mat].bitcast(U32).at[:, pair, :],
                    stage.at[pl.ds(pl.multiple_of(slot * D, D), D)], sem_w.at[slot])

    xpre_copy.start()
    pl.loop(0, NSLOT)(lambda slot: w_copy(0, slot, slot).start())
    mf_copy.start()

    lane = lax.broadcasted_iota(jnp.int32, (8, 128), 1)
    lanes = lax.broadcasted_iota(jnp.int32, (128, 128), 1)

    def a_forward(c, odd):
        row = pl.ds(pl.multiple_of(c * 8, 8), 8)
        lhs = []
        for blk in range(2):
            lo = xa[c, pl.ds(8 * blk, 8)].astype(F32).reshape(64, D)
            hi = xa[c, pl.ds(16 + 8 * blk, 8)].astype(F32).reshape(64, D)
            xh = lo - hi if odd else lo + hi
            planes = _bfly8([xh[:, 128 * i:128 * (i + 1)] for i in range(8)])
            lhs.append([jnp.concatenate(planes[t], axis=1).astype(BF16) for t in range(4)])
            yield
        lhs = [jnp.concatenate([lhs[0][t], lhs[1][t]], axis=0) for t in range(4)]
        x1 = {}

        def butterflies(t):
            v = x1.pop(t)
            y = _half_dft32([(v[8 * b:8 * b + 8, :128], v[8 * b:8 * b + 8, 128:])
                             for b in range(16)], odd)
            for r in range(16):
                ybuf[2 * r + odd, row, 128 * t:128 * (t + 1)] = _pack(*y[r])

        p0 = _dot(lhs[0][:, :128], _bf(mf[0, :64, :128]))
        p4 = _dot(lhs[0][:, 128:], _bf(mf[0, :64, 128:]))
        x1[1] = _dot(lhs[1], _bf(mf[1]))
        low = lanes < 64
        im = pltpu.roll(jnp.where(low, p4, p0), 64, 1)
        x1[0] = jnp.concatenate([jnp.where(low, p0, p4), jnp.where(lanes == 0, 0.0, im)], axis=1)
        acc = nyq[row, :] if odd else jnp.zeros((8, 128), F32)
        for b in range(16):
            k = 16 * odd + b
            v = im[8 * b:8 * b + 8]
            acc = jnp.where(lane == k, pltpu.roll(v, k, 1) if k else v, acc)
        nyq[row, :] = acc
        butterflies(0)
        yield
        x1[2] = _dot(lhs[2], _bf(mf[2]))
        x1[3] = _dot(lhs[3], _bf(mf[3]))
        butterflies(1)
        yield
        butterflies(2)
        yield
        butterflies(3)
        yield

    def a_filter_layout(it, i):
        base = (2 * it + i) * 512
        wr = [wraw[pl.ds(base + j, 64, stride=4), :] for j in range(4)]
        wi = [wraw[pl.ds(base + 256 + j, 64, stride=4), :] for j in range(4)]
        res = [(_low_halves, _high_halves)[k % 2](wr[k // 2], wi[k // 2]) for k in range(8)]
        for t, (lo, hi) in enumerate(RESIDUES):
            tile = jnp.concatenate([res[lo], res[hi]], axis=0).T
            dst = wp.at[pl.ds(pl.multiple_of(t * WP_ROWS + it * 264, 8), 264)]
            for m in range(4):
                dst[pl.ds(33 * (4 * i + m), 32), :] = tile[32 * m:32 * (m + 1)]

    def a_nyquist():
        b = nyq[...].astype(BF16)
        yr, yi = _dot(b, _bf(ms[0])), _dot(b, _bf(ms[1]))
        sub = lax.broadcasted_iota(jnp.int32, (8, 128), 0)
        wn = []
        for i in range(2):
            w = wnyq[i].astype(F32)
            spread = jnp.concatenate(
                [jnp.where(lane // 32 == sub % 4,
                           jnp.where(sub < 4, w[:, 256 * k:256 * k + 128],
                                     w[:, 256 * k + 128:256 * k + 256]), 0.0)
                 for k in range(8)], axis=0)
            wn.append(_dot(spread.astype(BF16), _bf(ms[4])))
        yield
        yield
        tc, ts = tw[0], tw[1]
        x2 = _dot(_bf(gf[0]), _bf(_pack(yr * tc - yi * ts, yr * ts + yi * tc)))
        yield
        yield
        a, b = x2[:64], x2[64:]
        u = _dot(_bf(gi[0]), _bf(_pack(a * wn[0] - b * wn[1], a * wn[1] + b * wn[0])))
        yield
        yield
        ur, ui = u[:64], u[64:]
        nyq[...] = (_dot((ur * tc + ui * ts).astype(BF16), _bf(ms[2]))
                    + _dot((ui * tc - ur * ts).astype(BF16), _bf(ms[3])))

    def a_filter(it, side=()):
        z = {}
        side = iter(side)

        def fwd(i):
            r = 8 * it + i
            x2 = _dot(_bf(gf[r]), _bf(ybuf[r]))
            tiles = []
            for t in range(4):
                w = wp[pl.ds(t * WP_ROWS + r, 64, stride=33), :]
                wr = pltpu.bitcast(w << 16, F32)
                wi = pltpu.bitcast(w & jnp.uint32(0xFFFF0000), F32)
                a, b = x2[:64, 128 * t:128 * (t + 1)], x2[64:, 128 * t:128 * (t + 1)]
                tiles.append(_pack(a * wr - b * wi, a * wi + b * wr))
            z[i] = jnp.concatenate(tiles, axis=1)

        def inv(i):
            r = 8 * it + i
            ubuf[r] = _dot(_bf(gi[r]), _bf(z.pop(i)))

        lag = 2
        for i in range(8 + lag):
            next(side, None)
            if i < 8:
                fwd(i)
            if i >= lag:
                inv(i - lag)

    def a_inverse(c, odd, halves):
        r0 = pl.multiple_of(c * 8, 8)
        planes = []

        def tile(t):
            cols = slice(128 * t, 128 * (t + 1))
            x3 = _half_idft32(
                [(ubuf[2 * r + odd, pl.ds(r0, 8), cols],
                  ubuf[2 * r + odd, pl.ds(64 + r0, 8), cols]) for r in range(16)], odd)
            re, im = [jnp.concatenate([v[p] for v in x3], axis=0) for p in range(2)]
            if t:
                o = _dot(jnp.concatenate([re, im], axis=1).astype(BF16), _bf(mi[t]))
                planes.append((o[:, :128], o[:, 128:]))
                return
            bn = nyq[pl.ds(r0, 8), :]
            bn = jnp.concatenate(
                [pltpu.roll(bn, 64 - 16 * odd - b, 1) for b in range(16)], axis=0)
            low = lanes < 64
            im = pltpu.roll(im, 64, 1)
            q0 = jnp.where(low, re, jnp.where(lanes == 64, bn, im))
            q4 = jnp.where(low, im, re)
            planes.append((_dot(q0.astype(BF16), _bf(mi[0, :64, :128])),
                           _dot(q4.astype(BF16), _bf(mi[0, :64, 128:]))))

        tile(0)
        yield
        tile(1)
        tile(2)
        yield
        tile(3)
        yield
        halves.append(jnp.concatenate(_bfly8_t(planes), axis=1))
        if odd:
            y = jnp.concatenate([halves[0] + halves[1], halves[0] - halves[1]], axis=0)
            xa[c] = y.reshape(32, 8, D).astype(BF16)
        yield

    def project_pair(mat, pair, slot, side):
        ev = stage[pl.ds(slot * D, D // 2, stride=2), :]
        od = stage[pl.ds(slot * D + 1, D // 2, stride=2), :]
        lo, hi = _low_halves(ev, od), _high_halves(ev, od)
        wqkv[6 * pair + mat] = lo
        wqkv[6 * pair + 3 + mat] = hi
        nslice = 1 if side is None else 4
        rows = NPRE // nslice
        for j in range(nslice):
            if side is not None:
                next(side)
            if j:
                lo, hi = wqkv[6 * pair + mat], wqkv[6 * pair + 3 + mat]
            p = _dot(_bf(xpre[rows // 2 * j:rows // 2 * (j + 1), :]),
                     _bf(jnp.concatenate([lo, hi], axis=1))).astype(BF16)
            pre[mat, 2 * pair, rows * j:rows * (j + 1), :] = p[:, :DH]
            pre[mat, 2 * pair + 1, rows * j:rows * (j + 1), :] = p[:, DH:]

    def project_loop(mat, npair, before, side, after):
        @pl.loop(0, 16 // npair)
        def _(it):
            first = npair * it
            slot0 = (16 * mat + first) % NSLOT
            for i in range(npair):
                w_copy(mat, first + i, slot0 + i).wait()
            before(it)
            work = side(it)
            for i in range(npair):
                project_pair(mat, first + i, slot0 + i, work)

            @pl.when(first + NSLOT < 16)
            def _():
                for i in range(npair):
                    w_copy(mat, first + NSLOT + i, slot0 + i).start()

            if mat < 2:
                @pl.when(first + NSLOT >= 16)
                def _():
                    for i in range(npair):
                        w_copy(mat + 1, first + NSLOT - 16 + i, slot0 + i).start()

            after(it)

    def nothing(it):
        return None

    def fetch_a_inputs(it):
        for cp in a_copies(it):
            cp.start()

    def wait_a_inputs(it):
        for cp in a_copies(it):
            cp.wait()

    def forward_fft(it):
        units = [a_forward(it, odd) for odd in range(2)]
        for u in range(2):
            for k in range(4):
                if u and k < 2:
                    next(units[0])
                next(units[u])
                if k == 2:
                    a_filter_layout(it, u)
                if u and k == 3:
                    next(units[u])
                    next(units[u])
                yield

    def fetch_wo(it):
        wo_copy(it).start()

    def inverse_fft(it):
        halves = []
        for odd in range(2):
            yield from a_inverse(it, odd, halves)

    def store_y(it):
        y_copy(it).start()

    xpre_copy.wait()
    xpre[...] = pltpu.bitcast(xpre3[...].reshape(NPRE, D), U32)
    project_loop(0, 2, nothing, nothing, fetch_a_inputs)
    for cp in filter_stage_copies:
        cp.start()
    mf_copy.wait()
    project_loop(1, 2, wait_a_inputs, forward_fft, fetch_wo)
    for cp in step_copies:
        cp.start()
    for cp in filter_stage_copies:
        cp.wait()
    a_filter(0, a_nyquist())
    pl.loop(1, 4)(a_filter)
    project_loop(2, 2, nothing, inverse_fft, store_y)

    for cp in step_copies + [wo_copy(n) for n in range(8)]:
        cp.wait()

    def segment(s, h, split):
        row = lax.broadcasted_iota(jnp.int32, (32, 48), 0)
        col = lax.broadcasted_iota(jnp.int32, (32, 48), 1)
        allowed = ((row < NMEM) | (col >= 32) | (col <= row)) & (col < 40)
        p0 = pl.ds(pl.multiple_of(s * 8, 8), 8)
        zeros = jnp.zeros((8, DH), BF16)
        st = {}

        def half(i, a):
            return _dot(h[:, 512 * a:512 * (a + 1)], _bf(wqkv[i, 256 * a:256 * (a + 1), :]))

        def qkv(hd):
            if hd == 0 and split:
                for i in range(3):
                    part[i] = half(i, 0)
                q, k, v = [(part[i] + half(i, 1)).astype(BF16) for i in range(3)]
            else:
                q, k, v = [_dot(h, _bf(wqkv[3 * hd + i])).astype(BF16) for i in range(3)]
            kvmem[0, hd, p0, :] = k[:NMEM]
            kvmem[1, hd, p0, :] = v[:NMEM]
            st[hd] = (q, k, v)

        def scores(hd):
            q, k, v = st[hd]
            ka = jnp.concatenate([k, pre[1, hd, p0, :], zeros], axis=0)
            sc = jnp.where(allowed, _dot_nt(q, ka) * scale, -jnp.inf)
            st[hd] = (_softmax(sc).astype(BF16), v)

        def context(hd):
            p, v = st.pop(hd)
            va = jnp.concatenate([v, pre[2, hd, p0, :], zeros], axis=0)
            obuf[:, hd * DH:(hd + 1) * DH] = _dot(p, va).astype(BF16)

        acc = [None] * 8

        def project(g):
            lhs = obuf[:, 4 * g * DH:4 * (g + 1) * DH]
            for n in range(8):
                t = _dot(lhs, _bf(wo[n, 256 * g:256 * (g + 1), :]))
                acc[n] = t if acc[n] is None else acc[n] + t

        lag_scores, lag_context = 1, 3
        for hd in range(H):
            qkv(hd)
            if hd >= lag_scores:
                scores(hd - lag_scores)
            if hd >= lag_context:
                context(hd - lag_context)
            if hd == 28:
                project(0)
        for t, g in enumerate(range(1, H // 4)):
            project(g)
            if t < lag_scores:
                scores(H + t - lag_scores)
            if t < lag_context:
                context(H + t - lag_context)
        return acc

    @pl.loop(0, NSEG // 4)
    def _(i):
        h = xs[2 * i, 0].reshape(32, D)
        for u in range(4):
            acc = segment(4 * i + u, h, u > 0)
            if u < 3:
                xt = xs[2 * i + (u + 1) // 2, (u + 1) % 2, pl.ds(1, 3)].astype(F32).reshape(24, D)
                h = jnp.concatenate(
                    [jnp.concatenate([acc[n][:NMEM], xt[:, 128 * n:128 * (n + 1)]],
                                     axis=0).astype(BF16) for n in range(8)], axis=1)
            ob = jnp.concatenate(acc, axis=1).astype(BF16).reshape(4, 8, D)
            xs[2 * i + u // 2, u % 2, pl.ds(1, 3)] = ob[1:]
        xs[2 * i + 2, 0, 0] = ob[0]

    o_copy.start()

    @pl.loop(0, 4)
    def _(g):
        row = lax.broadcasted_iota(jnp.int32, (64, 128), 0)
        col = lax.broadcasted_iota(jnp.int32, (64, 128), 1)
        allowed = ((col % 64) // 8 == row // 8) & ((col < 64) | (col % 8 <= row % 8))
        st = {}

        def rows(a):
            return pl.ds(pl.multiple_of(g * 128 + a * 64, 64), 64)

        def scores(hd):
            for a in range(2):
                ka = jnp.concatenate([kvmem[0, hd, rows(a), :], pre[1, hd, rows(a), :]], axis=0)
                sc = jnp.where(allowed, _dot_nt(pre[0, hd, rows(a), :], ka) * scale, -jnp.inf)
                st[hd, a] = _softmax(sc).astype(BF16)

        def context(hd):
            for a in range(2):
                va = jnp.concatenate([kvmem[1, hd, rows(a), :], pre[2, hd, rows(a), :]], axis=0)
                opre[a * 64:(a + 1) * 64, hd * DH:(hd + 1) * DH] = (
                    _dot(st.pop((hd, a)), va).astype(BF16))

        acc = None
        for c in range(H // 8 + 2):
            if c < H // 8:
                for hd in range(8 * c, 8 * c + 8):
                    scores(hd)
            if c >= 2:
                lhs = opre[:, 8 * (c - 2) * DH:8 * (c - 1) * DH]
                t = jnp.concatenate([_dot(lhs, _bf(wo[n, 512 * (c - 2):512 * (c - 1), :]))
                                     for n in range(8)], axis=1)
                acc = t if acc is None else acc + t
            if 1 <= c <= H // 8:
                for hd in range(8 * (c - 1), 8 * c):
                    context(hd)
        xs[pl.ds(g * 8, 8), :, 0] = acc.astype(BF16).reshape(8, 2, 8, D)
        opre_copy(g).start()

    for cp in [y_copy(c) for c in range(8)] + [o_copy] + [opre_copy(g) for g in range(4)]:
        cp.wait()


@functools.partial(jax.jit, static_argnames=("B_seg_len",))
def pallas_concat_heads__spectral_gfnet__memory_aug_recurrent_mem_tr__prompt_kernel(
    A_x, A_w_r, A_w_i, B_x, B_mem0, B_Wq, B_Wk, B_Wv, B_Wo, B_seg_len=SEG,
):
    assert A_x.shape == (1, S, D) and B_x.shape == (1, S, D)
    assert A_w_r.shape == A_w_i.shape == (S, D // 2 + 1)
    assert B_mem0.shape == (1, NMEM, D) and B_seg_len == SEG
    assert B_Wq.shape == B_Wk.shape == B_Wv.shape == (D, H, DH) and B_Wo.shape == (H, DH, D)

    vmem = pltpu.VMEM
    dma = pltpu.SemaphoreType.DMA
    scratch = [
        vmem((8, 32, 8, D), BF16),
        vmem((32 * 256 + 32, 128), U32),
        vmem((2, 1, S), BF16),
        vmem((4 * WP_ROWS + 32, 128), U32),
        vmem((4, 128, 256), U32),
        vmem((4, 128, 256), U32),
        vmem((5, 64, 128), U32),
        vmem((2, 64, 128), F32),
        vmem((32, 64, 128), U32),
        vmem((32, 64, 128), U32),
        vmem((32, 64, 512), U32),
        vmem((32, 128, 512), F32),
        vmem((64, 128), F32),
        vmem((33, 2, 4, 8, D), BF16),
        vmem((32, 2, 8, D), BF16),
        vmem((NPRE // 2, D), U32),
        vmem((NSLOT * D + 32, 128), U32),
        vmem((3 * H, D // 2, DH), U32),
        vmem((8, H * DH // 2, 128), U32),
        vmem((3, H, NPRE, DH), BF16),
        vmem((2, H, NPRE, DH), BF16),
        vmem((32, H * DH), BF16),
        vmem((128, H * DH), BF16),
        vmem((3, 32, DH), F32),
        dma((5,)), dma((8,)), dma((NSLOT,)),
    ]
    hbm = pl.BlockSpec(memory_space=pltpu.HBM)
    out = pl.pallas_call(
        _kernel,
        out_shape=jax.ShapeDtypeStruct((32, 2, 4, 8, 2 * D), BF16),
        in_specs=[hbm] * 15,
        out_specs=hbm,
        scratch_shapes=scratch,
        compiler_params=pltpu.CompilerParams(vmem_limit_bytes=124 * 1024 * 1024),
    )(A_x.reshape(32, 8, 8, D), A_w_r.T, A_w_i.T,
      B_x.reshape(32, 2, 4, 8, D), B_mem0.reshape(NMEM, D),
      B_Wq, B_Wk, B_Wv, B_Wo.reshape(H * DH, D),
      *[jnp.asarray(c) for c in _fft_constants()])
    return out.reshape(1, S, 2 * D)
```

```python
import functools

import numpy as np
import jax
import jax.numpy as jnp
from jax import lax
import jax.experimental.pallas as pl
import jax.experimental.pallas.tpu as pltpu

S, D = 2048, 1024
H, DH = 32, 128
NMEM, SEG = 8, 32
NSEG = S // SEG
NPRE = NSEG * 8
NSLOT = 12
WP_ROWS = 33 * 64
RESIDUES = ((0, 4), (1, 7), (2, 6), (3, 5))

F32, BF16, U32 = jnp.float32, jnp.bfloat16, jnp.uint32
_SQH = float(np.sqrt(0.5))


def _pack_rows(m):
    b = np.asarray(m, np.float32).astype(jnp.bfloat16).view(np.uint16).astype(np.uint32)
    return b[..., 0::2, :] | (b[..., 1::2, :] << 16)


@functools.lru_cache(maxsize=None)
def _fft_constants():
    idx = np.arange(128)
    mf = np.zeros((4, 256, 256))
    mi = np.zeros((4, 256, 256))
    for t, res in enumerate(RESIDUES):
        k = (8 * (idx % 64) + np.repeat(res, 64))[None, :]
        th = 2 * np.pi * ((idx[:, None] * k) % D) / D
        co, si = np.cos(th), np.sin(th)
        if t:
            sg = (-1.0 if t in (1, 2) else 1.0) * np.where(k % 8 == t, 1.0, -1.0)
            mf[t] = np.block([[co, -si], [sg * si, sg * co]])
            mi[t] = mf[t].T * (2.0 / (S * D))
        else:
            m0 = np.concatenate([co[:, :64], -si[:, :64]], axis=1)
            m0[:, 64] = (-1.0) ** idx
            m4 = np.concatenate([-si[:, 64:], co[:, 64:]], axis=1)
            once = np.where(idx % 64 == 0, 1.0, 2.0)
            mf[0, :128, :128], mf[0, :128, 128:] = m0, m4
            mi[0, :128, :128] = (m0 * once).T / (S * D)
            mi[0, :128, 128:] = m4.T * (2.0 / (S * D))
    gf = np.zeros((32, 128, 128))
    gi = np.zeros((32, 128, 128))
    for r in range(32):
        th = 2 * np.pi * ((idx[None, :64] * (32 * idx[:64, None] + r)) % S) / S
        gr, gim = np.cos(th), -np.sin(th)
        g = np.block([[gr, -gim], [gim, gr]])
        gf[r, :, 0::2], gf[r, :, 1::2] = g[:, :64], g[:, 64:]
        gi[r, :, 0::2], gi[r, :, 1::2] = g.T[:, :64], g.T[:, 64:]
    lane, r = idx[:, None], idx[None, :]
    live = (lane < 32) & (r < 32) & (lane // 16 == r % 2)
    th = 2 * np.pi * ((lane % 16) * r % 32) / 32
    fc, fs = np.cos(th) * live, -np.sin(th) * live
    small = np.stack([fc, fs, fc.T, fs.T,
                      (lane % 32 == r) * 1.0])
    th = 2 * np.pi * (idx[:64, None] * idx[None, :] % S) / S
    tw = np.stack([np.cos(th), -np.sin(th)]).astype(np.float32)
    return (_pack_rows(mf), _pack_rows(mi), _pack_rows(small), tw,
            _pack_rows(gf), _pack_rows(gi))


def _bfly8(x):
    x0, x1, x2, x3, x4, x5, x6, x7 = x
    t0, t1, t2, t3 = x0 + x4, x0 - x4, x2 + x6, x2 - x6
    t4, t5, t6, t7 = x1 + x5, x1 - x5, x3 + x7, x3 - x7
    u0, u1, u2, u3 = t0 + t2, t0 - t2, t4 + t6, t4 - t6
    p, q = _SQH * (t5 - t7), _SQH * (t5 + t7)
    return [(u0 + u2, u0 - u2), (t1 + p, t3 + q), (u1, u3), (t1 - p, t3 - q)]


def _bfly8_t(planes):
    (a0, a4), (a1r, a1i), (u1, u3), (a3r, a3i) = planes
    u0, u2 = a0 + a4, a0 - a4
    t1, p, t3, q = a1r + a3r, a1r - a3r, a1i + a3i, a1i - a3i
    t5, t7 = _SQH * (p + q), _SQH * (q - p)
    t0, t2, t4, t6 = u0 + u1, u0 - u1, u2 + u3, u2 - u3
    return [t0 + t1, t4 + t5, t2 + t3, t6 + t7, t0 - t1, t4 - t5, t2 - t3, t6 - t7]


def _dft4(z):
    (ar, ai), (br, bi), (cr, ci), (dr, di) = z
    er, ei, fr, fi = ar + cr, ai + ci, ar - cr, ai - ci
    gr, gi, hr, hi = br + dr, bi + di, br - dr, bi - di
    return [(er + gr, ei + gi), (fr + hi, fi - hr), (er - gr, ei - gi), (fr - hi, fi + hr)]


def _twiddle(z, e):
    re, im = z
    if e == 0:
        return z
    if e == 8:
        return im, -re
    if e == 4:
        return _SQH * (re + im), _SQH * (im - re)
    if e == 12:
        return _SQH * (im - re), -_SQH * (re + im)
    c, s = float(np.cos(np.pi * e / 16)), float(np.sin(np.pi * e / 16))
    return re * c + im * s, im * c - re * s


def _dft16(z):
    cols = [_dft4([z[a + 4 * b] for b in range(4)]) for a in range(4)]
    out = [None] * 16
    for r1 in range(4):
        y = _dft4([_twiddle(cols[a][r1], 2 * a * r1) for a in range(4)])
        for r2 in range(4):
            out[r1 + 4 * r2] = y[r2]
    return out


def _swap(z):
    return [(im, re) for re, im in z]


def _half_dft32(z, odd):
    return _dft16([_twiddle(v, b * odd) for b, v in enumerate(z)])


def _half_idft32(z, odd):
    return _swap([_twiddle(v, b * odd) for b, v in enumerate(_dft16(_swap(z)))])


def _bf(x):
    return pltpu.bitcast(x, BF16)


def _pack(re, im):
    return pltpu.pack_elementwise([re, im], packed_dtype=BF16)


def _low_halves(a, b):
    return (a & jnp.uint32(0xFFFF)) | (b << 16)


def _high_halves(a, b):
    return (a >> 16) | (b & jnp.uint32(0xFFFF0000))


def _dot(a, b):
    return jnp.dot(a, b, preferred_element_type=F32)


def _dot_nt(a, b):
    return lax.dot_general(a, b, (((1,), (1,)), ((), ())), preferred_element_type=F32)


def _softmax(sc):
    e = jnp.exp(sc - jnp.max(sc, axis=-1, keepdims=True))
    l = jnp.sum(e, axis=-1, keepdims=True)
    r = pltpu.reciprocal(l, approx=True)
    return e * (r * (2.0 - l * r))


def _kernel(ax_hbm, wr_hbm, wi_hbm, bx_hbm, mem0_hbm, wq_hbm, wk_hbm, wv_hbm, wo_hbm,
            mf_hbm, mi_hbm, ms_hbm, tw_hbm, gf_hbm, gi_hbm,
            out_hbm,
            xa, wraw, wnyq, wp, mf, mi, ms, tw, gf, gi, ybuf, ubuf, nyq,
            xs, xpre3, xpre, stage, wqkv, wo, pre, kvmem, obuf, opre, part,
            sem, sem_a, sem_w):
    copy = pltpu.make_async_copy
    w_hbm = (wq_hbm, wk_hbm, wv_hbm)
    f_hbm = (wr_hbm, wi_hbm)
    scale = DH ** -0.5

    def xpre_copy(j):
        return copy(bx_hbm.at[pl.ds(8 * j, 8), :, 0], xpre3.at[pl.ds(8 * j, 8)], sem_a.at[8 + j])

    mf_copy = copy(mf_hbm, mf, sem.at[1])
    filter_stage_copies = [
        copy(src, dst, sem.at[2])
        for src, dst in ((ms_hbm, ms), (tw_hbm, tw), (mi_hbm, mi), (gf_hbm, gf), (gi_hbm, gi),
                         (wr_hbm.at[pl.ds(D // 2, 1)], wnyq.at[0]),
                         (wi_hbm.at[pl.ds(D // 2, 1)], wnyq.at[1]))]
    step_copies = [
        copy(bx_hbm.at[:, :, pl.ds(1, 3)], xs.at[pl.ds(0, 32), :, pl.ds(1, 3)], sem.at[3]),
        copy(mem0_hbm, xs.at[0, 0, 0], sem.at[3])]
    o_copy = copy(xs.at[pl.ds(0, 32), :, pl.ds(1, 3)],
                  out_hbm.at[:, :, pl.ds(1, 3), :, pl.ds(D, D)], sem.at[4])

    def opre_copy(g):
        return copy(xs.at[pl.ds(8 * g, 8), :, 0],
                    out_hbm.at[pl.ds(8 * g, 8), :, 0, :, pl.ds(D, D)], sem.at[4])

    def y_copy(c):
        return copy(xa.at[c], out_hbm.at[:, c // 4, c % 4, :, pl.ds(0, D)], sem.at[4])

    def wo_copy(n):
        return copy(wo_hbm.bitcast(U32).at[:, pl.ds(pl.multiple_of(n * 128, 128), 128)],
                    wo.at[n], sem.at[3])

    def a_copies(c):
        copies = [copy(ax_hbm.at[:, c], xa.at[c], sem_a.at[c])]
        for kap in (2 * c, 2 * c + 1):
            for i in range(2):
                src = f_hbm[i].at[pl.ds(0, D // 2)].bitcast(U32)
                copies.append(copy(
                    src.at[:, pl.ds(pl.multiple_of(kap * 128, 128), 128)],
                    wraw.at[pl.ds(pl.multiple_of((kap * 2 + i) * 256, 256), 256)],
                    sem_a.at[c]))
        return copies

    def w_copy(mat, pair, slot):
        return copy(w_hbm[mat].bitcast(U32).at[:, pair, :],
                    stage.at[pl.ds(pl.multiple_of(slot * D, D), D)], sem_w.at[slot])

    pl.loop(0, 2)(lambda slot: w_copy(0, slot, slot).start())
    pl.loop(0, 4)(lambda j: xpre_copy(j).start())
    pl.loop(2, NSLOT)(lambda slot: w_copy(0, slot, slot).start())
    mf_copy.start()

    lane = lax.broadcasted_iota(jnp.int32, (8, 128), 1)
    lanes = lax.broadcasted_iota(jnp.int32, (128, 128), 1)

    def a_forward(c, odd):
        row = pl.ds(pl.multiple_of(c * 8, 8), 8)
        lhs = []
        for blk in range(2):
            lo = xa[c, pl.ds(8 * blk, 8)].astype(F32).reshape(64, D)
            hi = xa[c, pl.ds(16 + 8 * blk, 8)].astype(F32).reshape(64, D)
            xh = lo - hi if odd else lo + hi
            planes = _bfly8([xh[:, 128 * i:128 * (i + 1)] for i in range(8)])
            lhs.append([jnp.concatenate(planes[t], axis=1).astype(BF16) for t in range(4)])
            yield
        lhs = [jnp.concatenate([lhs[0][t], lhs[1][t]], axis=0) for t in range(4)]
        x1 = {}

        def butterflies(t):
            v = x1.pop(t)
            y = _half_dft32([(v[8 * b:8 * b + 8, :128], v[8 * b:8 * b + 8, 128:])
                             for b in range(16)], odd)
            for r in range(16):
                ybuf[2 * r + odd, row, 128 * t:128 * (t + 1)] = _pack(*y[r])

        p0 = _dot(lhs[0][:, :128], _bf(mf[0, :64, :128]))
        p4 = _dot(lhs[0][:, 128:], _bf(mf[0, :64, 128:]))
        x1[1] = _dot(lhs[1], _bf(mf[1]))
        low = lanes < 64
        im = pltpu.roll(jnp.where(low, p4, p0), 64, 1)
        x1[0] = jnp.concatenate([jnp.where(low, p0, p4), jnp.where(lanes == 0, 0.0, im)], axis=1)
        acc = nyq[row, :] if odd else jnp.zeros((8, 128), F32)
        for b in range(16):
            k = 16 * odd + b
            v = im[8 * b:8 * b + 8]
            acc = jnp.where(lane == k, pltpu.roll(v, k, 1) if k else v, acc)
        nyq[row, :] = acc
        butterflies(0)
        yield
        x1[2] = _dot(lhs[2], _bf(mf[2]))
        x1[3] = _dot(lhs[3], _bf(mf[3]))
        butterflies(1)
        yield
        butterflies(2)
        yield
        butterflies(3)
        yield

    def a_filter_layout(it, i):
        base = (2 * it + i) * 512
        wr = [wraw[pl.ds(base + j, 64, stride=4), :] for j in range(4)]
        wi = [wraw[pl.ds(base + 256 + j, 64, stride=4), :] for j in range(4)]
        res = [(_low_halves, _high_halves)[k % 2](wr[k // 2], wi[k // 2]) for k in range(8)]
        for t, (lo, hi) in enumerate(RESIDUES):
            tile = jnp.concatenate([res[lo], res[hi]], axis=0).T
            dst = wp.at[pl.ds(pl.multiple_of(t * WP_ROWS + it * 264, 8), 264)]
            for m in range(4):
                dst[pl.ds(33 * (4 * i + m), 32), :] = tile[32 * m:32 * (m + 1)]

    def a_nyquist():
        b = nyq[...].astype(BF16)
        yr, yi = _dot(b, _bf(ms[0])), _dot(b, _bf(ms[1]))
        sub = lax.broadcasted_iota(jnp.int32, (8, 128), 0)
        wn = []
        for i in range(2):
            w = wnyq[i].astype(F32)
            spread = jnp.concatenate(
                [jnp.where(lane // 32 == sub % 4,
                           jnp.where(sub < 4, w[:, 256 * k:256 * k + 128],
                                     w[:, 256 * k + 128:256 * k + 256]), 0.0)
                 for k in range(8)], axis=0)
            wn.append(_dot(spread.astype(BF16), _bf(ms[4])))
        yield
        yield
        tc, ts = tw[0], tw[1]
        x2 = _dot(_bf(gf[0]), _bf(_pack(yr * tc - yi * ts, yr * ts + yi * tc)))
        yield
        yield
        a, b = x2[:64], x2[64:]
        u = _dot(_bf(gi[0]), _bf(_pack(a * wn[0] - b * wn[1], a * wn[1] + b * wn[0])))
        yield
        yield
        ur, ui = u[:64], u[64:]
        nyq[...] = (_dot((ur * tc + ui * ts).astype(BF16), _bf(ms[2]))
                    + _dot((ui * tc - ur * ts).astype(BF16), _bf(ms[3])))

    def a_filter(it, side=()):
        z = {}
        side = iter(side)

        def fwd(i):
            r = 8 * it + i
            x2 = _dot(_bf(gf[r]), _bf(ybuf[r]))
            tiles = []
            for t in range(4):
                w = wp[pl.ds(t * WP_ROWS + r, 64, stride=33), :]
                wr = pltpu.bitcast(w << 16, F32)
                wi = pltpu.bitcast(w & jnp.uint32(0xFFFF0000), F32)
                a, b = x2[:64, 128 * t:128 * (t + 1)], x2[64:, 128 * t:128 * (t + 1)]
                tiles.append(_pack(a * wr - b * wi, a * wi + b * wr))
            z[i] = jnp.concatenate(tiles, axis=1)

        def inv(i):
            r = 8 * it + i
            ubuf[r] = _dot(_bf(gi[r]), _bf(z.pop(i)))

        lag = 2
        for i in range(8 + lag):
            next(side, None)
            if i < 8:
                fwd(i)
            if i >= lag:
                inv(i - lag)

    def a_inverse(c, odd, halves):
        r0 = pl.multiple_of(c * 8, 8)
        planes = []

        def tile(t):
            cols = slice(128 * t, 128 * (t + 1))
            x3 = _half_idft32(
                [(ubuf[2 * r + odd, pl.ds(r0, 8), cols],
                  ubuf[2 * r + odd, pl.ds(64 + r0, 8), cols]) for r in range(16)], odd)
            re, im = [jnp.concatenate([v[p] for v in x3], axis=0) for p in range(2)]
            if t:
                o = _dot(jnp.concatenate([re, im], axis=1).astype(BF16), _bf(mi[t]))
                planes.append((o[:, :128], o[:, 128:]))
                return
            bn = nyq[pl.ds(r0, 8), :]
            bn = jnp.concatenate(
                [pltpu.roll(bn, 64 - 16 * odd - b, 1) for b in range(16)], axis=0)
            low = lanes < 64
            im = pltpu.roll(im, 64, 1)
            q0 = jnp.where(low, re, jnp.where(lanes == 64, bn, im))
            q4 = jnp.where(low, im, re)
            planes.append((_dot(q0.astype(BF16), _bf(mi[0, :64, :128])),
                           _dot(q4.astype(BF16), _bf(mi[0, :64, 128:]))))

        tile(0)
        yield
        tile(1)
        tile(2)
        yield
        tile(3)
        yield
        halves.append(jnp.concatenate(_bfly8_t(planes), axis=1))
        if odd:
            y = jnp.concatenate([halves[0] + halves[1], halves[0] - halves[1]], axis=0)
            xa[c] = y.reshape(32, 8, D).astype(BF16)
        yield

    def regroup_pair(mat, pair, slot):
        ev = stage[pl.ds(slot * D, D // 2, stride=2), :]
        od = stage[pl.ds(slot * D + 1, D // 2, stride=2), :]
        lo, hi = _low_halves(ev, od), _high_halves(ev, od)
        wqkv[6 * pair + mat] = lo
        wqkv[6 * pair + 3 + mat] = hi
        return lo, hi

    def project_pair(mat, pair, slot, side):
        lo, hi = regroup_pair(mat, pair, slot)
        nslice = 1 if side is None else 4
        rows = NPRE // nslice
        for j in range(nslice):
            if side is not None:
                next(side)
            if j:
                lo, hi = wqkv[6 * pair + mat], wqkv[6 * pair + 3 + mat]
            p = _dot(_bf(xpre[rows // 2 * j:rows // 2 * (j + 1), :]),
                     _bf(jnp.concatenate([lo, hi], axis=1))).astype(BF16)
            pre[mat, 2 * pair, rows * j:rows * (j + 1), :] = p[:, :DH]
            pre[mat, 2 * pair + 1, rows * j:rows * (j + 1), :] = p[:, DH:]

    def project_loop(mat, npair, before, side, after, start=0):
        @pl.loop(start, 16 // npair)
        def _(it):
            first = npair * it
            slot0 = (16 * mat + first) % NSLOT
            for i in range(npair):
                w_copy(mat, first + i, slot0 + i).wait()
            before(it)
            work = side(it)
            for i in range(npair):
                project_pair(mat, first + i, slot0 + i, work)

            @pl.when(first + NSLOT < 16)
            def _():
                for i in range(npair):
                    w_copy(mat, first + NSLOT + i, slot0 + i).start()

            if mat < 2:
                @pl.when(first + NSLOT >= 16)
                def _():
                    for i in range(npair):
                        w_copy(mat + 1, first + NSLOT - 16 + i, slot0 + i).start()

            after(it)

    def nothing(it):
        return None

    def fetch_a_inputs(it):
        for cp in a_copies(it):
            cp.start()

    def wait_a_inputs(it):
        for cp in a_copies(it):
            cp.wait()

    def forward_fft(it):
        units = [a_forward(it, odd) for odd in range(2)]
        for u in range(2):
            for k in range(4):
                if u and k < 2:
                    next(units[0])
                next(units[u])
                if k == 2:
                    a_filter_layout(it, u)
                if u and k == 3:
                    next(units[u])
                    next(units[u])
                yield

    def fetch_wo(it):
        wo_copy(it).start()

    def inverse_fft(it):
        halves = []
        for odd in range(2):
            yield from a_inverse(it, odd, halves)

    def store_y(it):
        y_copy(it).start()

    for i in range(2):
        w_copy(0, i, i).wait()
        regroup_pair(0, i, i)
        w_copy(0, NSLOT + i, i).start()
    fetch_a_inputs(0)

    @pl.loop(0, 4)
    def _(j):
        xpre_copy(j).wait()
        x = xpre3[pl.ds(8 * j, 8)].reshape(128, D)
        xpre[pl.ds(pl.multiple_of(j * 64, 64), 64), :] = pltpu.bitcast(x, U32)
        w = jnp.concatenate([wqkv[3 * hd] for hd in range(4)], axis=1)
        p = _dot(x, _bf(w)).astype(BF16)
        for hd in range(4):
            pre[0, hd, pl.ds(pl.multiple_of(j * 128, 128), 128), :] = p[:, DH * hd:DH * (hd + 1)]

    project_loop(0, 2, nothing, nothing, fetch_a_inputs, start=1)
    for cp in filter_stage_copies:
        cp.start()
    mf_copy.wait()
    project_loop(1, 2, wait_a_inputs, forward_fft, fetch_wo)
    for cp in step_copies:
        cp.start()
    for cp in filter_stage_copies:
        cp.wait()
    a_filter(0, a_nyquist())
    pl.loop(1, 4)(a_filter)
    project_loop(2, 2, nothing, inverse_fft, store_y)

    for cp in step_copies + [wo_copy(n) for n in range(8)]:
        cp.wait()

    def segment(s, h, split):
        row = lax.broadcasted_iota(jnp.int32, (32, 48), 0)
        col = lax.broadcasted_iota(jnp.int32, (32, 48), 1)
        allowed = ((row < NMEM) | (col >= 32) | (col <= row)) & (col < 40)
        p0 = pl.ds(pl.multiple_of(s * 8, 8), 8)
        zeros = jnp.zeros((8, DH), BF16)
        st = {}

        def half(i, a):
            return _dot(h[:, 512 * a:512 * (a + 1)], _bf(wqkv[i, 256 * a:256 * (a + 1), :]))

        def qkv(hd):
            if hd == 0 and split:
                for i in range(3):
                    part[i] = half(i, 0)
                q, k, v = [(part[i] + half(i, 1)).astype(BF16) for i in range(3)]
            else:
                q, k, v = [_dot(h, _bf(wqkv[3 * hd + i])).astype(BF16) for i in range(3)]
            kvmem[0, hd, p0, :] = k[:NMEM]
            kvmem[1, hd, p0, :] = v[:NMEM]
            st[hd] = (q, k, v)

        def scores(hd):
            q, k, v = st[hd]
            ka = jnp.concatenate([k, pre[1, hd, p0, :], zeros], axis=0)
            sc = jnp.where(allowed, _dot_nt(q, ka) * scale, -jnp.inf)
            st[hd] = (_softmax(sc).astype(BF16), v)

        def context(hd):
            p, v = st.pop(hd)
            va = jnp.concatenate([v, pre[2, hd, p0, :], zeros], axis=0)
            obuf[:, hd * DH:(hd + 1) * DH] = _dot(p, va).astype(BF16)

        acc = [None] * 8

        def project(g):
            lhs = obuf[:, 4 * g * DH:4 * (g + 1) * DH]
            for n in range(8):
                t = _dot(lhs, _bf(wo[n, 256 * g:256 * (g + 1), :]))
                acc[n] = t if acc[n] is None else acc[n] + t

        lag_scores, lag_context = 1, 3
        for hd in range(H):
            qkv(hd)
            if hd >= lag_scores:
                scores(hd - lag_scores)
            if hd >= lag_context:
                context(hd - lag_context)
            if hd == 28:
                project(0)
        for t, g in enumerate(range(1, H // 4)):
            project(g)
            if t < lag_scores:
                scores(H + t - lag_scores)
            if t < lag_context:
                context(H + t - lag_context)
        return acc

    @pl.loop(0, NSEG // 4)
    def _(i):
        h = xs[2 * i, 0].reshape(32, D)
        for u in range(4):
            acc = segment(4 * i + u, h, u > 0)
            if u < 3:
                xt = xs[2 * i + (u + 1) // 2, (u + 1) % 2, pl.ds(1, 3)].astype(F32).reshape(24, D)
                h = jnp.concatenate(
                    [jnp.concatenate([acc[n][:NMEM], xt[:, 128 * n:128 * (n + 1)]],
                                     axis=0).astype(BF16) for n in range(8)], axis=1)
            ob = jnp.concatenate(acc, axis=1).astype(BF16).reshape(4, 8, D)
            xs[2 * i + u // 2, u % 2, pl.ds(1, 3)] = ob[1:]
        xs[2 * i + 2, 0, 0] = ob[0]

    o_copy.start()

    @pl.loop(0, 4)
    def _(g):
        row = lax.broadcasted_iota(jnp.int32, (64, 128), 0)
        col = lax.broadcasted_iota(jnp.int32, (64, 128), 1)
        allowed = ((col % 64) // 8 == row // 8) & ((col < 64) | (col % 8 <= row % 8))
        st = {}

        def rows(a):
            return pl.ds(pl.multiple_of(g * 128 + a * 64, 64), 64)

        def scores(hd):
            for a in range(2):
                ka = jnp.concatenate([kvmem[0, hd, rows(a), :], pre[1, hd, rows(a), :]], axis=0)
                sc = jnp.where(allowed, _dot_nt(pre[0, hd, rows(a), :], ka) * scale, -jnp.inf)
                st[hd, a] = _softmax(sc).astype(BF16)

        def context(hd):
            for a in range(2):
                va = jnp.concatenate([kvmem[1, hd, rows(a), :], pre[2, hd, rows(a), :]], axis=0)
                opre[a * 64:(a + 1) * 64, hd * DH:(hd + 1) * DH] = (
                    _dot(st.pop((hd, a)), va).astype(BF16))

        acc = None
        for c in range(H // 8 + 2):
            if c < H // 8:
                for hd in range(8 * c, 8 * c + 8):
                    scores(hd)
            if c >= 2:
                lhs = opre[:, 8 * (c - 2) * DH:8 * (c - 1) * DH]
                t = jnp.concatenate([_dot(lhs, _bf(wo[n, 512 * (c - 2):512 * (c - 1), :]))
                                     for n in range(8)], axis=1)
                acc = t if acc is None else acc + t
            if 1 <= c <= H // 8:
                for hd in range(8 * (c - 1), 8 * c):
                    context(hd)
        xs[pl.ds(g * 8, 8), :, 0] = acc.astype(BF16).reshape(8, 2, 8, D)
        opre_copy(g).start()

    for cp in [y_copy(c) for c in range(8)] + [o_copy] + [opre_copy(g) for g in range(4)]:
        cp.wait()


@functools.partial(jax.jit, static_argnames=("B_seg_len",))
def pallas_concat_heads__spectral_gfnet__memory_aug_recurrent_mem_tr__prompt_kernel(
    A_x, A_w_r, A_w_i, B_x, B_mem0, B_Wq, B_Wk, B_Wv, B_Wo, B_seg_len=SEG,
):
    assert A_x.shape == (1, S, D) and B_x.shape == (1, S, D)
    assert A_w_r.shape == A_w_i.shape == (S, D // 2 + 1)
    assert B_mem0.shape == (1, NMEM, D) and B_seg_len == SEG
    assert B_Wq.shape == B_Wk.shape == B_Wv.shape == (D, H, DH) and B_Wo.shape == (H, DH, D)

    vmem = pltpu.VMEM
    dma = pltpu.SemaphoreType.DMA
    scratch = [
        vmem((8, 32, 8, D), BF16),
        vmem((32 * 256 + 32, 128), U32),
        vmem((2, 1, S), BF16),
        vmem((4 * WP_ROWS + 32, 128), U32),
        vmem((4, 128, 256), U32),
        vmem((4, 128, 256), U32),
        vmem((5, 64, 128), U32),
        vmem((2, 64, 128), F32),
        vmem((32, 64, 128), U32),
        vmem((32, 64, 128), U32),
        vmem((32, 64, 512), U32),
        vmem((32, 128, 512), F32),
        vmem((64, 128), F32),
        vmem((33, 2, 4, 8, D), BF16),
        vmem((32, 2, 8, D), BF16),
        vmem((NPRE // 2, D), U32),
        vmem((NSLOT * D + 32, 128), U32),
        vmem((3 * H, D // 2, DH), U32),
        vmem((8, H * DH // 2, 128), U32),
        vmem((3, H, NPRE, DH), BF16),
        vmem((2, H, NPRE, DH), BF16),
        vmem((32, H * DH), BF16),
        vmem((128, H * DH), BF16),
        vmem((3, 32, DH), F32),
        dma((5,)), dma((12,)), dma((NSLOT,)),
    ]
    hbm = pl.BlockSpec(memory_space=pltpu.HBM)
    out = pl.pallas_call(
        _kernel,
        out_shape=jax.ShapeDtypeStruct((32, 2, 4, 8, 2 * D), BF16),
        in_specs=[hbm] * 15,
        out_specs=hbm,
        scratch_shapes=scratch,
        compiler_params=pltpu.CompilerParams(vmem_limit_bytes=124 * 1024 * 1024),
    )(A_x.reshape(32, 8, 8, D), A_w_r.T, A_w_i.T,
      B_x.reshape(32, 2, 4, 8, D), B_mem0.reshape(NMEM, D),
      B_Wq, B_Wk, B_Wv, B_Wo.reshape(H * DH, D),
      *[jnp.asarray(c) for c in _fft_constants()])
    return out.reshape(1, S, 2 * D)
```

```python
import functools

import numpy as np
import jax
import jax.numpy as jnp
from jax import lax
import jax.experimental.pallas as pl
import jax.experimental.pallas.tpu as pltpu

S, D = 2048, 1024
H, DH = 32, 128
NMEM, SEG = 8, 32
NSEG = S // SEG
NPRE = NSEG * 8
NSLOT = 12
WP_ROWS = 33 * 64
RESIDUES = ((0, 8, 4, 12), (1, 15, 9, 7), (2, 14, 10, 6), (3, 13, 11, 5))

FORWARD_SLOTS = ("0r0", "0r1", "0t0 0b0", "0t1 0b1 1r0", "0t2 0b2 1r1", "0t3 0b3 1t0",
                 "1t1 1b0 1t2 1b1 0f0", "1t3 1b2 1b3 1f0")
INVERSE_SLOTS = ("0t0", "0t1 0m1", "0t2 0m2", "0t3 0m3",
                 "1t0 0o0", "1t1 1m1", "1t2 1m2", "1t3 1m3 1o0")

F32, BF16, U32 = jnp.float32, jnp.bfloat16, jnp.uint32
_SQH = float(np.sqrt(0.5))
_IM_SIGN = (0.0, -1.0, -1.0, 1.0)


def _pack_rows(m):
    b = np.asarray(m, np.float32).astype(jnp.bfloat16).view(np.uint16).astype(np.uint32)
    return b[..., 0::2, :] | (b[..., 1::2, :] << 16)


@functools.lru_cache(maxsize=None)
def _fft_constants():
    idx = np.arange(128)
    mf = np.zeros((4, 128, 256))
    mi = np.zeros((4, 128, 256))
    for t, res in enumerate(RESIDUES):
        k = (16 * (idx % 32) + np.repeat(res, 32))[None, :]
        th = 2 * np.pi * (((idx % 64 if t else idx)[:, None] * k) % D) / D
        co, si = np.cos(th), np.sin(th)
        if t:
            sg = _IM_SIGN[t] * np.where(k % 8 == t, 1.0, -1.0)
            top = idx[:, None] < 64
            re, im = np.where(top, co, sg * si), np.where(top, -si, sg * co)
        else:
            re, im = co, -si
        ma = np.concatenate([re[:, :64], im[:, :64]], axis=1)
        mb = np.concatenate([im[:, 64:], re[:, 64:]], axis=1)
        weight = np.full(128, 2.0)
        if t == 0:
            ma[:, 64] = (-1.0) ** idx
            weight[[0, 64]] = 1.0
        mf[t] = np.concatenate([ma, mb], axis=1)
        mi[t] = np.concatenate([(ma * weight).T, mb.T * 2.0], axis=1) / (S * D)
    gf = np.zeros((32, 128, 128))
    gi = np.zeros((32, 128, 128))
    for r in range(32):
        th = 2 * np.pi * ((idx[None, :64] * (32 * idx[:64, None] + r)) % S) / S
        gr, gim = np.cos(th), -np.sin(th)
        g = np.block([[gr, -gim], [gim, gr]])
        gf[r, :, 0::2], gf[r, :, 1::2] = g[:, :64], g[:, 64:]
        gi[r, :, 0::2], gi[r, :, 1::2] = g.T[:, :64], g.T[:, 64:]
    lane, r = idx[:, None], idx[None, :]
    live = (lane < 32) & (r < 32) & (lane // 16 == r % 2)
    th = 2 * np.pi * ((lane % 16) * r % 32) / 32
    fc, fs = np.cos(th) * live, -np.sin(th) * live
    small = np.stack([fc, fs, fc.T, fs.T,
                      (lane % 32 == r) * 1.0])
    th = 2 * np.pi * (idx[:64, None] * idx[None, :] % S) / S
    tw = np.stack([np.cos(th), -np.sin(th)]).astype(np.float32)
    return (_pack_rows(mf), _pack_rows(mi), _pack_rows(small), tw,
            _pack_rows(gf), _pack_rows(gi))


def _bfly8(x):
    x0, x1, x2, x3, x4, x5, x6, x7 = x
    t0, t1, t2, t3 = x0 + x4, x0 - x4, x2 + x6, x2 - x6
    t4, t5, t6, t7 = x1 + x5, x1 - x5, x3 + x7, x3 - x7
    u0, u1, u2, u3 = t0 + t2, t0 - t2, t4 + t6, t4 - t6
    p, q = _SQH * (t5 - t7), _SQH * (t5 + t7)
    return [(u0 + u2, u0 - u2), (t1 + p, t3 + q), (u1, u3), (t1 - p, t3 - q)]


def _bfly8_t(planes):
    (a0, a4), (a1r, a1i), (u1, u3), (a3r, a3i) = planes
    u0, u2 = a0 + a4, a0 - a4
    t1, p, t3, q = a1r + a3r, a1r - a3r, a1i + a3i, a1i - a3i
    t5, t7 = _SQH * (p + q), _SQH * (q - p)
    t0, t2, t4, t6 = u0 + u1, u0 - u1, u2 + u3, u2 - u3
    return [t0 + t1, t4 + t5, t2 + t3, t6 + t7, t0 - t1, t4 - t5, t2 - t3, t6 - t7]


def _swap_halves(x):
    return pltpu.roll(x, 64, 1)


def _lane_twiddle(t, low):
    c, s = float(np.cos(np.pi * t / 8)), float(np.sin(np.pi * t / 8)) * _IM_SIGN[t]
    return c, jnp.where(low, s, -s)


def _bfly2(t, a, b, low):
    c, s = _lane_twiddle(t, low)
    ra, rb = _swap_halves(a), _swap_halves(b)
    p = jnp.where(low, a, rb)
    q = c * jnp.where(low, ra, b) + s * jnp.where(low, rb, a)
    return p + q, p - q


def _bfly2_t(t, ga, gb, low):
    c, s = _lane_twiddle(t, low)
    p, q = ga + gb, ga - gb
    v = c * q - s * _swap_halves(q)
    y = _swap_halves(jnp.where(low, v, p))
    return jnp.where(low, p, y), jnp.where(low, y, v)


def _dft4(z):
    (ar, ai), (br, bi), (cr, ci), (dr, di) = z
    er, ei, fr, fi = ar + cr, ai + ci, ar - cr, ai - ci
    gr, gi, hr, hi = br + dr, bi + di, br - dr, bi - di
    return [(er + gr, ei + gi), (fr + hi, fi - hr), (er - gr, ei - gi), (fr - hi, fi + hr)]


def _twiddle(z, e):
    re, im = z
    if e == 0:
        return z
    if e == 8:
        return im, -re
    if e == 4:
        return _SQH * (re + im), _SQH * (im - re)
    if e == 12:
        return _SQH * (im - re), -_SQH * (re + im)
    c, s = float(np.cos(np.pi * e / 16)), float(np.sin(np.pi * e / 16))
    return re * c + im * s, im * c - re * s


def _dft16(z):
    cols = [_dft4([z[a + 4 * b] for b in range(4)]) for a in range(4)]
    out = [None] * 16
    for r1 in range(4):
        y = _dft4([_twiddle(cols[a][r1], 2 * a * r1) for a in range(4)])
        for r2 in range(4):
            out[r1 + 4 * r2] = y[r2]
    return out


def _swap(z):
    return [(im, re) for re, im in z]


def _half_dft32(z, odd):
    return _dft16([_twiddle(v, b * odd) for b, v in enumerate(z)])


def _half_idft32(z, odd):
    return _swap([_twiddle(v, b * odd) for b, v in enumerate(_dft16(_swap(z)))])


def _bf(x):
    return pltpu.bitcast(x, BF16)


def _pack(re, im):
    return pltpu.pack_elementwise([re, im], packed_dtype=BF16)


def _low_halves(a, b):
    return (a & jnp.uint32(0xFFFF)) | (b << 16)


def _high_halves(a, b):
    return (a >> 16) | (b & jnp.uint32(0xFFFF0000))


def _dot(a, b):
    return jnp.dot(a, b, preferred_element_type=F32)


def _dot_nt(a, b):
    return lax.dot_general(a, b, (((1,), (1,)), ((), ())), preferred_element_type=F32)


def _softmax(sc):
    e = jnp.exp(sc - jnp.max(sc, axis=-1, keepdims=True))
    l = jnp.sum(e, axis=-1, keepdims=True)
    r = pltpu.reciprocal(l, approx=True)
    return e * (r * (2.0 - l * r))


def _kernel(ax_hbm, wr_hbm, wi_hbm, bx_hbm, mem0_hbm, wq_hbm, wk_hbm, wv_hbm, wo_hbm,
            mf_hbm, mi_hbm, ms_hbm, tw_hbm, gf_hbm, gi_hbm,
            out_hbm,
            xa, wraw, wnyq, wp, mf, mi, ms, tw, gf, gi, ybuf, ubuf, nyq,
            xs, xpre3, xpre, stage, wqkv, wo, pre, kvmem, obuf, opre, part,
            sem, sem_a, sem_w):
    copy = pltpu.make_async_copy
    w_hbm = (wq_hbm, wk_hbm, wv_hbm)
    f_hbm = (wr_hbm, wi_hbm)
    scale = DH ** -0.5

    def xpre_copy(j):
        return copy(bx_hbm.at[pl.ds(8 * j, 8), :, 0], xpre3.at[pl.ds(8 * j, 8)], sem_a.at[8 + j])

    mf_copy = copy(mf_hbm, mf, sem.at[0])
    filter_stage_copies = [
        copy(src, dst, sem.at[1])
        for src, dst in ((ms_hbm, ms), (tw_hbm, tw), (mi_hbm, mi), (gf_hbm, gf), (gi_hbm, gi),
                         (wr_hbm.at[pl.ds(D // 2, 1)], wnyq.at[0]),
                         (wi_hbm.at[pl.ds(D // 2, 1)], wnyq.at[1]))]
    step_copies = [
        copy(bx_hbm.at[:, :, pl.ds(1, 3)], xs.at[pl.ds(0, 32), :, pl.ds(1, 3)], sem.at[2]),
        copy(mem0_hbm, xs.at[0, 0, 0], sem.at[2])]
    o_copy = copy(xs.at[pl.ds(0, 32), :, pl.ds(1, 3)],
                  out_hbm.at[:, :, pl.ds(1, 3), :, pl.ds(D, D)], sem.at[3])

    def opre_copy(g):
        return copy(xs.at[pl.ds(8 * g, 8), :, 0],
                    out_hbm.at[pl.ds(8 * g, 8), :, 0, :, pl.ds(D, D)], sem.at[3])

    def y_copy(c):
        return copy(xa.at[c], out_hbm.at[:, c // 4, c % 4, :, pl.ds(0, D)], sem.at[3])

    def wo_copy(n):
        return copy(wo_hbm.bitcast(U32).at[:, pl.ds(pl.multiple_of(n * 128, 128), 128)],
                    wo.at[n], sem.at[2])

    def a_copies(c):
        copies = [copy(ax_hbm.at[:, c], xa.at[c], sem_a.at[c])]
        for kap in (2 * c, 2 * c + 1):
            for i in range(2):
                src = f_hbm[i].at[pl.ds(0, D // 2)].bitcast(U32)
                copies.append(copy(
                    src.at[:, pl.ds(pl.multiple_of(kap * 128, 128), 128)],
                    wraw.at[pl.ds(pl.multiple_of((kap * 2 + i) * 256, 256), 256)],
                    sem_a.at[c]))
        return copies

    def w_copy(mat, pair, slot):
        return copy(w_hbm[mat].bitcast(U32).at[:, pair, :],
                    stage.at[pl.ds(pl.multiple_of(slot * D, D), D)], sem_w.at[slot])

    pl.loop(0, 2)(lambda slot: w_copy(0, slot, slot).start())
    pl.loop(0, 4)(lambda j: xpre_copy(j).start())
    pl.loop(2, NSLOT)(lambda slot: w_copy(0, slot, slot).start())
    mf_copy.start()

    lane = lax.broadcasted_iota(jnp.int32, (8, 128), 1)
    lanes = lax.broadcasted_iota(jnp.int32, (128, 128), 1)
    low = lanes < 64

    def a_forward(c, odd):
        row = pl.ds(pl.multiple_of(c * 8, 8), 8)
        lhs, x1 = {}, {}

        def rows(blk):
            lo = xa[c, pl.ds(8 * blk, 8)].astype(F32).reshape(64, D)
            hi = xa[c, pl.ds(16 + 8 * blk, 8)].astype(F32).reshape(64, D)
            xh = lo - hi if odd else lo + hi
            planes = _bfly8([xh[:, 128 * i:128 * (i + 1)] for i in range(8)])
            for t in range(4):
                pair = _bfly2(t, *planes[t], low[:64]) if t else planes[0]
                lhs[blk, t] = [v.astype(BF16) for v in pair]

        def transform(t):
            pa, pb = [_dot(jnp.concatenate([lhs[0, t][p], lhs[1, t][p]], axis=0),
                           _bf(mf[t, :, 128 * p:128 * (p + 1)])) for p in range(2)]
            x1[t] = jnp.where(low, pa, pb), _swap_halves(jnp.where(low, pb, pa))

        def butterflies(t):
            re, im = x1.pop(t)
            if t == 0:
                acc = nyq[row, :] if odd else jnp.zeros((8, 128), F32)
                for b in range(16):
                    k = 16 * odd + b
                    v = im[8 * b:8 * b + 8]
                    acc = jnp.where(lane == k, pltpu.roll(v, k, 1) if k else v, acc)
                nyq[row, :] = acc
                im = jnp.where(lanes == 0, 0.0, im)
            y = _half_dft32([(re[8 * b:8 * b + 8], im[8 * b:8 * b + 8]) for b in range(16)], odd)
            for r in range(16):
                ybuf[2 * r + odd, row, 128 * t:128 * (t + 1)] = _pack(*y[r])

        return {"r": rows, "t": transform, "b": butterflies,
                "f": lambda _: a_filter_layout(c, odd)}

    def a_filter_layout(it, i):
        base = (2 * it + i) * 512
        wr = [wraw[pl.ds(base + j, 32, stride=8), :] for j in range(8)]
        wi = [wraw[pl.ds(base + 256 + j, 32, stride=8), :] for j in range(8)]
        res = [(_low_halves, _high_halves)[k % 2](wr[k // 2], wi[k // 2]) for k in range(16)]
        for t in range(4):
            tile = jnp.concatenate([res[k] for k in RESIDUES[t]], axis=0).T
            dst = wp.at[pl.ds(pl.multiple_of(t * WP_ROWS + it * 264, 8), 264)]
            for m in range(4):
                dst[pl.ds(33 * (4 * i + m), 32), :] = tile[32 * m:32 * (m + 1)]

    def a_nyquist():
        b = nyq[...].astype(BF16)
        yr, yi = _dot(b, _bf(ms[0])), _dot(b, _bf(ms[1]))
        sub = lax.broadcasted_iota(jnp.int32, (8, 128), 0)
        wn = []
        for i in range(2):
            w = wnyq[i].astype(F32)
            spread = jnp.concatenate(
                [jnp.where(lane // 32 == sub % 4,
                           jnp.where(sub < 4, w[:, 256 * k:256 * k + 128],
                                     w[:, 256 * k + 128:256 * k + 256]), 0.0)
                 for k in range(8)], axis=0)
            wn.append(_dot(spread.astype(BF16), _bf(ms[4])))
        yield
        yield
        tc, ts = tw[0], tw[1]
        x2 = _dot(_bf(gf[0]), _bf(_pack(yr * tc - yi * ts, yr * ts + yi * tc)))
        yield
        yield
        a, b = x2[:64], x2[64:]
        u = _dot(_bf(gi[0]), _bf(_pack(a * wn[0] - b * wn[1], a * wn[1] + b * wn[0])))
        yield
        yield
        ur, ui = u[:64], u[64:]
        nyq[...] = (_dot((ur * tc + ui * ts).astype(BF16), _bf(ms[2]))
                    + _dot((ui * tc - ur * ts).astype(BF16), _bf(ms[3])))

    def a_filter(it, side=()):
        z = {}
        side = iter(side)

        def fwd(i):
            r = 8 * it + i
            x2 = _dot(_bf(gf[r]), _bf(ybuf[r]))
            tiles = []
            for t in range(4):
                w = wp[pl.ds(t * WP_ROWS + r, 64, stride=33), :]
                wr = pltpu.bitcast(w << 16, F32)
                wi = pltpu.bitcast(w & jnp.uint32(0xFFFF0000), F32)
                a, b = x2[:64, 128 * t:128 * (t + 1)], x2[64:, 128 * t:128 * (t + 1)]
                tiles.append(_pack(a * wr - b * wi, a * wi + b * wr))
            z[i] = jnp.concatenate(tiles, axis=1)

        def inv(i):
            r = 8 * it + i
            ubuf[r] = _dot(_bf(gi[r]), _bf(z.pop(i)))

        lag = 2
        for i in range(8 + lag):
            next(side, None)
            if i < 8:
                fwd(i)
            if i >= lag:
                inv(i - lag)

    def a_inverse(c, odd, halves):
        r0 = pl.multiple_of(c * 8, 8)
        planes = {}

        def transform(t):
            cols = slice(128 * t, 128 * (t + 1))
            x3 = _half_idft32(
                [(ubuf[2 * r + odd, pl.ds(r0, 8), cols],
                  ubuf[2 * r + odd, pl.ds(64 + r0, 8), cols]) for r in range(16)], odd)
            re, im = [jnp.concatenate([v[p] for v in x3], axis=0) for p in range(2)]
            im = _swap_halves(im)
            hi = im
            if t == 0:
                bn = nyq[pl.ds(r0, 8), :]
                bn = jnp.concatenate(
                    [pltpu.roll(bn, 64 - 16 * odd - b, 1) for b in range(16)], axis=0)
                hi = jnp.where(lanes == 64, bn, im)
            planes[t] = (_dot(jnp.where(low, re, hi).astype(BF16), _bf(mi[t, :, :128])),
                         _dot(jnp.where(low, im, re).astype(BF16), _bf(mi[t, :, 128:])))

        def merge(t):
            planes[t] = _bfly2_t(t, *planes[t], low)

        def output(_):
            halves.append(jnp.concatenate(_bfly8_t([planes[t] for t in range(4)]), axis=1))
            if odd:
                y = jnp.concatenate([halves[0] + halves[1], halves[0] - halves[1]], axis=0)
                xa[c] = y.reshape(32, 8, D).astype(BF16)

        return {"t": transform, "m": merge, "o": output}

    def regroup_pair(mat, pair, slot):
        ev = stage[pl.ds(slot * D, D // 2, stride=2), :]
        od = stage[pl.ds(slot * D + 1, D // 2, stride=2), :]
        lo, hi = _low_halves(ev, od), _high_halves(ev, od)
        wqkv[6 * pair + mat] = lo
        wqkv[6 * pair + 3 + mat] = hi
        return lo, hi

    def project_pair(mat, pair, slot, side):
        lo, hi = regroup_pair(mat, pair, slot)
        nslice = 1 if side is None else 4
        rows = NPRE // nslice
        for j in range(nslice):
            if side is not None:
                next(side)
            if j:
                lo, hi = wqkv[6 * pair + mat], wqkv[6 * pair + 3 + mat]
            p = _dot(_bf(xpre[rows // 2 * j:rows // 2 * (j + 1), :]),
                     _bf(jnp.concatenate([lo, hi], axis=1))).astype(BF16)
            pre[mat, 2 * pair, rows * j:rows * (j + 1), :] = p[:, :DH]
            pre[mat, 2 * pair + 1, rows * j:rows * (j + 1), :] = p[:, DH:]

    def project_loop(mat, npair, before, side, after, start=0):
        @pl.loop(start, 16 // npair)
        def _(it):
            first = npair * it
            slot0 = (16 * mat + first) % NSLOT
            for i in range(npair):
                w_copy(mat, first + i, slot0 + i).wait()
            before(it)
            work = side(it)
            for i in range(npair):
                project_pair(mat, first + i, slot0 + i, work)

            @pl.when(first + NSLOT < 16)
            def _():
                for i in range(npair):
                    w_copy(mat, first + NSLOT + i, slot0 + i).start()

            if mat < 2:
                @pl.when(first + NSLOT >= 16)
                def _():
                    for i in range(npair):
                        w_copy(mat + 1, first + NSLOT - 16 + i, slot0 + i).start()

            after(it)

    def nothing(it):
        return None

    def fetch_a_inputs(it):
        for cp in a_copies(it):
            cp.start()

    def wait_a_inputs(it):
        for cp in a_copies(it):
            cp.wait()

    def in_slots(units, table):
        for slot in table:
            for unit, kind, index in slot.split():
                units[int(unit)][kind](int(index))
            yield

    def forward_fft(it):
        return in_slots([a_forward(it, odd) for odd in range(2)], FORWARD_SLOTS)

    def fetch_wo(it):
        wo_copy(it).start()

    def inverse_fft(it):
        halves = []
        return in_slots([a_inverse(it, odd, halves) for odd in range(2)], INVERSE_SLOTS)

    for i in range(2):
        w_copy(0, i, i).wait()
        regroup_pair(0, i, i)
        w_copy(0, NSLOT + i, i).start()
    fetch_a_inputs(0)

    @pl.loop(0, 4)
    def _(j):
        xpre_copy(j).wait()
        x = xpre3[pl.ds(8 * j, 8)].reshape(128, D)
        xpre[pl.ds(pl.multiple_of(j * 64, 64), 64), :] = pltpu.bitcast(x, U32)
        w = jnp.concatenate([wqkv[3 * hd] for hd in range(4)], axis=1)
        p = _dot(x, _bf(w)).astype(BF16)
        for hd in range(4):
            pre[0, hd, pl.ds(pl.multiple_of(j * 128, 128), 128), :] = p[:, DH * hd:DH * (hd + 1)]

    project_loop(0, 2, nothing, nothing, fetch_a_inputs, start=1)
    for cp in filter_stage_copies:
        cp.start()
    mf_copy.wait()
    project_loop(1, 2, wait_a_inputs, forward_fft, fetch_wo)
    for cp in step_copies:
        cp.start()
    for cp in filter_stage_copies:
        cp.wait()
    a_filter(0, a_nyquist())
    pl.loop(1, 4)(a_filter)
    project_loop(2, 2, nothing, inverse_fft, nothing)
    for c in range(8):
        y_copy(c).start()

    for cp in step_copies + [wo_copy(n) for n in range(8)]:
        cp.wait()

    def segment(s, h, split):
        row = lax.broadcasted_iota(jnp.int32, (32, 48), 0)
        col = lax.broadcasted_iota(jnp.int32, (32, 48), 1)
        allowed = ((row < NMEM) | (col >= 32) | (col <= row)) & (col < 40)
        p0 = pl.ds(pl.multiple_of(s * 8, 8), 8)
        zeros = jnp.zeros((8, DH), BF16)
        st = {}

        def half(i, a):
            return _dot(h[:, 512 * a:512 * (a + 1)], _bf(wqkv[i, 256 * a:256 * (a + 1), :]))

        def qkv(hd):
            if hd == 0 and split:
                for i in range(3):
                    part[i] = half(i, 0)
                q, k, v = [(part[i] + half(i, 1)).astype(BF16) for i in range(3)]
            else:
                q, k, v = [_dot(h, _bf(wqkv[3 * hd + i])).astype(BF16) for i in range(3)]
            kvmem[0, hd, p0, :] = k[:NMEM]
            kvmem[1, hd, p0, :] = v[:NMEM]
            st[hd] = (q, k, v)

        def scores(hd):
            q, k, v = st[hd]
            ka = jnp.concatenate([k, pre[1, hd, p0, :], zeros], axis=0)
            sc = jnp.where(allowed, _dot_nt(q, ka) * scale, -jnp.inf)
            st[hd] = (_softmax(sc).astype(BF16), v)

        def context(hd):
            p, v = st.pop(hd)
            va = jnp.concatenate([v, pre[2, hd, p0, :], zeros], axis=0)
            obuf[:, hd * DH:(hd + 1) * DH] = _dot(p, va).astype(BF16)

        acc = [None] * 8

        def project(g):
            lhs = obuf[:, 4 * g * DH:4 * (g + 1) * DH]
            for n in range(8):
                t = _dot(lhs, _bf(wo[n, 256 * g:256 * (g + 1), :]))
                acc[n] = t if acc[n] is None else acc[n] + t

        lag_scores, lag_context = 1, 3
        for hd in range(H):
            qkv(hd)
            if hd >= lag_scores:
                scores(hd - lag_scores)
            if hd >= lag_context:
                context(hd - lag_context)
            if hd == 28:
                project(0)
        for t, g in enumerate(range(1, H // 4)):
            project(g)
            if t < lag_scores:
                scores(H + t - lag_scores)
            if t < lag_context:
                context(H + t - lag_context)
        return acc

    @pl.loop(0, NSEG // 4)
    def _(i):
        h = xs[2 * i, 0].reshape(32, D)
        for u in range(4):
            acc = segment(4 * i + u, h, u > 0)
            if u < 3:
                xt = xs[2 * i + (u + 1) // 2, (u + 1) % 2, pl.ds(1, 3)].astype(F32).reshape(24, D)
                h = jnp.concatenate(
                    [jnp.concatenate([acc[n][:NMEM], xt[:, 128 * n:128 * (n + 1)]],
                                     axis=0).astype(BF16) for n in range(8)], axis=1)
            ob = jnp.concatenate(acc, axis=1).astype(BF16).reshape(4, 8, D)
            xs[2 * i + u // 2, u % 2, pl.ds(1, 3)] = ob[1:]
        xs[2 * i + 2, 0, 0] = ob[0]

    o_copy.start()

    @pl.loop(0, 4)
    def _(g):
        row = lax.broadcasted_iota(jnp.int32, (64, 128), 0)
        col = lax.broadcasted_iota(jnp.int32, (64, 128), 1)
        allowed = ((col % 64) // 8 == row // 8) & ((col < 64) | (col % 8 <= row % 8))
        st = {}

        def rows(a):
            return pl.ds(pl.multiple_of(g * 128 + a * 64, 64), 64)

        def scores(hd):
            for a in range(2):
                ka = jnp.concatenate([kvmem[0, hd, rows(a), :], pre[1, hd, rows(a), :]], axis=0)
                sc = jnp.where(allowed, _dot_nt(pre[0, hd, rows(a), :], ka) * scale, -jnp.inf)
                st[hd, a] = _softmax(sc).astype(BF16)

        def context(hd):
            for a in range(2):
                va = jnp.concatenate([kvmem[1, hd, rows(a), :], pre[2, hd, rows(a), :]], axis=0)
                opre[a * 64:(a + 1) * 64, hd * DH:(hd + 1) * DH] = (
                    _dot(st.pop((hd, a)), va).astype(BF16))

        acc = None
        for c in range(H // 8 + 2):
            if c < H // 8:
                for hd in range(8 * c, 8 * c + 8):
                    scores(hd)
            if c >= 2:
                lhs = opre[:, 8 * (c - 2) * DH:8 * (c - 1) * DH]
                t = jnp.concatenate([_dot(lhs, _bf(wo[n, 512 * (c - 2):512 * (c - 1), :]))
                                     for n in range(8)], axis=1)
                acc = t if acc is None else acc + t
            if 1 <= c <= H // 8:
                for hd in range(8 * (c - 1), 8 * c):
                    context(hd)
        xs[pl.ds(g * 8, 8), :, 0] = acc.astype(BF16).reshape(8, 2, 8, D)
        opre_copy(g).start()

    for cp in [y_copy(c) for c in range(8)] + [o_copy] + [opre_copy(g) for g in range(4)]:
        cp.wait()


@functools.partial(jax.jit, static_argnames=("B_seg_len",))
def pallas_concat_heads__spectral_gfnet__memory_aug_recurrent_mem_tr__prompt_kernel(
    A_x, A_w_r, A_w_i, B_x, B_mem0, B_Wq, B_Wk, B_Wv, B_Wo, B_seg_len=SEG,
):
    assert A_x.shape == (1, S, D) and B_x.shape == (1, S, D)
    assert A_w_r.shape == A_w_i.shape == (S, D // 2 + 1)
    assert B_mem0.shape == (1, NMEM, D) and B_seg_len == SEG
    assert B_Wq.shape == B_Wk.shape == B_Wv.shape == (D, H, DH) and B_Wo.shape == (H, DH, D)

    vmem = pltpu.VMEM
    dma = pltpu.SemaphoreType.DMA
    scratch = [
        vmem((8, 32, 8, D), BF16),
        vmem((32 * 256 + 32, 128), U32),
        vmem((2, 1, S), BF16),
        vmem((4 * WP_ROWS + 32, 128), U32),
        vmem((4, 64, 256), U32),
        vmem((4, 64, 256), U32),
        vmem((5, 64, 128), U32),
        vmem((2, 64, 128), F32),
        vmem((32, 64, 128), U32),
        vmem((32, 64, 128), U32),
        vmem((32, 64, 512), U32),
        vmem((32, 128, 512), F32),
        vmem((64, 128), F32),
        vmem((33, 2, 4, 8, D), BF16),
        vmem((32, 2, 8, D), BF16),
        vmem((NPRE // 2, D), U32),
        vmem((NSLOT * D + 32, 128), U32),
        vmem((3 * H, D // 2, DH), U32),
        vmem((8, H * DH // 2, 128), U32),
        vmem((3, H, NPRE, DH), BF16),
        vmem((2, H, NPRE, DH), BF16),
        vmem((32, H * DH), BF16),
        vmem((128, H * DH), BF16),
        vmem((3, 32, DH), F32),
        dma((4,)), dma((12,)), dma((NSLOT,)),
    ]
    hbm = pl.BlockSpec(memory_space=pltpu.HBM)
    out = pl.pallas_call(
        _kernel,
        out_shape=jax.ShapeDtypeStruct((32, 2, 4, 8, 2 * D), BF16),
        in_specs=[hbm] * 15,
        out_specs=hbm,
        scratch_shapes=scratch,
        compiler_params=pltpu.CompilerParams(vmem_limit_bytes=124 * 1024 * 1024),
    )(A_x.reshape(32, 8, 8, D), A_w_r.T, A_w_i.T,
      B_x.reshape(32, 2, 4, 8, D), B_mem0.reshape(NMEM, D),
      B_Wq, B_Wk, B_Wv, B_Wo.reshape(H * DH, D),
      *[jnp.asarray(c) for c in _fft_constants()])
    return out.reshape(1, S, 2 * D)
```

```python
import functools

import numpy as np
import jax
import jax.numpy as jnp
from jax import lax
import jax.experimental.pallas as pl
import jax.experimental.pallas.tpu as pltpu

S, D = 2048, 1024
H, DH = 32, 128
NMEM, SEG = 8, 32
NSEG = S // SEG
NPRE = NSEG * 8
NSLOT = 12
WP_ROWS = 33 * 64
RESIDUES = ((0, 8, 4, 12), (1, 15, 9, 7), (2, 14, 10, 6), (3, 13, 11, 5))

FORWARD_SLOTS = ("0r0", "0r1", "0t0 0b0", "0t1 0b1 1r0", "0t2 0b2 1r1", "0t3 0b3 1t0",
                 "1t1 1b0 1t2 1b1 0f0", "1t3 1b2 1b3 1f0")
INVERSE_SLOTS = ("0t0", "0t1 0m1", "0t2 0m2", "0t3 0m3",
                 "1t0 0o0", "1t1 1m1", "1t2 1m2", "1t3 1m3 1o0")

F32, BF16, U32 = jnp.float32, jnp.bfloat16, jnp.uint32
_SQH = float(np.sqrt(0.5))
_IM_SIGN = (0.0, -1.0, -1.0, 1.0)


def _pack_rows(m):
    b = np.asarray(m, np.float32).astype(jnp.bfloat16).view(np.uint16).astype(np.uint32)
    return b[..., 0::2, :] | (b[..., 1::2, :] << 16)


@functools.lru_cache(maxsize=None)
def _fft_constants():
    idx = np.arange(128)
    mf = np.zeros((4, 128, 256))
    mi = np.zeros((4, 128, 256))
    for t, res in enumerate(RESIDUES):
        k = (16 * (idx % 32) + np.repeat(res, 32))[None, :]
        th = 2 * np.pi * (((idx % 64 if t else idx)[:, None] * k) % D) / D
        co, si = np.cos(th), np.sin(th)
        if t:
            sg = _IM_SIGN[t] * np.where(k % 8 == t, 1.0, -1.0)
            top = idx[:, None] < 64
            re, im = np.where(top, co, sg * si), np.where(top, -si, sg * co)
        else:
            re, im = co, -si
        ma = np.concatenate([re[:, :64], im[:, :64]], axis=1)
        mb = np.concatenate([im[:, 64:], re[:, 64:]], axis=1)
        weight = np.full(128, 2.0)
        if t == 0:
            ma[:, 64] = (-1.0) ** idx
            weight[[0, 64]] = 1.0
        mf[t] = np.concatenate([ma, mb], axis=1)
        mi[t] = np.concatenate([(ma * weight).T, mb.T * 2.0], axis=1) / (S * D)
    gf = np.zeros((32, 128, 128))
    gi = np.zeros((32, 128, 128))
    for r in range(32):
        th = 2 * np.pi * ((idx[None, :64] * (32 * idx[:64, None] + r)) % S) / S
        gr, gim = np.cos(th), -np.sin(th)
        g = np.block([[gr, -gim], [gim, gr]])
        gf[r] = g[:, idx // 16 * 8 + idx % 8 + idx // 8 % 2 * 64]
        gi[r] = g.T
    lane, r = idx[:, None], idx[None, :]
    live = (lane < 32) & (r < 32) & (lane // 16 == r % 2)
    th = 2 * np.pi * ((lane % 16) * r % 32) / 32
    fc, fs = np.cos(th) * live, -np.sin(th) * live
    small = np.stack([fc, fs, fc.T, fs.T,
                      (lane % 32 == r) * 1.0])
    th = 2 * np.pi * (idx[:64, None] * idx[None, :] % S) / S
    tw = np.stack([np.cos(th), -np.sin(th)]).astype(np.float32)
    return (_pack_rows(mf), _pack_rows(mi), _pack_rows(small), tw,
            _pack_rows(gf), _pack_rows(gi))


def _bfly8(x):
    x0, x1, x2, x3, x4, x5, x6, x7 = x
    t0, t1, t2, t3 = x0 + x4, x0 - x4, x2 + x6, x2 - x6
    t4, t5, t6, t7 = x1 + x5, x1 - x5, x3 + x7, x3 - x7
    u0, u1, u2, u3 = t0 + t2, t0 - t2, t4 + t6, t4 - t6
    p, q = _SQH * (t5 - t7), _SQH * (t5 + t7)
    return [(u0 + u2, u0 - u2), (t1 + p, t3 + q), (u1, u3), (t1 - p, t3 - q)]


def _bfly8_t(planes):
    (a0, a4), (a1r, a1i), (u1, u3), (a3r, a3i) = planes
    u0, u2 = a0 + a4, a0 - a4
    t1, p, t3, q = a1r + a3r, a1r - a3r, a1i + a3i, a1i - a3i
    t5, t7 = _SQH * (p + q), _SQH * (q - p)
    t0, t2, t4, t6 = u0 + u1, u0 - u1, u2 + u3, u2 - u3
    return [t0 + t1, t4 + t5, t2 + t3, t6 + t7, t0 - t1, t4 - t5, t2 - t3, t6 - t7]


def _swap_halves(x):
    return pltpu.roll(x, 64, 1)


def _lane_twiddle(t, low):
    c, s = float(np.cos(np.pi * t / 8)), float(np.sin(np.pi * t / 8)) * _IM_SIGN[t]
    return c, jnp.where(low, s, -s)


def _bfly2(t, a, b, low):
    c, s = _lane_twiddle(t, low)
    ra, rb = _swap_halves(a), _swap_halves(b)
    p = jnp.where(low, a, rb)
    q = c * jnp.where(low, ra, b) + s * jnp.where(low, rb, a)
    return p + q, p - q


def _bfly2_t(t, ga, gb, low):
    c, s = _lane_twiddle(t, low)
    p, q = ga + gb, ga - gb
    v = c * q - s * _swap_halves(q)
    y = _swap_halves(jnp.where(low, v, p))
    return jnp.where(low, p, y), jnp.where(low, y, v)


def _dft4(z):
    (ar, ai), (br, bi), (cr, ci), (dr, di) = z
    er, ei, fr, fi = ar + cr, ai + ci, ar - cr, ai - ci
    gr, gi, hr, hi = br + dr, bi + di, br - dr, bi - di
    return [(er + gr, ei + gi), (fr + hi, fi - hr), (er - gr, ei - gi), (fr - hi, fi + hr)]


def _twiddle(z, e):
    re, im = z
    if e == 0:
        return z
    if e == 8:
        return im, -re
    if e == 4:
        return _SQH * (re + im), _SQH * (im - re)
    if e == 12:
        return _SQH * (im - re), -_SQH * (re + im)
    c, s = float(np.cos(np.pi * e / 16)), float(np.sin(np.pi * e / 16))
    return re * c + im * s, im * c - re * s


def _dft16(z):
    cols = [_dft4([z[a + 4 * b] for b in range(4)]) for a in range(4)]
    out = [None] * 16
    for r1 in range(4):
        y = _dft4([_twiddle(cols[a][r1], 2 * a * r1) for a in range(4)])
        for r2 in range(4):
            out[r1 + 4 * r2] = y[r2]
    return out


def _swap(z):
    return [(im, re) for re, im in z]


def _half_dft32(z, odd):
    return _dft16([_twiddle(v, b * odd) for b, v in enumerate(z)])


def _half_idft32(z, odd):
    return _swap([_twiddle(v, b * odd) for b, v in enumerate(_dft16(_swap(z)))])


def _bf(x):
    return pltpu.bitcast(x, BF16)


def _stack(*rows):
    return jnp.concatenate(rows, axis=0).astype(BF16)


def _low_halves(a, b):
    return (a & jnp.uint32(0xFFFF)) | (b << 16)


def _high_halves(a, b):
    return (a >> 16) | (b & jnp.uint32(0xFFFF0000))


def _dot(a, b):
    return jnp.dot(a, b, preferred_element_type=F32)


def _dot_nt(a, b):
    return lax.dot_general(a, b, (((1,), (1,)), ((), ())), preferred_element_type=F32)


def _softmax(sc):
    e = jnp.exp(sc - jnp.max(sc, axis=-1, keepdims=True))
    l = jnp.sum(e, axis=-1, keepdims=True)
    r = pltpu.reciprocal(l, approx=True)
    return e * (r * (2.0 - l * r))


def _kernel(ax_hbm, wr_hbm, wi_hbm, bx_hbm, mem0_hbm, wq_hbm, wk_hbm, wv_hbm, wo_hbm,
            mf_hbm, mi_hbm, ms_hbm, tw_hbm, gf_hbm, gi_hbm,
            out_hbm,
            xa, wraw, wnyq, wp, mf, mi, ms, tw, gf, gi, ybuf, ubuf, nyq,
            xs, xpre3, xpre, stage, wqkv, wo, pre, kvmem, obuf, opre, part,
            sem, sem_a, sem_w):
    copy = pltpu.make_async_copy
    w_hbm = (wq_hbm, wk_hbm, wv_hbm)
    f_hbm = (wr_hbm, wi_hbm)
    scale = DH ** -0.5

    def xpre_copy(j):
        return copy(bx_hbm.at[pl.ds(8 * j, 8), :, 0], xpre3.at[pl.ds(8 * j, 8)], sem_a.at[8 + j])

    mf_copy = copy(mf_hbm, mf, sem.at[0])
    filter_stage_copies = [
        copy(src, dst, sem.at[1])
        for src, dst in ((ms_hbm, ms), (tw_hbm, tw), (mi_hbm, mi), (gf_hbm, gf), (gi_hbm, gi),
                         (wr_hbm.at[pl.ds(D // 2, 1)], wnyq.at[0]),
                         (wi_hbm.at[pl.ds(D // 2, 1)], wnyq.at[1]))]
    step_copies = [
        copy(bx_hbm.at[:, :, pl.ds(1, 3)], xs.at[pl.ds(0, 32), :, pl.ds(1, 3)], sem.at[2]),
        copy(mem0_hbm, xs.at[0, 0, 0], sem.at[2])]
    o_copy = copy(xs.at[pl.ds(0, 32), :, pl.ds(1, 3)],
                  out_hbm.at[:, :, pl.ds(1, 3), :, pl.ds(D, D)], sem.at[3])

    def opre_copy(g):
        return copy(xs.at[pl.ds(8 * g, 8), :, 0],
                    out_hbm.at[pl.ds(8 * g, 8), :, 0, :, pl.ds(D, D)], sem.at[3])

    def y_copy(c):
        return copy(xa.at[c], out_hbm.at[:, c // 4, c % 4, :, pl.ds(0, D)], sem.at[3])

    def wo_copy(n):
        return copy(wo_hbm.bitcast(U32).at[:, pl.ds(pl.multiple_of(n * 128, 128), 128)],
                    wo.at[n], sem.at[2])

    def a_copies(c):
        copies = [copy(ax_hbm.at[:, c], xa.at[c], sem_a.at[c])]
        for kap in (2 * c, 2 * c + 1):
            for i in range(2):
                src = f_hbm[i].at[pl.ds(0, D // 2)].bitcast(U32)
                copies.append(copy(
                    src.at[:, pl.ds(pl.multiple_of(kap * 128, 128), 128)],
                    wraw.at[pl.ds(pl.multiple_of((kap * 2 + i) * 256, 256), 256)],
                    sem_a.at[c]))
        return copies

    def w_copy(mat, pair, slot):
        return copy(w_hbm[mat].bitcast(U32).at[:, pair, :],
                    stage.at[pl.ds(pl.multiple_of(slot * D, D), D)], sem_w.at[slot])

    pl.loop(0, 2)(lambda slot: w_copy(0, slot, slot).start())
    pl.loop(0, 4)(lambda j: xpre_copy(j).start())
    pl.loop(2, NSLOT)(lambda slot: w_copy(0, slot, slot).start())
    mf_copy.start()

    lane = lax.broadcasted_iota(jnp.int32, (8, 128), 1)
    lanes = lax.broadcasted_iota(jnp.int32, (128, 128), 1)
    low = lanes < 64

    def a_forward(c, odd):
        row = pl.ds(pl.multiple_of(c * 8, 8), 8)
        lhs, x1 = {}, {}

        def rows(blk):
            lo = xa[c, pl.ds(8 * blk, 8)].astype(F32).reshape(64, D)
            hi = xa[c, pl.ds(16 + 8 * blk, 8)].astype(F32).reshape(64, D)
            xh = lo - hi if odd else lo + hi
            planes = _bfly8([xh[:, 128 * i:128 * (i + 1)] for i in range(8)])
            for t in range(4):
                pair = _bfly2(t, *planes[t], low[:64]) if t else planes[0]
                lhs[blk, t] = [v.astype(BF16) for v in pair]

        def transform(t):
            pa, pb = [_dot(jnp.concatenate([lhs[0, t][p], lhs[1, t][p]], axis=0),
                           _bf(mf[t, :, 128 * p:128 * (p + 1)])) for p in range(2)]
            x1[t] = jnp.where(low, pa, pb), _swap_halves(jnp.where(low, pb, pa))

        def butterflies(t):
            re, im = x1.pop(t)
            if t == 0:
                acc = nyq[row, :] if odd else jnp.zeros((8, 128), F32)
                for b in range(16):
                    k = 16 * odd + b
                    v = im[8 * b:8 * b + 8]
                    acc = jnp.where(lane == k, pltpu.roll(v, k, 1) if k else v, acc)
                nyq[row, :] = acc
                im = jnp.where(lanes == 0, 0.0, im)
            y = _half_dft32([(re[8 * b:8 * b + 8], im[8 * b:8 * b + 8]) for b in range(16)], odd)
            for r in range(16):
                ybuf[2 * r + odd, t, pl.ds(pl.multiple_of(c * 16, 16), 16), :] = _stack(*y[r])

        return {"r": rows, "t": transform, "b": butterflies,
                "f": lambda _: a_filter_layout(c, odd)}

    def a_filter_layout(it, i):
        base = (2 * it + i) * 512
        wr = [wraw[pl.ds(base + j, 32, stride=8), :] for j in range(8)]
        wi = [wraw[pl.ds(base + 256 + j, 32, stride=8), :] for j in range(8)]
        res = [(_low_halves, _high_halves)[k % 2](wr[k // 2], wi[k // 2]) for k in range(16)]
        for t in range(4):
            tile = jnp.concatenate([res[k] for k in RESIDUES[t]], axis=0).T
            dst = wp.at[pl.ds(pl.multiple_of(t * WP_ROWS + it * 264, 8), 264)]
            for m in range(4):
                dst[pl.ds(33 * (4 * i + m), 32), :] = tile[32 * m:32 * (m + 1)]

    def a_nyquist():
        b = nyq[...].astype(BF16)
        yr, yi = _dot(b, _bf(ms[0])), _dot(b, _bf(ms[1]))
        sub = lax.broadcasted_iota(jnp.int32, (8, 128), 0)
        wn = []
        for i in range(2):
            w = wnyq[i].astype(F32)
            spread = jnp.concatenate(
                [jnp.where(lane // 32 == sub % 4,
                           jnp.where(sub < 4, w[:, 256 * k:256 * k + 128],
                                     w[:, 256 * k + 128:256 * k + 256]), 0.0)
                 for k in range(8)], axis=0)
            wn.append(_dot(spread.astype(BF16), _bf(ms[4])))
        yield
        yield
        tc, ts = tw[0], tw[1]
        yr, yi = yr * tc - yi * ts, yr * ts + yi * tc
        x2 = _dot(_bf(gf[0]), _stack(*[v[8 * c:8 * c + 8] for c in range(8) for v in (yr, yi)]))
        yield
        yield
        a, b = x2[:64], x2[64:]
        u = _dot(_bf(gi[0]), _stack(a * wn[0] - b * wn[1], a * wn[1] + b * wn[0]))
        yield
        yield
        ur, ui = u[:64], u[64:]
        nyq[...] = (_dot((ur * tc + ui * ts).astype(BF16), _bf(ms[2]))
                    + _dot((ui * tc - ur * ts).astype(BF16), _bf(ms[3])))

    def a_filter(it, side=()):
        z = {}
        side = iter(side)

        def fwd(i):
            r = 8 * it + i
            x2 = _dot(_bf(gf[r]), jnp.concatenate([ybuf[r, t] for t in range(4)], axis=1))
            w = jnp.concatenate([wp[pl.ds(t * WP_ROWS + r, 64, stride=33), :]
                                 for t in range(4)], axis=1)
            wr = pltpu.bitcast(w << 16, F32)
            wi = pltpu.bitcast(w & jnp.uint32(0xFFFF0000), F32)
            a, b = x2[:64], x2[64:]
            z[i] = _stack(a * wr - b * wi, a * wi + b * wr)

        def inv(i):
            r = 8 * it + i
            ubuf[r] = _dot(_bf(gi[r]), z.pop(i))

        lag = 2
        for i in range(8 + lag):
            next(side, None)
            if i < 8:
                fwd(i)
            if i >= lag:
                inv(i - lag)

    def a_inverse(c, odd, halves):
        r0 = pl.multiple_of(c * 8, 8)
        planes = {}

        def transform(t):
            cols = slice(128 * t, 128 * (t + 1))
            x3 = _half_idft32(
                [(ubuf[2 * r + odd, pl.ds(r0, 8), cols],
                  ubuf[2 * r + odd, pl.ds(64 + r0, 8), cols]) for r in range(16)], odd)
            re, im = [jnp.concatenate([v[p] for v in x3], axis=0) for p in range(2)]
            im = _swap_halves(im)
            hi = im
            if t == 0:
                bn = nyq[pl.ds(r0, 8), :]
                bn = jnp.concatenate(
                    [pltpu.roll(bn, 64 - 16 * odd - b, 1) for b in range(16)], axis=0)
                hi = jnp.where(lanes == 64, bn, im)
            planes[t] = (_dot(jnp.where(low, re, hi).astype(BF16), _bf(mi[t, :, :128])),
                         _dot(jnp.where(low, im, re).astype(BF16), _bf(mi[t, :, 128:])))

        def merge(t):
            planes[t] = _bfly2_t(t, *planes[t], low)

        def output(_):
            halves.append(jnp.concatenate(_bfly8_t([planes[t] for t in range(4)]), axis=1))
            if odd:
                y = jnp.concatenate([halves[0] + halves[1], halves[0] - halves[1]], axis=0)
                xa[c] = y.reshape(32, 8, D).astype(BF16)

        return {"t": transform, "m": merge, "o": output}

    def regroup_pair(mat, pair, slot):
        ev = stage[pl.ds(slot * D, D // 2, stride=2), :]
        od = stage[pl.ds(slot * D + 1, D // 2, stride=2), :]
        lo, hi = _low_halves(ev, od), _high_halves(ev, od)
        wqkv[6 * pair + mat] = lo
        wqkv[6 * pair + 3 + mat] = hi
        return lo, hi

    def project_pair(mat, pair, slot, side):
        lo, hi = regroup_pair(mat, pair, slot)
        nslice = 1 if side is None else 4
        rows = NPRE // nslice
        for j in range(nslice):
            if side is not None:
                next(side)
            if j:
                lo, hi = wqkv[6 * pair + mat], wqkv[6 * pair + 3 + mat]
            p = _dot(_bf(xpre[rows // 2 * j:rows // 2 * (j + 1), :]),
                     _bf(jnp.concatenate([lo, hi], axis=1))).astype(BF16)
            pre[mat, 2 * pair, rows * j:rows * (j + 1), :] = p[:, :DH]
            pre[mat, 2 * pair + 1, rows * j:rows * (j + 1), :] = p[:, DH:]

    def project_loop(mat, npair, before, side, after, start=0):
        @pl.loop(start, 16 // npair)
        def _(it):
            first = npair * it
            slot0 = (16 * mat + first) % NSLOT
            for i in range(npair):
                w_copy(mat, first + i, slot0 + i).wait()
            before(it)
            work = side(it)
            for i in range(npair):
                project_pair(mat, first + i, slot0 + i, work)

            @pl.when(first + NSLOT < 16)
            def _():
                for i in range(npair):
                    w_copy(mat, first + NSLOT + i, slot0 + i).start()

            if mat < 2:
                @pl.when(first + NSLOT >= 16)
                def _():
                    for i in range(npair):
                        w_copy(mat + 1, first + NSLOT - 16 + i, slot0 + i).start()

            after(it)

    def nothing(it):
        return None

    def fetch_a_inputs(it):
        for cp in a_copies(it):
            cp.start()

    def wait_a_inputs(it):
        for cp in a_copies(it):
            cp.wait()

    def in_slots(units, table):
        for slot in table:
            for unit, kind, index in slot.split():
                units[int(unit)][kind](int(index))
            yield

    def forward_fft(it):
        return in_slots([a_forward(it, odd) for odd in range(2)], FORWARD_SLOTS)

    def fetch_wo(it):
        wo_copy(it).start()

    def inverse_fft(it):
        halves = []
        return in_slots([a_inverse(it, odd, halves) for odd in range(2)], INVERSE_SLOTS)

    for i in range(2):
        w_copy(0, i, i).wait()
        regroup_pair(0, i, i)
        w_copy(0, NSLOT + i, i).start()
    fetch_a_inputs(0)

    @pl.loop(0, 4)
    def _(j):
        xpre_copy(j).wait()
        x = xpre3[pl.ds(8 * j, 8)].reshape(128, D)
        xpre[pl.ds(pl.multiple_of(j * 64, 64), 64), :] = pltpu.bitcast(x, U32)
        w = jnp.concatenate([wqkv[3 * hd] for hd in range(4)], axis=1)
        p = _dot(x, _bf(w)).astype(BF16)
        for hd in range(4):
            pre[0, hd, pl.ds(pl.multiple_of(j * 128, 128), 128), :] = p[:, DH * hd:DH * (hd + 1)]

    project_loop(0, 2, nothing, nothing, fetch_a_inputs, start=1)
    for cp in filter_stage_copies:
        cp.start()
    mf_copy.wait()
    project_loop(1, 2, wait_a_inputs, forward_fft, fetch_wo)
    for cp in step_copies:
        cp.start()
    for cp in filter_stage_copies:
        cp.wait()
    a_filter(0, a_nyquist())
    pl.loop(1, 4)(a_filter)
    project_loop(2, 2, nothing, inverse_fft, nothing)
    for c in range(8):
        y_copy(c).start()

    for cp in step_copies + [wo_copy(n) for n in range(8)]:
        cp.wait()

    def segment(s, h, split):
        row = lax.broadcasted_iota(jnp.int32, (32, 48), 0)
        col = lax.broadcasted_iota(jnp.int32, (32, 48), 1)
        allowed = ((row < NMEM) | (col >= 32) | (col <= row)) & (col < 40)
        p0 = pl.ds(pl.multiple_of(s * 8, 8), 8)
        zeros = jnp.zeros((8, DH), BF16)
        st = {}

        def half(i, a):
            return _dot(h[:, 512 * a:512 * (a + 1)], _bf(wqkv[i, 256 * a:256 * (a + 1), :]))

        def qkv(hd):
            if hd == 0 and split:
                for i in range(3):
                    part[i] = half(i, 0)
                q, k, v = [(part[i] + half(i, 1)).astype(BF16) for i in range(3)]
            else:
                q, k, v = [_dot(h, _bf(wqkv[3 * hd + i])).astype(BF16) for i in range(3)]
            kvmem[0, hd, p0, :] = k[:NMEM]
            kvmem[1, hd, p0, :] = v[:NMEM]
            st[hd] = (q, k, v)

        def scores(hd):
            q, k, v = st[hd]
            ka = jnp.concatenate([k, pre[1, hd, p0, :], zeros], axis=0)
            sc = jnp.where(allowed, _dot_nt(q, ka) * scale, -jnp.inf)
            st[hd] = (_softmax(sc).astype(BF16), v)

        def context(hd):
            p, v = st.pop(hd)
            va = jnp.concatenate([v, pre[2, hd, p0, :], zeros], axis=0)
            obuf[:, hd * DH:(hd + 1) * DH] = _dot(p, va).astype(BF16)

        acc = [None] * 8

        def project(g):
            lhs = obuf[:, 4 * g * DH:4 * (g + 1) * DH]
            for n in range(8):
                t = _dot(lhs, _bf(wo[n, 256 * g:256 * (g + 1), :]))
                acc[n] = t if acc[n] is None else acc[n] + t

        lag_scores, lag_context = 1, 3
        for hd in range(H):
            qkv(hd)
            if hd >= lag_scores:
                scores(hd - lag_scores)
            if hd >= lag_context:
                context(hd - lag_context)
            if hd == 28:
                project(0)
        for t, g in enumerate(range(1, H // 4)):
            project(g)
            if t < lag_scores:
                scores(H + t - lag_scores)
            if t < lag_context:
                context(H + t - lag_context)
        return acc

    @pl.loop(0, NSEG // 4)
    def _(i):
        h = xs[2 * i, 0].reshape(32, D)
        for u in range(4):
            acc = segment(4 * i + u, h, u > 0)
            if u < 3:
                xt = xs[2 * i + (u + 1) // 2, (u + 1) % 2, pl.ds(1, 3)].astype(F32).reshape(24, D)
                h = jnp.concatenate(
                    [jnp.concatenate([acc[n][:NMEM], xt[:, 128 * n:128 * (n + 1)]],
                                     axis=0).astype(BF16) for n in range(8)], axis=1)
            ob = jnp.concatenate(acc, axis=1).astype(BF16).reshape(4, 8, D)
            xs[2 * i + u // 2, u % 2, pl.ds(1, 3)] = ob[1:]
        xs[2 * i + 2, 0, 0] = ob[0]

    o_copy.start()

    @pl.loop(0, 4)
    def _(g):
        row = lax.broadcasted_iota(jnp.int32, (64, 128), 0)
        col = lax.broadcasted_iota(jnp.int32, (64, 128), 1)
        allowed = ((col % 64) // 8 == row // 8) & ((col < 64) | (col % 8 <= row % 8))
        st = {}

        def rows(a):
            return pl.ds(pl.multiple_of(g * 128 + a * 64, 64), 64)

        def scores(hd):
            for a in range(2):
                ka = jnp.concatenate([kvmem[0, hd, rows(a), :], pre[1, hd, rows(a), :]], axis=0)
                sc = jnp.where(allowed, _dot_nt(pre[0, hd, rows(a), :], ka) * scale, -jnp.inf)
                st[hd, a] = _softmax(sc).astype(BF16)

        def context(hd):
            for a in range(2):
                va = jnp.concatenate([kvmem[1, hd, rows(a), :], pre[2, hd, rows(a), :]], axis=0)
                opre[a * 64:(a + 1) * 64, hd * DH:(hd + 1) * DH] = (
                    _dot(st.pop((hd, a)), va).astype(BF16))

        acc = None
        for c in range(H // 8 + 2):
            if c < H // 8:
                for hd in range(8 * c, 8 * c + 8):
                    scores(hd)
            if c >= 2:
                lhs = opre[:, 8 * (c - 2) * DH:8 * (c - 1) * DH]
                t = jnp.concatenate([_dot(lhs, _bf(wo[n, 512 * (c - 2):512 * (c - 1), :]))
                                     for n in range(8)], axis=1)
                acc = t if acc is None else acc + t
            if 1 <= c <= H // 8:
                for hd in range(8 * (c - 1), 8 * c):
                    context(hd)
        xs[pl.ds(g * 8, 8), :, 0] = acc.astype(BF16).reshape(8, 2, 8, D)
        opre_copy(g).start()

    for cp in [y_copy(c) for c in range(8)] + [o_copy] + [opre_copy(g) for g in range(4)]:
        cp.wait()


@functools.partial(jax.jit, static_argnames=("B_seg_len",))
def pallas_concat_heads__spectral_gfnet__memory_aug_recurrent_mem_tr__prompt_kernel(
    A_x, A_w_r, A_w_i, B_x, B_mem0, B_Wq, B_Wk, B_Wv, B_Wo, B_seg_len=SEG,
):
    assert A_x.shape == (1, S, D) and B_x.shape == (1, S, D)
    assert A_w_r.shape == A_w_i.shape == (S, D // 2 + 1)
    assert B_mem0.shape == (1, NMEM, D) and B_seg_len == SEG
    assert B_Wq.shape == B_Wk.shape == B_Wv.shape == (D, H, DH) and B_Wo.shape == (H, DH, D)

    vmem = pltpu.VMEM
    dma = pltpu.SemaphoreType.DMA
    scratch = [
        vmem((8, 32, 8, D), BF16),
        vmem((32 * 256 + 32, 128), U32),
        vmem((2, 1, S), BF16),
        vmem((4 * WP_ROWS + 32, 128), U32),
        vmem((4, 64, 256), U32),
        vmem((4, 64, 256), U32),
        vmem((5, 64, 128), U32),
        vmem((2, 64, 128), F32),
        vmem((32, 64, 128), U32),
        vmem((32, 64, 128), U32),
        vmem((32, 4, 128, 128), BF16),
        vmem((32, 128, 512), F32),
        vmem((64, 128), F32),
        vmem((33, 2, 4, 8, D), BF16),
        vmem((32, 2, 8, D), BF16),
        vmem((NPRE // 2, D), U32),
        vmem((NSLOT * D + 32, 128), U32),
        vmem((3 * H, D // 2, DH), U32),
        vmem((8, H * DH // 2, 128), U32),
        vmem((3, H, NPRE, DH), BF16),
        vmem((2, H, NPRE, DH), BF16),
        vmem((32, H * DH), BF16),
        vmem((128, H * DH), BF16),
        vmem((3, 32, DH), F32),
        dma((4,)), dma((12,)), dma((NSLOT,)),
    ]
    hbm = pl.BlockSpec(memory_space=pltpu.HBM)
    out = pl.pallas_call(
        _kernel,
        out_shape=jax.ShapeDtypeStruct((32, 2, 4, 8, 2 * D), BF16),
        in_specs=[hbm] * 15,
        out_specs=hbm,
        scratch_shapes=scratch,
        compiler_params=pltpu.CompilerParams(vmem_limit_bytes=124 * 1024 * 1024),
    )(A_x.reshape(32, 8, 8, D), A_w_r.T, A_w_i.T,
      B_x.reshape(32, 2, 4, 8, D), B_mem0.reshape(NMEM, D),
      B_Wq, B_Wk, B_Wv, B_Wo.reshape(H * DH, D),
      *[jnp.asarray(c) for c in _fft_constants()])
    return out.reshape(1, S, 2 * D)
```
